```python
import jax
import jax.numpy as jnp

def _softmax(x, axis=-1):
    return jax.nn.softmax(x, axis=axis)

def _gelu(x):
    return jax.nn.gelu(x, approximate=True)

def _silu(x):
    return jax.nn.silu(x)

def _sigmoid(x):
    return jax.nn.sigmoid(x)

def _layernorm(x, axis=-1, eps=1e-05):
    m = jnp.mean(x, axis=axis, keepdims=True)
    v = jnp.var(x, axis=axis, keepdims=True)
    return (x - m) / jnp.sqrt(v + eps)

def _scatter_add(tgt, idx, src, axis=0):
    return tgt.at[idx].add(src)

def _segment_sum(src, seg, n):
    return jax.ops.segment_sum(src, seg, n)

class _Rng:

    def __init__(self, key):
        self._k = key

    def _next(self):
        self._k, sub = jax.random.split(self._k)
        return sub

    def normal(self, shape):
        return jax.random.normal(self._next(), shape, dtype=jnp.bfloat16)

    def randint(self, lo, hi, shape):
        return jax.random.randint(self._next(), shape, lo, hi, dtype=jnp.int32)

    def uniform(self, shape, lo=0.0, hi=1.0):
        return jax.random.uniform(self._next(), shape, jnp.bfloat16, lo, hi)

    def permutation(self, n):
        return jax.random.permutation(self._next(), n)
kernel_name = 'adaLN_cond__compressed_kv_cla__moe_arch_mod__prompt'

def setup_inputs():
    _rng = _Rng(jax.random.key(int.from_bytes(__import__("os").urandom(4), "little")))
    _w = lambda a: (lambda t: t.astype(jnp.bfloat16) if jnp.issubdtype(t.dtype, jnp.floating) else t)(jnp.asarray(a))

    def _A_setup():
        B, H, Sq, Sk, D, M = (1, 32, 2048, 2048, 128, 640)
        Dc = 4 * D
        return {'x': _w((lambda *s: _rng.normal(s) * 0.05)(B, Sq, M)), 'c_kv': _w((lambda *s: _rng.normal(s) * 0.05)(B, Sk, Dc)), 'w_q': _w((lambda *s: _rng.normal(s) * 0.05)(M, H, D) * M ** (-0.5)), 'w_uk': _w((lambda *s: _rng.normal(s) * 0.05)(Dc, H, D) * Dc ** (-0.5)), 'w_uv': _w((lambda *s: _rng.normal(s) * 0.05)(Dc, H, D) * Dc ** (-0.5)), 'w_o': _w((lambda *s: _rng.normal(s) * 0.05)(H, D, M) * (H * D) ** (-0.5))}
    _A_in = _A_setup()

    def _B_setup():
        B, S, D, F, C = (1, 2048, 640, 1728, 8)
        return {'x': _w((lambda *s: _rng.normal(s) * 0.05)(B, S, D)), 'w_r': _w((lambda *s: _rng.normal(s) * 0.05)(D)), 'w_gate': _w((lambda *s: _rng.normal(s) * 0.05)(D, F)), 'w_up': _w((lambda *s: _rng.normal(s) * 0.05)(D, F)), 'w_down': _w((lambda *s: _rng.normal(s) * 0.05)(F, D))}
    _B_in = _B_setup()
    return {'A_x': _A_in['x'], 'A_c_kv': _A_in['c_kv'], 'A_w_q': _A_in['w_q'], 'A_w_uk': _A_in['w_uk'], 'A_w_uv': _A_in['w_uv'], 'A_w_o': _A_in['w_o'], 'B_x': _B_in['x'], 'B_w_r': _B_in['w_r'], 'B_w_gate': _B_in['w_gate'], 'B_w_up': _B_in['w_up'], 'B_w_down': _B_in['w_down'], 'c': _w((lambda *s: _rng.normal(s) * 0.05)(1, 640)), 'w_mod': _w((lambda *s: _rng.normal(s) * 0.05)(640, 6 * 640) * 640 ** (-0.5))}

def reference(A_x, A_c_kv, A_w_q, A_w_uk, A_w_uv, A_w_o, B_x, B_w_r, B_w_gate, B_w_up, B_w_down, c, w_mod):

    def _A_ref(x, c_kv, w_q, w_uk, w_uv, w_o):
        B, Sq, M = (x.shape[0], x.shape[1], x.shape[2])
        Sk = c_kv.shape[1]
        H, D = (w_q.shape[1], w_q.shape[2])
        q = jnp.einsum('bqm,mhd->bhqd', x, w_q)
        k = jnp.einsum('bkc,chd->bhkd', c_kv, w_uk)
        v = jnp.einsum('bkc,chd->bhkd', c_kv, w_uv)
        scores = jnp.einsum('bhqd,bhkd->bhqk', q, k) * D ** (-0.5)
        off = Sk - Sq
        qi = jnp.arange(Sq)[:, None]
        kj = jnp.arange(Sk)[None, :]
        cmask = kj <= qi + off
        scores = jnp.where(cmask[None, None], scores, -1000000000.0)
        p = _softmax(scores, axis=-1)
        ctx = jnp.einsum('bhqk,bhkd->bhqd', p, v)
        return jnp.einsum('bhqd,hdm->bqm', ctx, w_o)

    def _B_ref(x, w_r, w_gate, w_up, w_down):
        B, S, D = x.shape
        C = 8
        r = x @ w_r
        idx = jnp.argsort(-r, axis=-1)[:, :C]
        idx_e = jnp.repeat(idx.reshape(B, C, 1), D, axis=2)
        x_sel = jnp.take_along_axis(x, idx_e, axis=1)
        g = _silu(x_sel @ w_gate)
        u = x_sel @ w_up
        y = g * u @ w_down
        r_sel = _sigmoid(jnp.take_along_axis(r, idx, axis=1))
        y = y * r_sel.reshape(B, C, 1)
        b_off = (jnp.arange(B) * S).reshape(B, 1)
        flat_idx = (idx + b_off).reshape(B * C)
        zero = (x * 0.0).reshape(B * S, D)
        upd = _scatter_add(zero, flat_idx, y.reshape(B * C, D), axis=0)
        return x + upd.reshape(B, S, D)
    x = A_x
    mod = (_silu(c) @ w_mod).reshape(c.shape[0], 6, 1, -1)
    sa, ca, ga, sb, cb, gb = (mod[:, 0].copy(), mod[:, 1].copy(), mod[:, 2].copy(), mod[:, 3].copy(), mod[:, 4].copy(), mod[:, 5].copy())
    h = _layernorm(x, axis=-1) * (1 + ca) + sa
    x = x + ga * _A_ref(h, A_c_kv, A_w_q, A_w_uk, A_w_uv, A_w_o)
    h = _layernorm(x, axis=-1) * (1 + cb) + sb
    x = x + gb * _B_ref(h, B_w_r, B_w_gate, B_w_up, B_w_down)
    return x
```

```python
import jax
import jax.numpy as jnp
from jax import lax
import jax.experimental.pallas as pl
import jax.experimental.pallas.tpu as pltpu

BF = jnp.bfloat16
F32 = jnp.float32
I32 = jnp.int32
U32 = jnp.uint32

S = 2048
M = 640
C = 512
H = 32
D = 128
F = 1728
TOPK = 8
EPS = 1e-5
LOG2E = 1.4426950408889634
QSCALE = D ** -0.5 * LOG2E
MASKED = -1e9 * LOG2E

T = 128
BQ = 256
CH = 32
MT = M // T
CT = C // T

_OFF = {}
_ROWS = 0
for _name, _n in (
    ("H", MT * S // 2), ("C", CT * S // 2),
    ("Q", S // 2), ("K", S // 2), ("V", S // 2), ("X", S // 2),
    ("Wq", M // 2), ("Wk", C // 2), ("Wv", C // 2),
    ("S", 2 * (S // T) * BQ), ("SD", S // 2),
    ("MX", S), ("M", S), ("L", S), ("ACC", 3 * BQ), ("PA", S),
    ("O", MT * S), ("D", T),
):
    _OFF[_name] = _ROWS
    _ROWS += _n

_SEQ = (
    "q0 k0 q1 k1 v0 v1 A0+A1 A0 q2 k2 B0 A1 q3 v2 B1 B0+A2 A2 k3 q4 v3 "
    "B2 B1+A3 A3 k4 o0 v4 B3 B2+A4 A4 q5 k5 v5 o1 B4 B3+A5 A5 q6 k6 v6 o2 "
    "B5 B4+A6 A6 q7 k7 v7 o3 B6 B5+A7 A7 o4 o5 B6+B7 B7 o6 o7"
)
_RES_LAG, _CTX_LAG, _MAX_LAG, _SUM_LAG = 200, 240, 128, 32


def _slots():
    lanes = []
    for word in _SEQ.split():
        if "+" in word:
            lanes.append(tuple(
                (p[0], int(p[1:]), 2 * int(p[1:]) + 1, T) for p in word.split("+")))
        else:
            k, i = word[0], int(word[1:])
            n = {"q": MT, "k": CT, "v": CT, "o": MT, "A": 2 * i + 1, "B": 2 * i + 1}[k]
            lanes += [((k, i, j, 0),) for j in range(n)]
    assert len(lanes) % 4 == 0
    return [lanes[s:s + 4] for s in range(0, len(lanes), 4)]


def _nt(a, b):
    return lax.dot_general(a, b, (((1,), (1,)), ((), ())), preferred_element_type=F32)


def _nn(a, b):
    return jnp.dot(a, b, preferred_element_type=F32)


def _rnd(x):
    return x.astype(BF).astype(F32)


def _pack(x):
    return pltpu.bitcast(x.astype(BF), F32)


def _select_head(src, slot, r, parity):
    even = pltpu.bitcast(src[slot, r // 2:r // 2 + 8, 0], U32).reshape(8, T)
    odd = pltpu.bitcast(src[slot, r // 2:r // 2 + 8, 1], U32).reshape(8, T)
    down = (16 * parity).astype(U32)
    word = ((even >> down) & 0xFFFF) | ((odd >> down) << 16)
    return pltpu.bitcast(word, F32)


def _head(w, zero, wo, pairs, next_slot, next_parity):
    def ordered(r, n):
        return w[pl.ds(zero + r, n), :]

    def load(r, n):
        return w[r:r + n, :]

    def store(r, v):
        w[r:r + v.shape[0], :] = v

    def s_row(i, j, t, half):
        if half:
            return _OFF["SD"] + i * T + t - T
        return _OFF["S"] + ((i % 2) * (S // T) + j) * BQ + t

    events = []

    def at(time, rank, fn):
        events.append((time, rank, len(events), fn))

    slots = _slots()
    left = {}
    for slot in slots:
        for lane in slot:
            for k, i, _, t0 in lane:
                for t in range(t0, BQ, CH):
                    left[k, i, t] = left.get((k, i, t), 0) + 1
    has_sum, has_acc, last_use = set(), set(), {}

    for s, slot in enumerate(slots):
        base = BQ * s
        jobs = ([(lane[0], -T) for lane in slot if len(lane) == 2]
                + [(lane[0], 0) for lane in slot if len(lane) == 1]
                + [(lane[1], 0) for lane in slot if len(lane) == 2])
        lhs, res, groups = {}, {}, {}
        for job, shift in jobs:
            groups.setdefault((job[0], job[1], shift), []).append(job)
            last_use[job[0]] = base + BQ

        for (k, i, shift), group in groups.items():
            for t in range(0, BQ, CH):
                live = [job for job in group if t >= job[3]]
                if not live:
                    continue

                def fetch(k=k, i=i, t=t, live=live, lhs=lhs, first=(i, t) not in has_sum):
                    r = i * BQ + t
                    if k in "qkv":
                        src = _OFF["H" if k == "q" else "C"] + r // 2
                        for job in live:
                            get = ordered if job == live[0] else load
                            lhs[job, t] = get(src + job[2] * S // 2, CH // 2)
                    elif k in "Ao":
                        v = ordered(_OFF["Q" if k == "A" else "X"] + r // 2, CH // 2)
                        for job in live:
                            lhs[job, t] = v
                            if k == "A" and job[2] == 2 * i + t // T:
                                lhs["d", job, t] = ordered(_OFF["D"] + t % T, 8)
                    else:
                        m = ordered(_OFF["M"] + r, CH)
                        l = None if first else load(_OFF["L"] + r, CH)
                        for job in live:
                            p = jnp.exp2(load(s_row(i, job[2], t, job[3]), CH) - m)
                            l = p if l is None else l + p
                            lhs[job, t] = p
                        lhs["l", i, t] = l

                at(base + shift + t, 1, fetch)
                if k == "B":
                    has_sum.add((i, t))
                    at(base + shift + t + CH - 16 + _SUM_LAG, 0,
                       lambda i=i, t=t, lhs=lhs: store(_OFF["L"] + i * BQ + t, lhs["l", i, t]))

        for job, shift in jobs:
            def matmul(job=job, lhs=lhs, res=res):
                k, _, j, t0 = job
                a = jnp.concatenate([lhs[job, t] for t in range(t0, BQ, CH)], axis=0)
                a = a.astype(BF) if k == "B" else pltpu.bitcast(a, BF)
                if k == "o":
                    res[job] = _nn(a, wo[:, j * T:(j + 1) * T])
                    return
                region = {"A": "K", "B": "V"}.get(k, "W" + k)
                b = pltpu.bitcast(load(_OFF[region] + j * T // 2, T // 2), BF)
                res[job] = _nt(a, b) if k == "A" else _nn(a, b)

            at(base + shift + BQ - CH, 2, matmul)

        for (k, i, shift), group in groups.items():
            for t in range(0, BQ, CH):
                live = [job for job in group if t >= job[3]]
                if not live:
                    continue
                first = (k, i, t) not in has_acc
                has_acc.add((k, i, t))
                left[k, i, t] -= len(live)
                last = left[k, i, t] == 0

                def finish(k=k, i=i, t=t, live=live, lhs=lhs, res=res, first=first, last=last):
                    r = i * BQ + t
                    parts = [res[job][t - job[3]:t - job[3] + CH] for job in live]
                    if k == "o":
                        for job, v in zip(live, parts):
                            a = _OFF["O"] + job[2] * S + r
                            store(a, load(a, CH) + v)
                    elif k == "A":
                        mx = None if first else load(_OFF["MX"] + r, CH)
                        for job, v in zip(live, parts):
                            if job[2] == 2 * i + t // T:
                                d = lhs["d", job, t]
                                v = jnp.concatenate(
                                    [jnp.where(d <= u, v[u:u + 8], MASKED)
                                     for u in range(0, CH, 8)], axis=0)
                            store(s_row(i, job[2], t, job[3]), v)
                            mx = v if mx is None else jnp.maximum(mx, v)
                        if last:
                            res["m", i, t] = jnp.broadcast_to(
                                jnp.max(mx, axis=1, keepdims=True), (CH, T))
                        else:
                            store(_OFF["MX"] + r, mx)
                    else:
                        a = _OFF["PA"] + r if k == "B" else _OFF["ACC"] + "qkv".index(k) * BQ + t
                        acc = None if first else load(a, CH)
                        for v in parts:
                            acc = v if acc is None else acc + v
                        if not last:
                            store(a, acc)
                        elif k == "B":
                            l = jnp.sum(load(_OFF["L"] + r, CH), axis=1, keepdims=True)
                            store(_OFF["X"] + r // 2, _pack(acc * (1.0 / l)))
                        elif k == "q":
                            store(_OFF["Q"] + r // 2, _pack(acc * QSCALE))
                        else:
                            store(_OFF[k.upper()] + r // 2, _pack(acc))

                ready = base + shift + t + CH - 16 + (_CTX_LAG if k == "B" and last else _RES_LAG)
                when = max(base + shift + BQ, ready)
                at(when, 0, finish)
                if k == "A" and last:
                    at(max(when, ready + _MAX_LAG), 0,
                       lambda i=i, t=t, res=res: store(_OFF["M"] + i * BQ + t, res["m", i, t]))

    todo = [(k, r) for k, n in (("q", M), ("k", C), ("v", C)) for r in range(0, n, 16)]
    start = max(last_use[k] for k in "qkv")
    span = BQ * (len(slots) - 1) - start
    for n, (k, r) in enumerate(todo):
        at(start + span * n // len(todo), 0,
           lambda k=k, r=r: store(_OFF["W" + k] + r // 2,
                                  _select_head(pairs[k], next_slot, r, next_parity)))

    for event in sorted(events, key=lambda e: e[:3]):
        event[3]()


def _norm2(x1, scale, shift):
    mean = jnp.mean(x1, axis=1, keepdims=True)
    var = jnp.mean(jnp.square(x1 - mean), axis=1, keepdims=True)
    std = _rnd(jnp.sqrt(_rnd(_rnd(var) + EPS)))
    n = _rnd(_rnd(x1 - _rnd(mean)) * (1.0 / std))
    return (_rnd(n * scale) + shift).astype(BF)


def _kernel(x_hbm, ckv_hbm, wq_hbm, wk_hbm, wv_hbm, wo_hbm, wr_hbm, wg_hbm, wu_hbm,
            wd_hbm, c_hbm, wmod_hbm, out_hbm,
            w, x_v, ckv_v, wq_v, wk_v, wv_v, wo_v, wr_v, wg_v, wu_v, wd_v, c_v,
            wmod_a, wmod_b, out_v, sem_in, sem_x, sem_c, sem_w, sem_o, sem_out, sem_fix):
    pairs = {"q": wq_v, "k": wk_v, "v": wv_v}
    nb = S // BQ

    def rows(i):
        return pl.ds(i * BQ, BQ)

    def pair_copies(p):
        heads = pl.ds(2 * p, 2)
        return [pltpu.make_async_copy(src.at[:, :, heads, :], dst.at[p % 2], sem_w.at[3 * (p % 2) + n])
                for n, (src, dst) in enumerate(((wq_hbm, wq_v), (wk_hbm, wk_v), (wv_hbm, wv_v)))]

    def wo_copy(h):
        return pltpu.make_async_copy(wo_hbm.at[h], wo_v.at[h % 2], sem_o.at[h % 2])

    c_copy = pltpu.make_async_copy(c_hbm, c_v, sem_in.at[0])
    mod_a_copy = pltpu.make_async_copy(wmod_hbm.at[:, pl.ds(0, 2 * M)], wmod_a, sem_in.at[1])
    x_copies = [pltpu.make_async_copy(x_hbm.at[rows(i)], x_v.at[rows(i)], sem_x.at[i])
                for i in range(nb)]
    ckv_copies = [pltpu.make_async_copy(ckv_hbm.at[rows(i)], ckv_v.at[rows(i)], sem_c.at[i])
                  for i in range(nb)]
    late_copies = [
        pltpu.make_async_copy(src, dst, sem_in.at[2 + n]) for n, (src, dst) in enumerate((
            (wmod_hbm.at[:, pl.ds(2 * M, 4 * M)], wmod_b), (wr_hbm, wr_v),
            (wg_hbm, wg_v), (wu_hbm, wu_v), (wd_hbm, wd_v)))]
    for copy in [c_copy, mod_a_copy] + pair_copies(0) + x_copies + ckv_copies + [wo_copy(0)]:
        copy.start()

    w[_OFF["O"]:_OFF["O"] + MT * S, :] = jnp.zeros((MT * S, T), F32)
    w[_OFF["D"]:_OFF["D"] + T, :] = (
        lax.broadcasted_iota(I32, (T, T), 1) - lax.broadcasted_iota(I32, (T, T), 0)).astype(F32)

    def silu_c():
        c = jnp.broadcast_to(c_v[...].astype(F32), (16, M))
        return (c * jax.nn.sigmoid(c)).astype(BF)

    c_copy.wait()
    mod_a_copy.wait()
    mod = _rnd(_nn(silu_c(), wmod_a[...])[:1])
    shift_a, scale_a = mod[:, :M], _rnd(1.0 + mod[:, M:])

    for copy in pair_copies(0):
        copy.wait()
    for k, n in (("q", M), ("k", C), ("v", C)):
        for r in range(0, n, 16):
            a = _OFF["W" + k] + r // 2
            w[a:a + 8, :] = _select_head(pairs[k], 0, r, jnp.zeros((), I32))

    for i in range(nb):
        x_copies[i].wait()
        x = x_v[rows(i), :].astype(F32)
        xc = x - jnp.mean(x, axis=1, keepdims=True)
        var = jnp.mean(xc * xc, axis=1, keepdims=True)
        h = _pack(xc * lax.rsqrt(var + EPS) * scale_a + shift_a)
        for j in range(MT):
            a = _OFF["H"] + (j * S + i * BQ) // 2
            w[a:a + BQ // 2, :] = h[:, j * T:(j + 1) * T]
    for i in range(nb):
        ckv_copies[i].wait()
        ckv = pltpu.bitcast(ckv_v[rows(i), :], F32)
        for j in range(CT):
            a = _OFF["C"] + (j * S + i * BQ) // 2
            w[a:a + BQ // 2, :] = ckv[:, j * T:(j + 1) * T]
    for copy in late_copies:
        copy.start()

    def head_step(h, carry):
        nxt = jnp.minimum(h + 1, H - 1)
        wo_copy(h).wait()

        @pl.when(h + 1 < H)
        def _():
            wo_copy(h + 1).start()

        @pl.when(jnp.logical_and(h % 2 == 0, h + 2 < H))
        def _():
            for copy in pair_copies(h // 2 + 1):
                copy.start()

        @pl.when(jnp.logical_and(h % 2 == 1, h + 1 < H))
        def _():
            for copy in pair_copies(h // 2 + 1):
                copy.wait()

        zero = pl.multiple_of((h // H) * 16, 16)
        _head(w, zero, wo_v.at[h % 2], pairs, (nxt // 2) % 2, nxt % 2)
        return carry

    lax.fori_loop(0, H, head_step, 0)

    for copy in late_copies:
        copy.wait()
    mod = _rnd(_nn(silu_c(), wmod_b[...])[:1])
    gate_a, shift_b = mod[:, :M], mod[:, M:2 * M]
    scale_b, gate_b = _rnd(1.0 + mod[:, 2 * M:3 * M]), mod[:, 3 * M:]
    w_r = jnp.broadcast_to(wr_v[...].astype(F32).reshape(1, M), (16, M)).astype(BF)

    out_copies = [pltpu.make_async_copy(out_v.at[rows(i)], out_hbm.at[rows(i)], sem_out.at[i])
                  for i in range(nb)]
    sub = lax.broadcasted_iota(I32, (nb, BQ), 0)
    score = jnp.zeros((nb, BQ), F32)
    for i in range(nb):
        attn = jnp.concatenate(
            [w[_OFF["O"] + j * S + i * BQ:_OFF["O"] + j * S + (i + 1) * BQ, :] for j in range(MT)],
            axis=1)
        x1 = _rnd(x_v[rows(i), :].astype(F32) + gate_a * attn)
        for j in range(MT):
            a = _OFF["O"] + j * S + i * BQ
            w[a:a + BQ, :] = x1[:, j * T:(j + 1) * T]
        h2 = _norm2(x1, scale_b, shift_b)
        out_v[rows(i), :] = (x1 + gate_b * h2.astype(F32)).astype(BF)
        out_copies[i].start()
        score = jnp.where(sub == i, _nt(w_r, h2)[:nb], score)

    score = _rnd(score)
    bits = pltpu.bitcast(jnp.where(score == 0.0, 0.0, score), I32) >> 16
    rank = jnp.where(bits < 0, -1 - bits, bits + 0x8000)
    rank = jnp.where(score != score, 0, rank)
    row = sub * BQ + lax.broadcasted_iota(I32, (nb, BQ), 1)
    key = pltpu.bitcast((rank << 11) | (S - 1 - row) | (1 << 29), F32)
    picked = []
    for _ in range(TOPK):
        top = jnp.max(jnp.max(key, axis=1, keepdims=True), axis=0, keepdims=True)
        key = jnp.where(key == top, 0.0, key)
        top = pltpu.bitcast(jnp.broadcast_to(top, (8, T)), I32)
        picked.append(S - 1 - (top[0, 0] & (S - 1)))

    x1 = jnp.concatenate(
        [jnp.concatenate([w[pl.ds(_OFF["O"] + j * S + r, 1), :] for j in range(MT)], axis=1)
         for r in picked], axis=0)
    h2 = _norm2(x1, scale_b, shift_b)
    g = _rnd(_nt(h2, wg_v[...]))
    u = _rnd(_nt(h2, wu_v[...]))
    y = _nn((_rnd(g * jax.nn.sigmoid(g)) * u).astype(BF), wd_v[...])
    r_sel = _rnd(jnp.sum(h2.astype(F32) * w_r[:TOPK].astype(F32), axis=1, keepdims=True))
    new = x1 + gate_b * (h2.astype(F32) + y * jax.nn.sigmoid(r_sel))

    for copy in out_copies:
        copy.wait()
    groups = [pl.ds(pl.multiple_of((r // 16) * 16, 16), 16) for r in picked]
    line = lax.broadcasted_iota(I32, (16, M), 0)
    for n, r in enumerate(picked):
        old = out_v[groups[n], :].astype(F32)
        out_v[groups[n], :] = jnp.where(line == r % 16, new[n:n + 1], old).astype(BF)

    fixes = []
    for n, r in enumerate(picked):
        fresh = True
        for earlier in picked[:n]:
            fresh = jnp.logical_and(fresh, earlier // 16 != r // 16)
        fixes.append((fresh, pltpu.make_async_copy(
            out_v.at[groups[n]], out_hbm.at[groups[n]], sem_fix.at[n])))
    for fresh, copy in fixes:
        pl.when(fresh)(copy.start)
    for fresh, copy in fixes:
        pl.when(fresh)(copy.wait)


@jax.jit
def pallas_adaLN_cond__compressed_kv_cla__moe_arch_mod__prompt_kernel(
    A_x: jax.Array,
    A_c_kv: jax.Array,
    A_w_q: jax.Array,
    A_w_uk: jax.Array,
    A_w_uv: jax.Array,
    A_w_o: jax.Array,
    B_x: jax.Array,
    B_w_r: jax.Array,
    B_w_gate: jax.Array,
    B_w_up: jax.Array,
    B_w_down: jax.Array,
    c: jax.Array,
    w_mod: jax.Array,
):
    del B_x
    assert A_x.shape == (1, S, M) and A_c_kv.shape == (1, S, C)
    assert A_w_q.shape == (M, H, D) and B_w_gate.shape == (M, F)
    dma = pltpu.SemaphoreType.DMA
    out = pl.pallas_call(
        _kernel,
        in_specs=[pl.BlockSpec(memory_space=pl.ANY)] * 12,
        out_specs=pl.BlockSpec(memory_space=pl.ANY),
        out_shape=jax.ShapeDtypeStruct((S, M), BF),
        scratch_shapes=[
            pltpu.VMEM((_ROWS, T), F32),
            pltpu.VMEM((S, M), BF), pltpu.VMEM((S, C), BF),
            pltpu.VMEM((2, M // 2, 2, 2, D), BF), pltpu.VMEM((2, C // 2, 2, 2, D), BF),
            pltpu.VMEM((2, C // 2, 2, 2, D), BF), pltpu.VMEM((2, D, M), BF),
            pltpu.VMEM((M,), BF),
            pltpu.VMEM((F, M), BF), pltpu.VMEM((F, M), BF), pltpu.VMEM((F, M), BF),
            pltpu.VMEM((1, M), BF),
            pltpu.VMEM((M, 2 * M), BF), pltpu.VMEM((M, 4 * M), BF),
            pltpu.VMEM((S, M), BF),
            dma((7,)), dma((S // BQ,)), dma((S // BQ,)), dma((6,)), dma((2,)),
            dma((S // BQ,)), dma((TOPK,)),
        ],
        compiler_params=pltpu.CompilerParams(vmem_limit_bytes=100 * 2 ** 20),
        name="adaln_attn_moe",
    )(A_x[0], A_c_kv[0], A_w_q.reshape(M // 2, 2, H, D), A_w_uk.reshape(C // 2, 2, H, D),
      A_w_uv.reshape(C // 2, 2, H, D), A_w_o, B_w_r,
      B_w_gate.T, B_w_up.T, B_w_down, c, w_mod)
    return out[None]
```

```python
import jax
import jax.numpy as jnp
from jax import lax
import jax.experimental.pallas as pl
import jax.experimental.pallas.tpu as pltpu

BF = jnp.bfloat16
F32 = jnp.float32
I32 = jnp.int32
U32 = jnp.uint32

S = 2048
M = 640
C = 512
H = 32
D = 128
F = 1728
TOPK = 8
EPS = 1e-5
LOG2E = 1.4426950408889634
QSCALE = D ** -0.5 * LOG2E
MASKED = -1e9 * LOG2E

T = 128
BQ = 256
CH = 32
MT = M // T
CT = C // T

_OFF = {}
_ROWS = 0
for _name, _n in (
    ("H", MT * S // 2), ("C", CT * S // 2),
    ("Q", S // 2), ("K", S // 2), ("V", S // 2), ("X", S // 2),
    ("Wq", M // 2), ("Wk", C // 2), ("Wv", C // 2),
    ("S", (S // BQ) ** 2 * BQ), ("SD", S // 2),
    ("MX", S), ("M", S), ("L", S), ("ACC", 3 * BQ), ("PA", S),
    ("O", MT * S), ("D", T), ("R", 16), ("MOD", 5 * MT * 8),
):
    _OFF[_name] = _ROWS
    _ROWS += _n

_SEQ = (
    "q0 k0 q1 k1 q2 v0 A0+A1 A0 q3 q4 B0 A1 k2 v1 q5 B1 B0+A2 A2 q6 q7 v2 k3 "
    "B2 B1+A3 A3 v3 k4 k5 k6 k7 B3 B2+A4 A4 v4 v5 v6 v7 B4 B3+A5 A5 o0 o1 "
    "B5 B4+A6 A6 o2 o3 B6 B5+A7 A7 o4 o5 B6+B7 B7 o6 o7"
)
_SEQ_FIRST = (
    "A0+A1 A0 A1 A2+A3 A2 A3 q4 q5 q6 q7 B0+B1 B0 B1 A4+A5 A4 B2+B3 B2 B3 o0 o1 A5 A6+A7 A6 "
    "B4+B5 B4 B5 o2 o3 A7 o4 o5 B6+B7 B6 B7 o6 o7"
)
_SEQ_LAST = (
    "q0 q1 k0 k1 v0 A0+A1 A0 A1 v1 q2 k2 B0+B1 B0 B1 k3 q3 o0 o1 A2+A3 A2 v2 k4 q4 v3 "
    "B2+A4 B2 A3 q5 k5 o2 B3+A5 B3 A4 v4 q6 k6 o3 B4+A6 B4 A5 v5 q7 k7 o4 "
    "B5+A7 B5 A6 v6 o5 v7 A7 B6 B6+B7 B7 o6 o7"
)
_RES_LAG, _CTX_LAG, _MAX_LAG, _SUM_LAG = 200, 240, 128, 32
import os
_FIN_STEP, _FIN_LAG = eval(os.environ.get('FS','(96, 192)')), int(os.environ.get('FL',176))


def _slots(seq):
    lanes = []
    for word in seq.split():
        if "+" in word:
            lanes.append(tuple(
                (p[0], int(p[1:]), 2 * int(p[1:]) + 1, T) for p in word.split("+")))
        else:
            k, (i, *part) = word[0], map(int, word[1:].split(":"))
            n = {"q": MT, "k": CT, "v": CT, "o": MT, "A": 2 * i + 1, "B": 2 * i + 1}[k]
            lanes += [((k, i, j, 0),) for j in range(*(part or [n]))]
    assert len(lanes) % 4 == 0
    return [lanes[s:s + 4] for s in range(0, len(lanes), 4)]


def _nt(a, b):
    return lax.dot_general(a, b, (((1,), (1,)), ((), ())), preferred_element_type=F32)


def _nn(a, b):
    return jnp.dot(a, b, preferred_element_type=F32)


def _rnd(x):
    if x.shape == (16, T):
        y = _rnd(jnp.concatenate([x[:8], x[8:]], axis=1))
        return jnp.concatenate([y[:, :T], y[:, T:]], axis=0)
    return x.astype(BF).astype(F32)


def _pack(x):
    return pltpu.bitcast(x.astype(BF), F32)


def _select_head(src, slot, r, parity):
    even = pltpu.bitcast(src[slot, r // 2:r // 2 + 8, 0], U32).reshape(8, T)
    odd = pltpu.bitcast(src[slot, r // 2:r // 2 + 8, 1], U32).reshape(8, T)
    down = jnp.asarray(16 * parity, U32)
    word = ((even >> down) & 0xFFFF) | ((odd >> down) << 16)
    return pltpu.bitcast(word, F32)


def _head(seq, w, zero, wo, *, assign=False, next_weights=None, finalize=None):
    def load(r, n):
        return w[r:r + n, :]

    def ordered(r, n):
        head = w[pl.ds(zero + r, 8), :]
        return head if n == 8 else jnp.concatenate([head, load(r + 8, n - 8)], axis=0)

    def store(r, v):
        w[r:r + v.shape[0], :] = v

    def s_row(i, j, t, half):
        if half:
            return _OFF["SD"] + i * T + t - T
        return _OFF["S"] + (i * i + j) * BQ + t

    events = []

    def at(time, rank, fn):
        events.append((time, rank, len(events), fn))

    slots = _slots(seq)
    left = {}
    for slot in slots:
        for lane in slot:
            for k, i, _, t0 in lane:
                for t in range(t0, BQ, CH):
                    left[k, i, t] = left.get((k, i, t), 0) + 1
    has_sum, has_acc, last_use, complete = set(), set(), {}, {}
    pending = {}

    def expect(*tag):
        pending[tag] = pending.get(tag, 0) + 1
        return pending[tag]

    def settled(*tag):
        assert not pending.get(tag), tag

    for s, slot in enumerate(slots):
        base = BQ * s
        jobs = ([(lane[0], -T) for lane in slot if len(lane) == 2]
                + [(lane[0], 0) for lane in slot if len(lane) == 1]
                + [(lane[1], 0) for lane in slot if len(lane) == 2])
        lhs, res, groups = {}, {}, {}
        for job, shift in jobs:
            groups.setdefault((job[0], job[1], shift), []).append(job)
            last_use[job[0]] = base + BQ

        for (k, i, shift), group in groups.items():
            for t in range(0, BQ, CH):
                live = [job for job in group if t >= job[3]]
                if not live:
                    continue

                def fetch(k=k, i=i, t=t, live=live, lhs=lhs, first=(i, t) not in has_sum):
                    r = i * BQ + t
                    if k in "qkv":
                        src = _OFF["H" if k == "q" else "C"] + r // 2
                        for job in live:
                            get = ordered if job == live[0] else load
                            lhs[job, t] = get(src + job[2] * S // 2, CH // 2)
                    elif k in "Ao":
                        settled("q" if k == "A" else "B", i, t)
                        v = ordered(_OFF["Q" if k == "A" else "X"] + r // 2, CH // 2)
                        for job in live:
                            lhs[job, t] = v
                            if k == "A" and job[2] == 2 * i + t // T:
                                lhs["d", job, t] = ordered(_OFF["D"] + t % T, 8)
                    else:
                        settled("A", i, t)
                        settled("m", i, t)
                        settled("l", i, t)
                        expect("l", i, t)
                        m = ordered(_OFF["M"] + r, CH)
                        l = None if first else load(_OFF["L"] + r, CH)
                        for job in live:
                            p = jnp.exp2(load(s_row(i, job[2], t, job[3]), CH) - m)
                            l = p if l is None else l + p
                            lhs[job, t] = p
                        lhs["l", i, t] = l

                at(base + shift + t, 1, fetch)
                if k == "B":
                    has_sum.add((i, t))

                    def keep_sum(i=i, t=t, lhs=lhs):
                        pending["l", i, t] -= 1
                        store(_OFF["L"] + i * BQ + t, lhs["l", i, t])

                    at(base + shift + t + CH - 16 + _SUM_LAG, 0, keep_sum)

        for job, shift in jobs:
            def matmul(job=job, lhs=lhs, res=res):
                k, _, j, t0 = job
                a = jnp.concatenate([lhs[job, t] for t in range(t0, BQ, CH)], axis=0)
                a = a.astype(BF) if k == "B" else pltpu.bitcast(a, BF)
                if k == "o":
                    res[job] = _nn(a, wo[:, j * T:(j + 1) * T])
                    return
                region = {"A": "K", "B": "V"}.get(k, "W" + k)
                if k in "AB":
                    settled(region.lower(), j // 2, (j % 2) * T + T - CH)
                b = pltpu.bitcast(load(_OFF[region] + j * T // 2, T // 2), BF)
                res[job] = _nt(a, b) if k == "A" else _nn(a, b)

            at(base + shift + BQ - CH, 2, matmul)

        for (k, i, shift), group in groups.items():
            for t in range(0, BQ, CH):
                live = [job for job in group if t >= job[3]]
                if not live:
                    continue
                first = (k, i, t) not in has_acc
                has_acc.add((k, i, t))
                left[k, i, t] -= len(live)
                last = left[k, i, t] == 0

                def finish(k=k, i=i, t=t, live=live, lhs=lhs, res=res, first=first, last=last):
                    r = i * BQ + t
                    pending[k, i, t] -= 1
                    assert k == "o" or last == (pending[k, i, t] == 0), (k, i, t)
                    parts = [res[job][t - job[3]:t - job[3] + CH] for job in live]
                    if k == "o":
                        for job, v in zip(live, parts):
                            a = _OFF["O"] + job[2] * S + r
                            store(a, v if assign else load(a, CH) + v)
                    elif k == "A":
                        mx = None if first else load(_OFF["MX"] + r, CH)
                        for job, v in zip(live, parts):
                            if job[2] == 2 * i + t // T:
                                d = lhs["d", job, t]
                                v = jnp.concatenate(
                                    [jnp.where(d <= u, v[u:u + 8], MASKED)
                                     for u in range(0, CH, 8)], axis=0)
                            store(s_row(i, job[2], t, job[3]), v)
                            mx = v if mx is None else jnp.maximum(mx, v)
                        if last:
                            res["m", i, t] = jnp.broadcast_to(
                                jnp.max(mx, axis=1, keepdims=True), (CH, T))
                        else:
                            store(_OFF["MX"] + r, mx)
                    else:
                        a = _OFF["PA"] + r if k == "B" else _OFF["ACC"] + "qkv".index(k) * BQ + t
                        acc = None if first else load(a, CH)
                        for v in parts:
                            acc = v if acc is None else acc + v
                        if not last:
                            store(a, acc)
                        elif k == "B":
                            settled("l", i, t)
                            l = jnp.sum(load(_OFF["L"] + r, CH), axis=1, keepdims=True)
                            store(_OFF["X"] + r // 2, _pack(acc * (1.0 / l)))
                        elif k == "q":
                            store(_OFF["Q"] + r // 2, _pack(acc * QSCALE))
                        else:
                            store(_OFF[k.upper()] + r // 2, _pack(acc))

                ready = base + shift + t + CH - 16 + (_CTX_LAG if k == "B" and last else _RES_LAG)
                when = max(base + shift + BQ, ready)
                expect(k, i, t)
                at(when, 0, finish)
                if k == "o" and last:
                    complete[i * BQ + t] = when
                if k == "A" and last:
                    def keep_max(i=i, t=t, res=res):
                        pending["m", i, t] -= 1
                        store(_OFF["M"] + i * BQ + t, res["m", i, t])

                    expect("m", i, t)
                    at(max(when, ready + _MAX_LAG), 0, keep_max)

    busy = [any(job[0] == "B" for s2 in (max(s - 1, 0), s) for lane in slots[s2] for job in lane)
            for s in range(len(slots))]
    if next_weights:
        todo = [(k, r) for k, n in (("q", M), ("k", C), ("v", C)) for r in range(0, n, 16)]
        calm = [s for s in range(last_use.get("q", 0) // BQ, len(slots) - 2) if not busy[s]]
        for n, (k, r) in enumerate(todo):
            step = BQ * len(calm) * n // len(todo)
            time = BQ * calm[step // BQ] + step % BQ
            assert time >= last_use.get(k, 0)
            at(time, 0, lambda k=k, r=r: next_weights(k, r))
    if finalize:
        time = 0
        for r in range(0, S, 16):
            heavy = time // BQ < len(slots) and busy[time // BQ]
            time = max(time + _FIN_STEP[heavy], complete[r // CH * CH])
            for delay, fn in finalize(r):
                at(time + delay, 0, fn)

    for event in sorted(events, key=lambda e: e[:3]):
        event[3]()


def _row_sum(tiles):
    total = tiles[0]
    for tile in tiles[1:]:
        total = total + tile
    return jnp.broadcast_to(jnp.sum(total, axis=1, keepdims=True), total.shape)


def _mean(x1):
    return _row_sum(x1) * (1.0 / M)


def _inv_std(x1, mean):
    var = _row_sum([jnp.square(t - mean) for t in x1]) * (1.0 / M)
    return 1.0 / _rnd(jnp.sqrt(_rnd(_rnd(var) + EPS)))


def _norm2(x1, mean, inv_std, scale, shift):
    mean = _rnd(mean)
    return [_rnd((t - mean) * inv_std * a + b) for t, a, b in zip(x1, scale, shift)]


def _kernel(x_hbm, ckv_hbm, wq_hbm, wk_hbm, wv_hbm, wo_hbm, wr_hbm, wg_hbm, wu_hbm,
            wd_hbm, c_hbm, wmod_hbm, out_hbm,
            w, x_v, ckv_v, wq_v, wk_v, wv_v, wo_v, wr_v, wg_v, wu_v, wd_v, c_v,
            wmod_a, wmod_b, out_v, sem_in, sem_x, sem_c, sem_w, sem_o, sem_out, sem_fix):
    pairs = {"q": wq_v, "k": wk_v, "v": wv_v}
    nb = S // BQ

    def rows(i, n=1):
        return pl.ds(i * BQ, n * BQ)

    def pair_copies(p):
        heads = pl.ds(2 * p, 2)
        return [pltpu.make_async_copy(src.at[:, :, heads, :], dst.at[p % 2],
                                      sem_w.at[3 * (p % 2) + n])
                for n, (src, dst) in enumerate(((wq_hbm, wq_v), (wk_hbm, wk_v), (wv_hbm, wv_v)))]

    def wo_copy(h):
        return pltpu.make_async_copy(wo_hbm.at[h], wo_v.at[h % 2], sem_o.at[h % 2])

    def weights_of(h):
        def select(k, r):
            a = _OFF["W" + k] + r // 2
            w[a:a + 8, :] = _select_head(pairs[k], (h // 2) % 2, r, h % 2)
        return select

    def weight(k, n):
        return pltpu.bitcast(w[_OFF["W" + k]:_OFF["W" + k] + n // 2, :], BF)

    def put(region, i, v):
        for j in range(v.shape[1] // T):
            a = _OFF[region] + (j * S + i * BQ) // 2
            w[a:a + v.shape[0], :] = v[:, j * T:(j + 1) * T]

    def silu_c():
        c = jnp.broadcast_to(c_v[...].astype(F32), (16, M))
        return (c * jax.nn.sigmoid(c)).astype(BF)

    wq_copy, wk_copy, wv_copy = pair_copies(0)
    c_copy = pltpu.make_async_copy(c_hbm, c_v, sem_in.at[0])
    mod_a_copy = pltpu.make_async_copy(wmod_hbm.at[:, pl.ds(0, 2 * M)], wmod_a, sem_in.at[1])
    x_copies = [pltpu.make_async_copy(x_hbm.at[rows(i)], x_v.at[rows(i)], sem_x.at[i])
                for i in range(nb)]
    ckv_copies = [pltpu.make_async_copy(ckv_hbm.at[rows(i, 2)], ckv_v.at[rows(i, 2)], sem_c.at[i])
                  for i in range(0, nb, 2)]
    late_copies = [
        pltpu.make_async_copy(src, dst, sem_in.at[2 + n]) for n, (src, dst) in enumerate((
            (wmod_hbm.at[:, pl.ds(2 * M, 4 * M)], wmod_b), (wr_hbm, wr_v),
            (wg_hbm, wg_v), (wu_hbm, wu_v), (wd_hbm, wd_v)))]
    batches = iter([
        [wk_copy, wv_copy], [ckv_copies[0], wq_copy], ckv_copies[1:2], ckv_copies[2:],
        [c_copy, mod_a_copy], [], x_copies[:2], x_copies[2:4], x_copies[4:6],
        x_copies[6:] + [wo_copy(0)], pair_copies(1) + [wo_copy(1)]])

    def start_more():
        for copy in next(batches, []):
            copy.start()

    start_more()
    start_more()

    w[_OFF["D"]:_OFF["D"] + T, :] = (
        lax.broadcasted_iota(I32, (T, T), 1) - lax.broadcasted_iota(I32, (T, T), 0)).astype(F32)
    w[_OFF["R"]:_OFF["R"] + 16, :] = jnp.zeros((16, T), F32)
    for k, copy in (("k", wk_copy), ("v", wv_copy)):
        copy.wait()
        start_more()
        for r in range(0, C, 16):
            weights_of(0)(k, r)
    for i, copy in zip(range(0, nb, 2), ckv_copies):
        copy.wait()
        start_more()
        ckv = ckv_v[rows(i, 2), :]
        put("C", i, pltpu.bitcast(ckv, F32))
        put("K", i, _pack(_nn(ckv, weight("k", C))))
        put("V", i, _pack(_nn(ckv, weight("v", C))))
    origin = pl.multiple_of(pltpu.bitcast(w[_OFF["R"]:_OFF["R"] + 8, :], I32)[0, 0], 16)
    wq_copy.wait()
    for r in range(0, M, 16):
        weights_of(0)("q", r)
    c_copy.wait()
    mod_a_copy.wait()
    start_more()
    mod = _rnd(_nn(silu_c(), wmod_a[...])[:1])
    shift_a, scale_a = mod[:, :M], _rnd(1.0 + mod[:, M:])

    def project_q(i):
        h = jnp.concatenate(
            [w[pl.ds(_OFF["H"] + (j * S + i * BQ) // 2, BQ // 2), :] for j in range(MT)], axis=1)
        put("Q", i, _pack(_nn(pltpu.bitcast(h, BF), weight("q", M)) * QSCALE))

    for i in range(nb):
        x_copies[i].wait()
        if i % 2 == 0:
            start_more()
        if 0 < i <= nb // 2:
            project_q(i - 1)
        x = x_v[rows(i), :].astype(F32)
        xc = x - jnp.mean(x, axis=1, keepdims=True)
        var = jnp.mean(xc * xc, axis=1, keepdims=True)
        put("H", i, _pack(xc * lax.rsqrt(var + EPS) * scale_a + shift_a))
    wo_copy(0).wait()

    _head(_SEQ_FIRST, w, origin, wo_v.at[0], assign=True, next_weights=weights_of(1))

    def head_step(h, carry):
        wo_copy(h).wait()

        @pl.when(h % 2 == 1)
        def _():
            for copy in pair_copies(h // 2 + 1):
                copy.wait()

        wo_copy(h + 1).start()
        for n, copy in enumerate(late_copies):
            pl.when(h == 2 * n + 1)(copy.start)

        @pl.when(jnp.logical_and(h % 2 == 0, h + 2 < H))
        def _():
            for copy in pair_copies(h // 2 + 1):
                copy.start()

        _head(_SEQ, w, origin, wo_v.at[h % 2], next_weights=weights_of(h + 1))
        return carry

    lax.fori_loop(1, H - 1, head_step, 0)

    for copy in [wo_copy(H - 1)] + late_copies:
        copy.wait()
    mod = _rnd(_nn(silu_c(), wmod_b[...])[:8])
    w_r = jnp.broadcast_to(wr_v[...].astype(F32).reshape(1, M), (8, M))
    for n, v in enumerate((mod[:, :M], mod[:, M:2 * M], _rnd(1.0 + mod[:, 2 * M:3 * M]),
                           mod[:, 3 * M:], w_r)):
        for j in range(MT):
            a = _OFF["MOD"] + (n * MT + j) * 8
            w[a:a + 8, :] = v[:, j * T:(j + 1) * T]

    def vector(name, n):
        a = _OFF["MOD"] + ("gate_a", "shift_b", "scale_b", "gate_b", "w_r").index(name) * MT * 8
        return [jnp.concatenate([w[a + 8 * j:a + 8 * j + 8, :]] * (n // 8), axis=0)
                for j in range(MT)]

    out_copies = [pltpu.make_async_copy(out_v.at[rows(i)], out_hbm.at[rows(i)], sem_out.at[i])
                  for i in range(nb)]

    def finalize(r):
        kept = {}
        x1_at = [pl.ds(_OFF["O"] + j * S + r, 16) for j in range(MT)]
        mean_at, inv_at = pl.ds(_OFF["MX"] + r, 16), pl.ds(_OFF["M"] + r, 16)

        def residual():
            x = x_v[r:r + 16, :].astype(F32)
            x1 = [_rnd(x[:, j * T:(j + 1) * T] + g * w[x1_at[j], :])
                  for j, g in enumerate(vector("gate_a", 16))]
            for j in range(MT):
                w[x1_at[j], :] = x1[j]
            kept["mean"] = _mean(x1)

        def keep_mean():
            w[mean_at, :] = kept["mean"]

        def keep_inv_std():
            w[inv_at, :] = _inv_std([w[a, :] for a in x1_at], w[mean_at, :])

        def output():
            x1 = [w[a, :] for a in x1_at]
            h2 = _norm2(x1, w[mean_at, :], w[inv_at, :],
                        vector("scale_b", 16), vector("shift_b", 16))
            out = [t + g * h for t, g, h in zip(x1, vector("gate_b", 16), h2)]
            out_v[r:r + 16, :] = jnp.concatenate(out, axis=1).astype(BF)
            score = _row_sum([h * v for h, v in zip(h2, vector("w_r", 16))])
            at = pl.ds(_OFF["R"] + r // (8 * T) * 8, 8)
            lane = lax.broadcasted_iota(I32, (8, T), 1)
            a = r // 8 % T
            w[at, :] = jnp.where(lane == a, score[:8], jnp.where(lane == a + 1, score[8:], w[at, :]))
            if (r + 16) % BQ == 0:
                out_copies[r // BQ].start()

        return [(32, residual), (32 + _FIN_LAG, keep_mean), (32 + 2 * _FIN_LAG + 64, keep_inv_std),
                (32 + 3 * _FIN_LAG + 128, output)]

    _head(_SEQ_LAST, w, origin, wo_v.at[(H - 1) % 2], finalize=finalize)

    score = _rnd(w[_OFF["R"]:_OFF["R"] + 16, :])
    bits = pltpu.bitcast(jnp.where(score == 0.0, 0.0, score), I32) >> 16
    rank = jnp.where(bits < 0, -1 - bits, bits + 0x8000)
    rank = jnp.where(score != score, 0, rank)
    sub = lax.broadcasted_iota(I32, (16, T), 0)
    row = (sub >> 3) * (8 * T) + 8 * lax.broadcasted_iota(I32, (16, T), 1) + (sub & 7)
    key = pltpu.bitcast((rank << 11) | (S - 1 - row) | (1 << 29), F32)
    picked = []
    for _ in range(TOPK):
        top = jnp.max(jnp.max(key, axis=0, keepdims=True), axis=1, keepdims=True)
        key = jnp.where(key == top, 0.0, key)
        top = pltpu.bitcast(jnp.broadcast_to(top, (8, T)), I32)
        picked.append(S - 1 - (top[0, 0] & (S - 1)))

    def gather(at):
        return jnp.concatenate([w[pl.ds(at + r, 1), :] for r in picked], axis=0)

    x1 = [gather(_OFF["O"] + j * S) for j in range(MT)]
    h2 = _norm2(x1, gather(_OFF["MX"]), gather(_OFF["M"]),
                vector("scale_b", 8), vector("shift_b", 8))
    r_sel = _rnd(_row_sum([h * v for h, v in zip(h2, vector("w_r", 8))]))[:, :1]
    x1, h2 = jnp.concatenate(x1, axis=1), jnp.concatenate(h2, axis=1)
    g = _rnd(_nt(h2.astype(BF), wg_v[...]))
    u = _rnd(_nt(h2.astype(BF), wu_v[...]))
    y = _nn((_rnd(g * jax.nn.sigmoid(g)) * u).astype(BF), wd_v[...])
    new = x1 + jnp.concatenate(vector("gate_b", 8), axis=1) * (h2 + y * jax.nn.sigmoid(r_sel))

    for copy in out_copies:
        copy.wait()
    groups = [pl.ds(pl.multiple_of((r >> 4) << 4, 16), 16) for r in picked]
    line = lax.broadcasted_iota(I32, (16, M), 0)
    for n, r in enumerate(picked):
        old = out_v[groups[n], :].astype(F32)
        out_v[groups[n], :] = jnp.where(line == (r & 15), new[n:n + 1], old).astype(BF)

    fixes = []
    for n, r in enumerate(picked):
        fresh = True
        for earlier in picked[:n]:
            fresh = jnp.logical_and(fresh, (earlier >> 4) != (r >> 4))
        fixes.append((fresh, pltpu.make_async_copy(
            out_v.at[groups[n]], out_hbm.at[groups[n]], sem_fix.at[n])))
    for fresh, copy in fixes:
        pl.when(fresh)(copy.start)
    for fresh, copy in fixes:
        pl.when(fresh)(copy.wait)


@jax.jit
def pallas_adaLN_cond__compressed_kv_cla__moe_arch_mod__prompt_kernel(
    A_x: jax.Array,
    A_c_kv: jax.Array,
    A_w_q: jax.Array,
    A_w_uk: jax.Array,
    A_w_uv: jax.Array,
    A_w_o: jax.Array,
    B_x: jax.Array,
    B_w_r: jax.Array,
    B_w_gate: jax.Array,
    B_w_up: jax.Array,
    B_w_down: jax.Array,
    c: jax.Array,
    w_mod: jax.Array,
):
    del B_x
    assert A_x.shape == (1, S, M) and A_c_kv.shape == (1, S, C)
    assert A_w_q.shape == (M, H, D) and B_w_gate.shape == (M, F)
    dma = pltpu.SemaphoreType.DMA
    out = pl.pallas_call(
        _kernel,
        in_specs=[pl.BlockSpec(memory_space=pl.ANY)] * 12,
        out_specs=pl.BlockSpec(memory_space=pl.ANY),
        out_shape=jax.ShapeDtypeStruct((S, M), BF),
        scratch_shapes=[
            pltpu.VMEM((_ROWS, T), F32),
            pltpu.VMEM((S, M), BF), pltpu.VMEM((S, C), BF),
            pltpu.VMEM((2, M // 2, 2, 2, D), BF), pltpu.VMEM((2, C // 2, 2, 2, D), BF),
            pltpu.VMEM((2, C // 2, 2, 2, D), BF), pltpu.VMEM((2, D, M), BF),
            pltpu.VMEM((M,), BF),
            pltpu.VMEM((F, M), BF), pltpu.VMEM((F, M), BF), pltpu.VMEM((F, M), BF),
            pltpu.VMEM((1, M), BF),
            pltpu.VMEM((M, 2 * M), BF), pltpu.VMEM((M, 4 * M), BF),
            pltpu.VMEM((S, M), BF),
            dma((7,)), dma((S // BQ,)), dma((S // BQ,)), dma((6,)), dma((2,)),
            dma((S // BQ,)), dma((TOPK,)),
        ],
        compiler_params=pltpu.CompilerParams(vmem_limit_bytes=100 * 2 ** 20),
        name="adaln_attn_moe",
    )(A_x[0], A_c_kv[0], A_w_q.reshape(M // 2, 2, H, D), A_w_uk.reshape(C // 2, 2, H, D),
      A_w_uv.reshape(C // 2, 2, H, D), A_w_o, B_w_r,
      B_w_gate.T, B_w_up.T, B_w_down, c, w_mod)
    return out[None]
```

```python
import jax
import jax.numpy as jnp
from jax import lax
import jax.experimental.pallas as pl
import jax.experimental.pallas.tpu as pltpu

BF = jnp.bfloat16
F32 = jnp.float32
I32 = jnp.int32
U32 = jnp.uint32

S = 2048
M = 640
C = 512
H = 32
D = 128
F = 1728
TOPK = 8
EPS = 1e-5
LOG2E = 1.4426950408889634
QSCALE = D ** -0.5 * LOG2E
MASKED = -1e9 * LOG2E

T = 128
BQ = 256
CH = 32
MT = M // T
CT = C // T

_OFF = {}
_ROWS = 0
for _name, _n in (
    ("H", MT * S // 2), ("C", CT * S // 2),
    ("Q", S // 2), ("K", S // 2), ("V", S // 2), ("X", S // 2),
    ("Wq", M // 2), ("Wk", C // 2), ("Wv", C // 2),
    ("S", (S // BQ) ** 2 * BQ), ("SD", S // 2),
    ("MX", S), ("M", S), ("L", S), ("ACC", 3 * BQ), ("PA", S),
    ("O", MT * S), ("D", T), ("R", 16), ("MOD", 5 * MT * 8),
):
    _OFF[_name] = _ROWS
    _ROWS += _n

_SEQ = (
    "q0 k0 q1 k1 q2 v0 A0+A1 A0 q3 q4 B0 A1 k2 v1 q5 B1 B0+A2 A2 q6 q7 v2 k3 "
    "B2 B1+A3 A3 v3 k4 k5 k6 k7 B3 B2+A4 A4 v4 v5 v6 v7 B4 B3+A5 A5 o0 o1 "
    "B5 B4+A6 A6 o2 o3 B6 B5+A7 A7 o4 o5 B6+B7 B7 o6 o7"
)
_SEQ_FIRST = (
    "A0+A1 A0 A1 A2+A3 A2 A3 B0+B1 B0 B1 A4+A5 A4 B2+B3 B2 B3 o0 o1 A5 A6+A7 A6 "
    "B4+B5 B4 B5 o2 o3 A7 o4 o5 B6+B7 B6 B7 o6 o7"
)
_SEQ_LAST = (
    "q0 q1 k0 k1 v0 A0+A1 A0 A1 v1 q2 k2 B0+B1 B0 B1 k3 q3 o0 o1 A2+A3 A2 v2 k4 q4 v3 "
    "B2+A4 B2 A3 q5 k5 o2 B3+A5 B3 A4 v4 q6 k6 o3 B4+A6 B4 A5 v5 q7 k7 o4 "
    "B5+A7 B5 A6 v6 o5 v7 A7 B6 B6+B7 B7 o6 o7"
)
_RES_LAG, _CTX_LAG, _MAX_LAG, _SUM_LAG = 224, 240, 144, 32
import os
_FIN_STEP, _FIN_LAG = eval(os.environ.get('FS','(80, 192)')), int(os.environ.get('FL',176))
_FIN_TILE = int(os.environ.get('FT',0))


def _slots(seq):
    lanes = []
    for word in seq.split():
        if "+" in word:
            lanes.append(tuple(
                (p[0], int(p[1:]), 2 * int(p[1:]) + 1, T) for p in word.split("+")))
        else:
            k, (i, *part) = word[0], map(int, word[1:].split(":"))
            n = {"q": MT, "k": CT, "v": CT, "o": MT, "A": 2 * i + 1, "B": 2 * i + 1}[k]
            lanes += [((k, i, j, 0),) for j in range(*(part or [n]))]
    assert len(lanes) % 4 == 0
    return [lanes[s:s + 4] for s in range(0, len(lanes), 4)]


def _nt(a, b):
    return lax.dot_general(a, b, (((1,), (1,)), ((), ())), preferred_element_type=F32)


def _nn(a, b):
    return jnp.dot(a, b, preferred_element_type=F32)


def _rnd(x):
    if x.shape == (16, T):
        y = _rnd(jnp.concatenate([x[:8], x[8:]], axis=1))
        return jnp.concatenate([y[:, :T], y[:, T:]], axis=0)
    return x.astype(BF).astype(F32)


def _pack(x):
    return pltpu.bitcast(x.astype(BF), F32)


def _select_head(src, slot, r, parity):
    even = pltpu.bitcast(src[slot, r // 2:r // 2 + 8, 0], U32).reshape(8, T)
    odd = pltpu.bitcast(src[slot, r // 2:r // 2 + 8, 1], U32).reshape(8, T)
    down = jnp.asarray(16 * parity, U32)
    word = ((even >> down) & 0xFFFF) | ((odd >> down) << 16)
    return pltpu.bitcast(word, F32)


def _head(seq, w, zero, wo, *, assign=False, next_weights=None, residual=None,
          finalize=None):
    def load(r, n):
        return w[r:r + n, :]

    def ordered(r, n):
        head = w[pl.ds(zero + r, 8), :]
        return head if n == 8 else jnp.concatenate([head, load(r + 8, n - 8)], axis=0)

    def store(r, v):
        w[r:r + v.shape[0], :] = v

    def s_row(i, j, t, half):
        if half:
            return _OFF["SD"] + i * T + t - T
        return _OFF["S"] + (i * i + j) * BQ + t

    events = []

    def at(time, rank, fn):
        events.append((time, rank, len(events), fn))

    slots = _slots(seq)
    left = {}
    for slot in slots:
        for lane in slot:
            for k, i, _, t0 in lane:
                for t in range(t0, BQ, CH):
                    left[k, i, t] = left.get((k, i, t), 0) + 1
    has_sum, has_acc, last_use, complete = set(), set(), {}, {}
    pending = {}

    def expect(*tag):
        pending[tag] = pending.get(tag, 0) + 1
        return pending[tag]

    def settled(*tag):
        assert not pending.get(tag), tag

    for s, slot in enumerate(slots):
        base = BQ * s
        jobs = ([(lane[0], -T) for lane in slot if len(lane) == 2]
                + [(lane[0], 0) for lane in slot if len(lane) == 1]
                + [(lane[1], 0) for lane in slot if len(lane) == 2])
        lhs, res, groups = {}, {}, {}
        for job, shift in jobs:
            groups.setdefault((job[0], job[1], shift), []).append(job)
            last_use[job[0]] = base + BQ

        for (k, i, shift), group in groups.items():
            for t in range(0, BQ, CH):
                live = [job for job in group if t >= job[3]]
                if not live:
                    continue

                def fetch(k=k, i=i, t=t, live=live, lhs=lhs, first=(i, t) not in has_sum):
                    r = i * BQ + t
                    if k in "qkv":
                        src = _OFF["H" if k == "q" else "C"] + r // 2
                        for job in live:
                            get = ordered if job == live[0] else load
                            lhs[job, t] = get(src + job[2] * S // 2, CH // 2)
                    elif k in "Ao":
                        settled("q" if k == "A" else "B", i, t)
                        v = ordered(_OFF["Q" if k == "A" else "X"] + r // 2, CH // 2)
                        for job in live:
                            lhs[job, t] = v
                            if k == "A" and job[2] == 2 * i + t // T:
                                lhs["d", job, t] = ordered(_OFF["D"] + t % T, 8)
                    else:
                        settled("A", i, t)
                        settled("m", i, t)
                        settled("l", i, t)
                        expect("l", i, t)
                        m = ordered(_OFF["M"] + r, CH)
                        l = None if first else load(_OFF["L"] + r, CH)
                        for job in live:
                            p = jnp.exp2(load(s_row(i, job[2], t, job[3]), CH) - m)
                            l = p if l is None else l + p
                            lhs[job, t] = p
                        lhs["l", i, t] = l

                at(base + shift + t, 1, fetch)
                if k == "B":
                    has_sum.add((i, t))

                    def keep_sum(i=i, t=t, lhs=lhs):
                        pending["l", i, t] -= 1
                        store(_OFF["L"] + i * BQ + t, lhs["l", i, t])

                    at(base + shift + t + CH - 16 + _SUM_LAG, 0, keep_sum)

        for job, shift in jobs:
            def matmul(job=job, lhs=lhs, res=res):
                k, _, j, t0 = job
                a = jnp.concatenate([lhs[job, t] for t in range(t0, BQ, CH)], axis=0)
                a = a.astype(BF) if k == "B" else pltpu.bitcast(a, BF)
                if k == "o":
                    res[job] = _nn(a, wo[:, j * T:(j + 1) * T])
                    return
                region = {"A": "K", "B": "V"}.get(k, "W" + k)
                if k in "AB":
                    settled(region.lower(), j // 2, (j % 2) * T + T - CH)
                b = pltpu.bitcast(load(_OFF[region] + j * T // 2, T // 2), BF)
                res[job] = _nt(a, b) if k == "A" else _nn(a, b)

            at(base + shift + BQ - CH, 2, matmul)

        for (k, i, shift), group in groups.items():
            for t in range(0, BQ, CH):
                live = [job for job in group if t >= job[3]]
                if not live:
                    continue
                first = (k, i, t) not in has_acc
                has_acc.add((k, i, t))
                left[k, i, t] -= len(live)
                last = left[k, i, t] == 0

                def finish(k=k, i=i, t=t, live=live, lhs=lhs, res=res, first=first, last=last):
                    r = i * BQ + t
                    pending[k, i, t] -= 1
                    assert k == "o" or last == (pending[k, i, t] == 0), (k, i, t)
                    parts = [res[job][t - job[3]:t - job[3] + CH] for job in live]
                    if k == "o":
                        for job, v in zip(live, parts):
                            a = _OFF["O"] + job[2] * S + r
                            v = v if assign else load(a, CH) + v
                            store(a, residual(job[2], r, v) if residual else v)
                    elif k == "A":
                        mx = None if first else load(_OFF["MX"] + r, CH)
                        for job, v in zip(live, parts):
                            if job[2] == 2 * i + t // T:
                                d = lhs["d", job, t]
                                v = jnp.concatenate(
                                    [jnp.where(d <= u, v[u:u + 8], MASKED)
                                     for u in range(0, CH, 8)], axis=0)
                            store(s_row(i, job[2], t, job[3]), v)
                            mx = v if mx is None else jnp.maximum(mx, v)
                        if last:
                            res["m", i, t] = jnp.broadcast_to(
                                jnp.max(mx, axis=1, keepdims=True), (CH, T))
                        else:
                            store(_OFF["MX"] + r, mx)
                    else:
                        a = _OFF["PA"] + r if k == "B" else _OFF["ACC"] + "qkv".index(k) * BQ + t
                        acc = None if first else load(a, CH)
                        for v in parts:
                            acc = v if acc is None else acc + v
                        if not last:
                            store(a, acc)
                        elif k == "B":
                            settled("l", i, t)
                            l = jnp.sum(load(_OFF["L"] + r, CH), axis=1, keepdims=True)
                            store(_OFF["X"] + r // 2, _pack(acc * (1.0 / l)))
                        elif k == "q":
                            store(_OFF["Q"] + r // 2, _pack(acc * QSCALE))
                        else:
                            store(_OFF[k.upper()] + r // 2, _pack(acc))

                ready = base + shift + t + CH - 16 + (_CTX_LAG if k == "B" and last else _RES_LAG)
                when = max(base + shift + BQ, ready)
                expect(k, i, t)
                at(when, 0, finish)
                if k == "o" and last:
                    complete[i * BQ + t] = when
                if k == "A" and last:
                    def keep_max(i=i, t=t, res=res):
                        pending["m", i, t] -= 1
                        store(_OFF["M"] + i * BQ + t, res["m", i, t])

                    expect("m", i, t)
                    at(max(when, ready + _MAX_LAG), 0, keep_max)

    busy = [any(job[0] == "B" for s2 in (max(s - 1, 0), s) for lane in slots[s2] for job in lane)
            for s in range(len(slots))]
    if next_weights:
        todo = [(k, r) for k, n in (("q", M), ("k", C), ("v", C)) for r in range(0, n, 16)]
        calm = [s for s in range(last_use.get("q", 0) // BQ, len(slots) - 2) if not busy[s]]
        for n, (k, r) in enumerate(todo):
            step = BQ * len(calm) * n // len(todo)
            time = BQ * calm[step // BQ] + step % BQ
            assert time >= last_use.get(k, 0)
            at(time, 0, lambda k=k, r=r: next_weights(k, r))
    if finalize:
        time = 0
        for r in range(0, S, 16):
            heavy = time // BQ < len(slots) and busy[time // BQ]
            time = max(time + _FIN_STEP[heavy], complete[r // CH * CH])
            for delay, fn in finalize(r):
                at(time + delay, 0, fn)

    for event in sorted(events, key=lambda e: e[:3]):
        event[3]()


def _row_sum(tiles):
    total = tiles[0]
    for tile in tiles[1:]:
        total = total + tile
    return jnp.broadcast_to(jnp.sum(total, axis=1, keepdims=True), total.shape)


def _mean(x1):
    return _row_sum(x1) * (1.0 / M)


def _inv_std(x1, mean):
    var = _row_sum([jnp.square(t - mean) for t in x1]) * (1.0 / M)
    return 1.0 / _rnd(jnp.sqrt(_rnd(_rnd(var) + EPS)))


def _norm2(x1, mean, inv_std, scale, shift):
    mean = _rnd(mean)
    return [_rnd((t - mean) * inv_std * a + b) for t, a, b in zip(x1, scale, shift)]


def _kernel(x_hbm, ckv_hbm, wq_hbm, wk_hbm, wv_hbm, wo_hbm, wr_hbm, wg_hbm, wu_hbm,
            wd_hbm, c_hbm, wmod_hbm, out_hbm,
            w, x_v, ckv_v, wq_v, wk_v, wv_v, wo_v, wr_v, wg_v, wu_v, wd_v, c_v,
            wmod_a, wmod_b, out_v, sem_in, sem_x, sem_c, sem_w, sem_o, sem_out, sem_fix):
    pairs = {"q": wq_v, "k": wk_v, "v": wv_v}
    nb = S // BQ

    def rows(i, n=1):
        return pl.ds(i * BQ, n * BQ)

    def pair_copies(p):
        heads = pl.ds(2 * p, 2)
        return [pltpu.make_async_copy(src.at[:, :, heads, :], dst.at[(p & 1)],
                                      sem_w.at[3 * ((p & 1)) + n])
                for n, (src, dst) in enumerate(((wq_hbm, wq_v), (wk_hbm, wk_v), (wv_hbm, wv_v)))]

    def wo_copy(h):
        return pltpu.make_async_copy(wo_hbm.at[h], wo_v.at[(h & 1)], sem_o.at[(h & 1)])

    def weights_of(h):
        def select(k, r):
            a = _OFF["W" + k] + r // 2
            w[a:a + 8, :] = _select_head(pairs[k], (h >> 1) & 1, r, (h & 1))
        return select

    def weight(k, n):
        return pltpu.bitcast(w[_OFF["W" + k]:_OFF["W" + k] + n // 2, :], BF)

    def put(region, i, v):
        for j in range(v.shape[1] // T):
            a = _OFF[region] + (j * S + i * BQ) // 2
            w[a:a + v.shape[0], :] = v[:, j * T:(j + 1) * T]

    def silu_c():
        c = jnp.broadcast_to(c_v[...].astype(F32), (16, M))
        return (c * jax.nn.sigmoid(c)).astype(BF)

    c_copy = pltpu.make_async_copy(c_hbm, c_v, sem_in.at[0])
    mod_a_copy = pltpu.make_async_copy(wmod_hbm.at[:, pl.ds(0, 2 * M)], wmod_a, sem_in.at[1])
    late_copies = [
        pltpu.make_async_copy(src, dst, sem_in.at[2 + n]) for n, (src, dst) in enumerate((
            (wmod_hbm.at[:, pl.ds(2 * M, 4 * M)], wmod_b), (wr_hbm, wr_v),
            (wg_hbm, wg_v), (wu_hbm, wu_v), (wd_hbm, wd_v)))]

    def block_copies(i):
        return [pltpu.make_async_copy(x_hbm.at[rows(i)], x_v.at[rows(i)], sem_x.at[i]),
                pltpu.make_async_copy(ckv_hbm.at[rows(i)], ckv_v.at[rows(i)], sem_c.at[i])]

    def start(copies):
        for copy in copies:
            copy.start()

    def wait(copies):
        for copy in copies:
            copy.wait()

    start(pair_copies(0) + [c_copy, mod_a_copy])
    w[_OFF["D"]:_OFF["D"] + T, :] = (
        lax.broadcasted_iota(I32, (T, T), 1) - lax.broadcasted_iota(I32, (T, T), 0)).astype(F32)
    w[_OFF["R"]:_OFF["R"] + 16, :] = jnp.zeros((16, T), F32)
    wait(pair_copies(0))
    start(block_copies(0))
    for k, n in (("q", M), ("k", C), ("v", C)):
        for r in range(0, n, 16):
            weights_of(0)(k, r)
    origin = pl.multiple_of(pltpu.bitcast(w[_OFF["R"]:_OFF["R"] + 8, :], I32)[0, 0], 16)
    wait([c_copy, mod_a_copy])
    start(block_copies(1))
    mod = _rnd(_nn(silu_c(), wmod_a[...])[:1])
    shift_a, scale_a = mod[:, :M], _rnd(1.0 + mod[:, M:])

    for i in range(nb):
        wait(block_copies(i))
        start(block_copies(i + 2) if i + 2 < nb else
              [wo_copy(i + 2 - nb)] + (pair_copies(1) if i == nb - 1 else []))
        ckv = pltpu.bitcast(ckv_v[rows(i), :], F32)
        put("C", i, ckv)
        put("K", i, _pack(_nn(pltpu.bitcast(ckv, BF), weight("k", C))))
        put("V", i, _pack(_nn(pltpu.bitcast(ckv, BF), weight("v", C))))
        x = x_v[rows(i), :].astype(F32)
        xc = x - jnp.mean(x, axis=1, keepdims=True)
        var = jnp.mean(xc * xc, axis=1, keepdims=True)
        h = _pack(xc * lax.rsqrt(var + EPS) * scale_a + shift_a)
        put("H", i, h)
        h, wq = pltpu.bitcast(h, BF), weight("q", M)
        q = _nn(h[:, :4 * T], wq[:4 * T])
        q += jnp.concatenate([_nn(h[t:t + BQ // 4, 4 * T:], wq[4 * T:])
                              for t in range(0, BQ, BQ // 4)], axis=0)
        put("Q", i, _pack(q * QSCALE))
    wo_copy(0).wait()

    _head(_SEQ_FIRST, w, origin, wo_v.at[0], assign=True, next_weights=weights_of(1))

    def head_step(h, carry):
        wo_copy(h).wait()

        @pl.when((h & 1) == 1)
        def _():
            for copy in pair_copies((h >> 1) + 1):
                copy.wait()

        wo_copy(h + 1).start()
        for n, copy in enumerate(late_copies):
            pl.when(h == 2 * n + 1)(copy.start)

        @pl.when(jnp.logical_and((h & 1) == 0, h + 2 < H))
        def _():
            for copy in pair_copies((h >> 1) + 1):
                copy.start()

        _head(_SEQ, w, origin, wo_v.at[(h & 1)], next_weights=weights_of(h + 1))
        return carry

    lax.fori_loop(1, H - 1, head_step, 0)

    for copy in [wo_copy(H - 1)] + late_copies:
        copy.wait()
    vectors = ("gate_a", "shift_b", "scale_b", "gate_b", "w_r")

    def set_vector(name, v):
        for j in range(MT):
            a = _OFF["MOD"] + (vectors.index(name) * MT + j) * 8
            w[a:a + 8, :] = v[:, j * T:(j + 1) * T]

    def vector(name, n, tiles=range(MT)):
        a = _OFF["MOD"] + vectors.index(name) * MT * 8
        return [jnp.concatenate([w[a + 8 * j:a + 8 * j + 8, :]] * (n // 8), axis=0)
                for j in tiles]

    mod = _rnd(_nn(silu_c(), wmod_b[...])[:8])
    set_vector("gate_a", mod[:, :M])
    set_vector("shift_b", mod[:, M:2 * M])
    set_vector("scale_b", _rnd(1.0 + mod[:, 2 * M:3 * M]))
    set_vector("gate_b", mod[:, 3 * M:])
    set_vector("w_r", jnp.broadcast_to(wr_v[...].astype(F32).reshape(1, M), (8, M)))
    out_copies = [pltpu.make_async_copy(out_v.at[rows(i)], out_hbm.at[rows(i)], sem_out.at[i])
                  for i in range(nb)]

    def residual(j, r, attn):
        gate, = vector("gate_a", 16, [j])
        x = x_v[r:r + CH, j * T:(j + 1) * T].astype(F32)
        return jnp.concatenate(
            [_rnd(x[t:t + 16] + gate * attn[t:t + 16]) for t in range(0, CH, 16)], axis=0)

    def finalize(r):
        x1_at = [pl.ds(_OFF["O"] + j * S + r, 16) for j in range(MT)]
        mean_at, inv_at = pl.ds(_OFF["MX"] + r, 16), pl.ds(_OFF["M"] + r, 16)

        def keep_mean():
            w[mean_at, :] = _mean([w[a, :] for a in x1_at])

        def keep_inv_std():
            w[inv_at, :] = _inv_std([w[a, :] for a in x1_at], w[mean_at, :])

        def output():
            x1 = [w[a, :] for a in x1_at]
            h2 = _norm2(x1, w[mean_at, :], w[inv_at, :],
                        vector("scale_b", 16), vector("shift_b", 16))
            out = [t + g * h for t, g, h in zip(x1, vector("gate_b", 16), h2)]
            out_v[r:r + 16, :] = jnp.concatenate(out, axis=1).astype(BF)
            score = _row_sum([h * v for h, v in zip(h2, vector("w_r", 16))])
            at = pl.ds(_OFF["R"] + r // (8 * T) * 8, 8)
            lane = lax.broadcasted_iota(I32, (8, T), 1)
            a = r // 8 % T
            w[at, :] = jnp.where(lane == a, score[:8],
                                 jnp.where(lane == a + 1, score[8:], w[at, :]))
            if (r + 16) % BQ == 0:
                out_copies[r // BQ].start()

        return [(_FIN_LAG, keep_mean), (2 * _FIN_LAG + 64, keep_inv_std),
                (3 * _FIN_LAG + 128 + _FIN_TILE, output)]

    _head(_SEQ_LAST, w, origin, wo_v.at[(H - 1) % 2], residual=residual, finalize=finalize)

    score = _rnd(w[_OFF["R"]:_OFF["R"] + 16, :])
    bits = pltpu.bitcast(jnp.where(score == 0.0, 0.0, score), I32) >> 16
    rank = jnp.where(bits < 0, -1 - bits, bits + 0x8000)
    rank = jnp.where(score != score, 0, rank)
    sub = lax.broadcasted_iota(I32, (16, T), 0)
    row = (sub >> 3) * (8 * T) + 8 * lax.broadcasted_iota(I32, (16, T), 1) + (sub & 7)
    key = pltpu.bitcast((rank << 11) | (S - 1 - row) | (1 << 29), F32)
    picked = []
    for _ in range(TOPK):
        top = jnp.max(jnp.max(key, axis=0, keepdims=True), axis=1, keepdims=True)
        key = jnp.where(key == top, 0.0, key)
        top = pltpu.bitcast(jnp.broadcast_to(top, (8, T)), I32)
        picked.append(S - 1 - (top[0, 0] & (S - 1)))

    wait(out_copies)

    def gather(at):
        return jnp.concatenate([w[pl.ds(at + r, 1), :] for r in picked], axis=0)

    x1 = [gather(_OFF["O"] + j * S) for j in range(MT)]
    h2 = _norm2(x1, gather(_OFF["MX"]), gather(_OFF["M"]),
                vector("scale_b", 8), vector("shift_b", 8))
    r_sel = _rnd(_row_sum([h * v for h, v in zip(h2, vector("w_r", 8))]))[:, :1]
    x1, h2 = jnp.concatenate(x1, axis=1), jnp.concatenate(h2, axis=1)
    g = _rnd(_nt(h2.astype(BF), wg_v[...]))
    u = _rnd(_nt(h2.astype(BF), wu_v[...]))
    y = _nn((_rnd(g * jax.nn.sigmoid(g)) * u).astype(BF), wd_v[...])
    new = x1 + jnp.concatenate(vector("gate_b", 8), axis=1) * (h2 + y * jax.nn.sigmoid(r_sel))

    groups = [pl.ds(pl.multiple_of((r >> 4) << 4, 16), 16) for r in picked]
    line = lax.broadcasted_iota(I32, (16, M), 0)
    for n, r in enumerate(picked):
        old = out_v[groups[n], :].astype(F32)
        out_v[groups[n], :] = jnp.where(line == (r & 15), new[n:n + 1], old).astype(BF)

    fixes = []
    for n, r in enumerate(picked):
        fresh = True
        for earlier in picked[:n]:
            fresh = jnp.logical_and(fresh, (earlier >> 4) != (r >> 4))
        fixes.append((fresh, pltpu.make_async_copy(
            out_v.at[groups[n]], out_hbm.at[groups[n]], sem_fix.at[n])))
    for fresh, copy in fixes:
        pl.when(fresh)(copy.start)
    for fresh, copy in fixes:
        pl.when(fresh)(copy.wait)


@jax.jit
def pallas_adaLN_cond__compressed_kv_cla__moe_arch_mod__prompt_kernel(
    A_x: jax.Array,
    A_c_kv: jax.Array,
    A_w_q: jax.Array,
    A_w_uk: jax.Array,
    A_w_uv: jax.Array,
    A_w_o: jax.Array,
    B_x: jax.Array,
    B_w_r: jax.Array,
    B_w_gate: jax.Array,
    B_w_up: jax.Array,
    B_w_down: jax.Array,
    c: jax.Array,
    w_mod: jax.Array,
):
    del B_x
    assert A_x.shape == (1, S, M) and A_c_kv.shape == (1, S, C)
    assert A_w_q.shape == (M, H, D) and B_w_gate.shape == (M, F)
    dma = pltpu.SemaphoreType.DMA
    out = pl.pallas_call(
        _kernel,
        in_specs=[pl.BlockSpec(memory_space=pl.ANY)] * 12,
        out_specs=pl.BlockSpec(memory_space=pl.ANY),
        out_shape=jax.ShapeDtypeStruct((S, M), BF),
        scratch_shapes=[
            pltpu.VMEM((_ROWS, T), F32),
            pltpu.VMEM((S, M), BF), pltpu.VMEM((S, C), BF),
            pltpu.VMEM((2, M // 2, 2, 2, D), BF), pltpu.VMEM((2, C // 2, 2, 2, D), BF),
            pltpu.VMEM((2, C // 2, 2, 2, D), BF), pltpu.VMEM((2, D, M), BF),
            pltpu.VMEM((M,), BF),
            pltpu.VMEM((F, M), BF), pltpu.VMEM((F, M), BF), pltpu.VMEM((F, M), BF),
            pltpu.VMEM((1, M), BF),
            pltpu.VMEM((M, 2 * M), BF), pltpu.VMEM((M, 4 * M), BF),
            pltpu.VMEM((S, M), BF),
            dma((7,)), dma((S // BQ,)), dma((S // BQ,)), dma((6,)), dma((2,)),
            dma((S // BQ,)), dma((TOPK,)),
        ],
        compiler_params=pltpu.CompilerParams(vmem_limit_bytes=100 * 2 ** 20),
        name="adaln_attn_moe",
    )(A_x[0], A_c_kv[0], A_w_q.reshape(M // 2, 2, H, D), A_w_uk.reshape(C // 2, 2, H, D),
      A_w_uv.reshape(C // 2, 2, H, D), A_w_o, B_w_r,
      B_w_gate.T, B_w_up.T, B_w_down, c, w_mod)
    return out[None]
```

```python
import jax
import jax.numpy as jnp
from jax import lax
import jax.experimental.pallas as pl
import jax.experimental.pallas.tpu as pltpu

BF = jnp.bfloat16
F32 = jnp.float32
I32 = jnp.int32
U32 = jnp.uint32

S = 2048
M = 640
C = 512
H = 32
D = 128
F = 1728
TOPK = 8
EPS = 1e-5
LOG2E = 1.4426950408889634
QSCALE = D ** -0.5 * LOG2E
MASKED = -1e9 * LOG2E

T = 128
BQ = 256
CH = 64
MT = M // T
CT = C // T

_OFF = {}
_ROWS = 0
for _name, _n in (
    ("H", MT * S // 2), ("C", CT * S // 2),
    ("Q", S // 2), ("K", S // 2), ("V", S // 2), ("X", S // 2),
    ("Wq", M // 2), ("Wk", C // 2), ("Wv", C // 2),
    ("S", (S // BQ) ** 2 * BQ), ("SD", S // 2),
    ("MX", S), ("M", S), ("L", S), ("ACC", 3 * BQ), ("PA", S),
    ("O", MT * S), ("D", T), ("R", 16), ("PAD", 8), ("MOD", 5 * MT * 8),
):
    _OFF[_name] = _ROWS
    _ROWS += _n

_SEQ = (
    "q0 k0 q1 k1 q2 v0 A0+A1 A0 q3 q4 B0 A1 k2 v1 q5 B1 B0+A2 A2 q6 q7 v2 k3 "
    "B2 B1+A3 A3 v3 k4 k5 k6 k7 B3 B2+A4 A4 v4 v5 v6 v7 B4 B3+A5 A5 o0 o1 "
    "B5 B4+A6 A6 o2 o3 B6 B5+A7 A7 o4 o5 B6+B7 B7 o6 o7"
)
_SEQ_FIRST = (
    "A0+A1 A0 A1 A2+A3 A2 A3 B0+B1 B0 B1 A4+A5 A4 B2+B3 B2 B3 o0 o1 A5 A6+A7 A6 "
    "B4+B5 B4 B5 o2 o3 A7 o4 o5 B6+B7 B6 B7 o6 o7"
)
_SEQ_LAST = (
    "q0 q1 k0 k1 v0 A0+A1 A0 A1 v1 q2 k2 B0+B1 B0 B1 k3 q3 o0 o1 A2+A3 A2 v2 k4 q4 v3 "
    "B2+A4 B2 A3 q5 k5 o2 B3+A5 B3 A4 v4 q6 k6 o3 B4+A6 B4 A5 v5 q7 k7 o4 "
    "B5+A7 B5 A6 v6 o5 v7 A7 B6 B6+B7 B7 o6 o7"
)
_RES_LAG, _CTX_LAG, _MAX_LAG, _SUM_LAG = 208, 208, 192, 80
import os
_FIN_STEP, _FIN_LAG = eval(os.environ.get('FS','(80, 192)')), int(os.environ.get('FL',176))
FR = int(os.environ.get('FR',16))
_SEQ_LAST=os.environ.get('SL',_SEQ_LAST)
_FIN_TILE = int(os.environ.get('FT',0))


def _slots(seq):
    lanes = []
    for word in seq.split():
        if "+" in word:
            lanes.append(tuple(
                (p[0], int(p[1:]), 2 * int(p[1:]) + 1, T) for p in word.split("+")))
        else:
            k, (i, *part) = word[0], map(int, word[1:].split(":"))
            n = {"q": MT, "k": CT, "v": CT, "o": MT, "A": 2 * i + 1, "B": 2 * i + 1}[k]
            lanes += [((k, i, j, 0),) for j in range(*(part or [n]))]
    assert len(lanes) % 4 == 0
    return [lanes[s:s + 4] for s in range(0, len(lanes), 4)]


def _nt(a, b):
    return lax.dot_general(a, b, (((1,), (1,)), ((), ())), preferred_element_type=F32)


def _nn(a, b):
    return jnp.dot(a, b, preferred_element_type=F32)


def _rnd(x):
    if x.shape[1] == T and x.shape[0] % 16 == 0:
        half = x.shape[0] // 2
        y = _rnd(jnp.concatenate([x[:half], x[half:]], axis=1))
        return jnp.concatenate([y[:, :T], y[:, T:]], axis=0)
    return x.astype(BF).astype(F32)


def _pack(x):
    return pltpu.bitcast(x.astype(BF), F32)


def _select_head(src, slot, r, parity):
    even = pltpu.bitcast(src[slot, r // 2:r // 2 + 8, 0], U32).reshape(8, T)
    odd = pltpu.bitcast(src[slot, r // 2:r // 2 + 8, 1], U32).reshape(8, T)
    down = jnp.asarray(16 * parity, U32)
    word = ((even >> down) & 0xFFFF) | ((odd >> down) << 16)
    return pltpu.bitcast(word, F32)


def _head(seq, w, zero, wo, *, assign=False, next_weights=None, residual=None,
          finalize=None, extras=()):
    def load(r, n):
        return w[r:r + n, :]

    def ordered(r, n):
        head = w[pl.ds(zero + r, 8), :]
        return head if n == 8 else jnp.concatenate([head, load(r + 8, n - 8)], axis=0)

    def store(r, v):
        w[r:r + v.shape[0], :] = v

    def s_row(i, j, t, half):
        if half:
            return _OFF["SD"] + i * T + t - T
        return _OFF["S"] + (i * i + j) * BQ + t

    events = []

    def at(time, rank, fn):
        events.append((time, rank, len(events), fn))

    slots = _slots(seq)
    left = {}
    for slot in slots:
        for lane in slot:
            for k, i, _, t0 in lane:
                for t in range(t0, BQ, CH):
                    left[k, i, t] = left.get((k, i, t), 0) + 1
    has_sum, has_acc, last_use, complete = set(), set(), {}, {}
    pending = {}

    def expect(*tag):
        pending[tag] = pending.get(tag, 0) + 1
        return pending[tag]

    def settled(*tag):
        assert not pending.get(tag), tag

    for s, slot in enumerate(slots):
        base = BQ * s
        jobs = ([(lane[0], -T) for lane in slot if len(lane) == 2]
                + [(lane[0], 0) for lane in slot if len(lane) == 1]
                + [(lane[1], 0) for lane in slot if len(lane) == 2])
        lhs, res, groups = {}, {}, {}
        for job, shift in jobs:
            groups.setdefault((job[0], job[1], shift), []).append(job)
            last_use[job[0]] = base + BQ

        for (k, i, shift), group in groups.items():
            for t in range(0, BQ, CH):
                live = [job for job in group if t >= job[3]]
                if not live:
                    continue

                def fetch(k=k, i=i, t=t, live=live, lhs=lhs, first=(i, t) not in has_sum):
                    r = i * BQ + t
                    if k in "qkv":
                        src = _OFF["H" if k == "q" else "C"] + r // 2
                        for job in live:
                            get = ordered if job == live[0] else load
                            lhs[job, t] = get(src + job[2] * S // 2, CH // 2)
                    elif k in "Ao":
                        settled("q" if k == "A" else "B", i, t)
                        v = ordered(_OFF["Q" if k == "A" else "X"] + r // 2, CH // 2)
                        for job in live:
                            lhs[job, t] = v
                            if k == "A" and job[2] == 2 * i + t // T:
                                lhs["d", job, t] = ordered(_OFF["D"] + t % T, 8)
                    else:
                        settled("A", i, t)
                        settled("m", i, t)
                        settled("l", i, t)
                        expect("l", i, t)
                        m = ordered(_OFF["M"] + r, CH)
                        l = None if first else load(_OFF["L"] + r, CH)
                        for job in live:
                            p = jnp.exp2(load(s_row(i, job[2], t, job[3]), CH) - m)
                            l = p if l is None else l + p
                            lhs[job, t] = p
                        lhs["l", i, t] = l

                at(base + shift + t, 1, fetch)
                if k == "B":
                    has_sum.add((i, t))

                    def keep_sum(i=i, t=t, lhs=lhs):
                        pending["l", i, t] -= 1
                        store(_OFF["L"] + i * BQ + t, lhs["l", i, t])

                    at(base + shift + t + CH - 16 + _SUM_LAG, 0, keep_sum)

        for job, shift in jobs:
            def matmul(job=job, lhs=lhs, res=res):
                k, _, j, t0 = job
                a = jnp.concatenate([lhs[job, t] for t in range(t0, BQ, CH)], axis=0)
                a = a.astype(BF) if k == "B" else pltpu.bitcast(a, BF)
                if k == "o":
                    res[job] = _nn(a, wo[:, j * T:(j + 1) * T])
                    return
                region = {"A": "K", "B": "V"}.get(k, "W" + k)
                if k in "AB":
                    settled(region.lower(), j // 2, (j % 2) * T + T - CH)
                b = pltpu.bitcast(load(_OFF[region] + j * T // 2, T // 2), BF)
                res[job] = _nt(a, b) if k == "A" else _nn(a, b)

            at(base + shift + BQ - CH, 2, matmul)

        for (k, i, shift), group in groups.items():
            for t in range(0, BQ, CH):
                live = [job for job in group if t >= job[3]]
                if not live:
                    continue
                first = (k, i, t) not in has_acc
                has_acc.add((k, i, t))
                left[k, i, t] -= len(live)
                last = left[k, i, t] == 0

                def finish(k=k, i=i, t=t, live=live, lhs=lhs, res=res, first=first, last=last):
                    r = i * BQ + t
                    pending[k, i, t] -= 1
                    assert k == "o" or last == (pending[k, i, t] == 0), (k, i, t)
                    parts = [res[job][t - job[3]:t - job[3] + CH] for job in live]
                    if k == "o":
                        for job, v in zip(live, parts):
                            a = _OFF["O"] + job[2] * S + r
                            v = v if assign else load(a, CH) + v
                            store(a, residual(job[2], r, v) if residual else v)
                    elif k == "A":
                        mx = None if first else load(_OFF["MX"] + r, CH)
                        for job, v in zip(live, parts):
                            if job[2] == 2 * i + t // T:
                                d = lhs["d", job, t]
                                v = jnp.concatenate(
                                    [jnp.where(d <= u, v[u:u + 8], MASKED)
                                     for u in range(0, CH, 8)], axis=0)
                            store(s_row(i, job[2], t, job[3]), v)
                            mx = v if mx is None else jnp.maximum(mx, v)
                        if last:
                            res["m", i, t] = jnp.broadcast_to(
                                jnp.max(mx, axis=1, keepdims=True), (CH, T))
                        else:
                            store(_OFF["MX"] + r, mx)
                    else:
                        a = _OFF["PA"] + r if k == "B" else _OFF["ACC"] + "qkv".index(k) * BQ + t
                        acc = None if first else load(a, CH)
                        for v in parts:
                            acc = v if acc is None else acc + v
                        if not last:
                            store(a, acc)
                        elif k == "B":
                            settled("l", i, t)
                            l = jnp.sum(load(_OFF["L"] + r, CH), axis=1, keepdims=True)
                            store(_OFF["X"] + r // 2, _pack(acc * (1.0 / l)))
                        elif k == "q":
                            store(_OFF["Q"] + r // 2, _pack(acc * QSCALE))
                        else:
                            store(_OFF[k.upper()] + r // 2, _pack(acc))

                ready = base + shift + t + CH - 16 + (_CTX_LAG if k == "B" and last else _RES_LAG)
                when = max(base + shift + BQ, ready)
                expect(k, i, t)
                at(when, 0, finish)
                if k == "o" and last:
                    complete[i * BQ + t] = when
                if k == "A" and last:
                    def keep_max(i=i, t=t, res=res):
                        pending["m", i, t] -= 1
                        store(_OFF["M"] + i * BQ + t, res["m", i, t])

                    expect("m", i, t)
                    at(max(when, ready + _MAX_LAG), 0, keep_max)

    busy = [any(job[0] == "B" for s2 in (max(s - 1, 0), s) for lane in slots[s2] for job in lane)
            for s in range(len(slots))]
    if next_weights:
        todo = [(k, r) for k, n in (("q", M), ("k", C), ("v", C)) for r in range(0, n, 16)]
        calm = [s for s in range(last_use.get("q", 0) // BQ, len(slots) - 2) if not busy[s]]
        for n, (k, r) in enumerate(todo):
            step = BQ * len(calm) * n // len(todo)
            time = BQ * calm[step // BQ] + step % BQ
            assert time >= last_use.get(k, 0)
            at(time, 0, lambda k=k, r=r: next_weights(k, r))
    for time, fn in extras:
        at(time, 0, fn)
    if finalize:
        time = 0
        for r in range(0, S, FR):
            heavy = time // BQ < len(slots) and busy[time // BQ]
            time = max(time + _FIN_STEP[heavy], complete[r // CH * CH])
            for delay, fn in finalize(r):
                at(time + delay, 0, fn)

    for event in sorted(events, key=lambda e: e[:3]):
        event[3]()


def _row_sum(tiles):
    total = tiles[0]
    for tile in tiles[1:]:
        total = total + tile
    return jnp.broadcast_to(jnp.sum(total, axis=1, keepdims=True), total.shape)


def _mean(x1):
    return _row_sum(x1) * (1.0 / M)


def _inv_std(x1, mean):
    var = _row_sum([jnp.square(t - mean) for t in x1]) * (1.0 / M)
    return 1.0 / _rnd(jnp.sqrt(_rnd(_rnd(var) + EPS)))


def _norm2(x1, mean, inv_std, scale, shift):
    mean = _rnd(mean)
    return [_rnd((t - mean) * inv_std * a + b) for t, a, b in zip(x1, scale, shift)]


def _kernel(x_hbm, ckv_hbm, wq_hbm, wk_hbm, wv_hbm, wo_hbm, wr_hbm, wg_hbm, wu_hbm,
            wd_hbm, c_hbm, wmod_hbm, out_hbm,
            w, x_v, ckv_v, wq_v, wk_v, wv_v, wo_v, wr_v, wgu_v, wgu_t, wd_v, c_v,
            wmod_v, silu_v, mod_v, out_v, sem_in, sem_x, sem_c, sem_w, sem_o, sem_out, sem_fix):
    pairs = {"q": wq_v, "k": wk_v, "v": wv_v}
    nb = S // BQ

    def rows(i, n=1):
        return pl.ds(i * BQ, n * BQ)

    def pair_copies(p):
        heads = pl.ds(2 * p, 2)
        return [pltpu.make_async_copy(src.at[:, :, heads, :], dst.at[(p & 1)],
                                      sem_w.at[3 * ((p & 1)) + n])
                for n, (src, dst) in enumerate(((wq_hbm, wq_v), (wk_hbm, wk_v), (wv_hbm, wv_v)))]

    def wo_copy(h):
        return pltpu.make_async_copy(wo_hbm.at[h], wo_v.at[(h & 1)], sem_o.at[(h & 1)])

    def weights_of(h):
        def select(k, r):
            a = _OFF["W" + k] + r // 2
            w[a:a + 8, :] = _select_head(pairs[k], (h >> 1) & 1, r, (h & 1))
        return select

    def weight(k, n):
        return pltpu.bitcast(w[_OFF["W" + k]:_OFF["W" + k] + n // 2, :], BF)

    def put(region, i, v):
        for j in range(v.shape[1] // T):
            a = _OFF[region] + (j * S + i * BQ) // 2
            w[a:a + v.shape[0], :] = v[:, j * T:(j + 1) * T]

    c_copy = pltpu.make_async_copy(c_hbm, c_v, sem_in.at[0])
    early, late = pl.ds(0, 2 * M), pl.ds(2 * M, 4 * M)
    mod_a_copy, mod_b_copy, wg_copy, wu_copy, wd_copy, wr_copy = [
        pltpu.make_async_copy(src, dst, sem_in.at[1 + n]) for n, (src, dst) in enumerate((
            (wmod_hbm.at[:, early], wmod_v.at[:, early]),
            (wmod_hbm.at[:, late], wmod_v.at[:, late]),
            (wg_hbm, wgu_v.at[pl.ds(0, F)]), (wu_hbm, wgu_v.at[pl.ds(F, F)]),
            (wd_hbm, wd_v), (wr_hbm, wr_v)))]

    def block_copies(i):
        return [pltpu.make_async_copy(x_hbm.at[rows(i)], x_v.at[rows(i)], sem_x.at[i]),
                pltpu.make_async_copy(ckv_hbm.at[rows(i)], ckv_v.at[rows(i)], sem_c.at[i])]

    def start(copies):
        for copy in copies:
            copy.start()

    def wait(copies):
        for copy in copies:
            copy.wait()

    start(pair_copies(0) + [c_copy, mod_a_copy])
    w[_OFF["D"]:_OFF["D"] + T, :] = (
        lax.broadcasted_iota(I32, (T, T), 1) - lax.broadcasted_iota(I32, (T, T), 0)).astype(F32)
    w[_OFF["R"]:_OFF["R"] + 16, :] = jnp.zeros((16, T), F32)
    wait(pair_copies(0))
    start(block_copies(0))
    for k, n in (("q", M), ("k", C), ("v", C)):
        for r in range(0, n, 16):
            weights_of(0)(k, r)
    origin = pl.multiple_of(pltpu.bitcast(w[_OFF["R"]:_OFF["R"] + 8, :], I32)[0, 0], 16)
    c_copy.wait()
    c = jnp.broadcast_to(c_v[...].astype(F32), (16, M))
    silu_c = (c * jax.nn.sigmoid(c)).astype(BF)
    silu_v[...] = jnp.concatenate([silu_c.astype(F32)] * (T // 16), axis=0).T
    mod_a_copy.wait()
    start(block_copies(1))
    mod = _rnd(_nn(silu_c, wmod_v[:, early])[:1])
    shift_a, scale_a = mod[:, :M], _rnd(1.0 + mod[:, M:])

    for i in range(nb):
        wait(block_copies(i))
        start(block_copies(i + 2) if i + 2 < nb else
              [wo_copy(i + 2 - nb)] + (pair_copies(1) if i == nb - 1 else []))
        ckv = pltpu.bitcast(ckv_v[rows(i), :], F32)
        put("C", i, ckv)
        put("K", i, _pack(_nn(pltpu.bitcast(ckv, BF), weight("k", C))))
        put("V", i, _pack(_nn(pltpu.bitcast(ckv, BF), weight("v", C))))
        x = x_v[rows(i), :].astype(F32)
        xc = x - jnp.mean(x, axis=1, keepdims=True)
        var = jnp.mean(xc * xc, axis=1, keepdims=True)
        h = _pack(xc * lax.rsqrt(var + EPS) * scale_a + shift_a)
        put("H", i, h)
        h, wq = pltpu.bitcast(h, BF), weight("q", M)
        q = _nn(h[:, :4 * T], wq[:4 * T])
        q += jnp.concatenate([_nn(h[t:t + BQ // 4, 4 * T:], wq[4 * T:])
                              for t in range(0, BQ, BQ // 4)], axis=0)
        put("Q", i, _pack(q * QSCALE))
    wo_copy(0).wait()
    start([wg_copy, wu_copy])

    _head(_SEQ_FIRST, w, origin, wo_v.at[0], assign=True, next_weights=weights_of(1))

    wait([wg_copy, wu_copy])

    def head_step(h, carry):
        wo_copy(h).wait()
        pl.when(h == 2 * MT)(mod_b_copy.wait)

        @pl.when((h & 1) == 1)
        def _():
            for copy in pair_copies((h >> 1) + 1):
                copy.wait()

        wo_copy(h + 1).start()
        for n, copy in enumerate((mod_b_copy, wd_copy, wr_copy)):
            pl.when(h == 2 * n + 1)(copy.start)

        @pl.when(jnp.logical_and((h & 1) == 0, h + 2 < H))
        def _():
            for copy in pair_copies((h >> 1) + 1):
                copy.start()

        pad = pl.ds(_OFF["PAD"], 8)

        def modulation(k):
            lanes, ks = pl.ds(pl.multiple_of((h - 1) * T, T), T), pl.ds(k * T, T)
            part = jnp.sum(silu_v[ks, :] * wmod_v[ks, lanes].astype(F32), axis=0, keepdims=True)
            total = jnp.broadcast_to(part, (8, T)) + (w[pad, :] if k else 0.0)
            w[pad, :] = total
            if k == MT - 1:
                mod_v[h - 1] = total

        def transpose():
            n = jnp.minimum(h - 1, 2 * F // T - 1)
            wgu_t[n] = pltpu.bitcast(wgu_v[pl.ds(pl.multiple_of(n * T, T), T), :].T, F32)
            w[pad, :] = wgu_t[n + origin, :8, :]

        extras = [(T * (k + 1), lambda k=k: modulation(k)) for k in range(MT)]
        _head(_SEQ, w, origin, wo_v.at[(h & 1)], next_weights=weights_of(h + 1),
              extras=extras + [(5 * BQ, transpose)])
        return carry

    assert H - 2 == 6 * MT >= 2 * F // T
    lax.fori_loop(1, H - 1, head_step, 0)

    wait([wo_copy(H - 1), wd_copy, wr_copy])
    vectors = ("gate_a", "shift_b", "scale_b", "gate_b", "w_r")

    def set_vector(name, v):
        for j in range(MT):
            a = _OFF["MOD"] + (vectors.index(name) * MT + j) * 8
            w[a:a + 8, :] = v[:, j * T:(j + 1) * T]

    def vector(name, n, tiles=range(MT)):
        a = _OFF["MOD"] + vectors.index(name) * MT * 8
        return [jnp.concatenate([w[a + 8 * j:a + 8 * j + 8, :]] * (n // 8), axis=0)
                for j in tiles]

    mod = _rnd(jnp.concatenate([mod_v[j] for j in range(2 * MT, 6 * MT)], axis=1))
    set_vector("gate_a", mod[:, :M])
    set_vector("shift_b", mod[:, M:2 * M])
    set_vector("scale_b", _rnd(1.0 + mod[:, 2 * M:3 * M]))
    set_vector("gate_b", mod[:, 3 * M:])
    set_vector("w_r", jnp.broadcast_to(wr_v[...].astype(F32).reshape(1, M), (8, M)))
    out_copies = [pltpu.make_async_copy(out_v.at[rows(i)], out_hbm.at[rows(i)], sem_out.at[i])
                  for i in range(nb)]

    def residual(j, r, attn):
        gate, = vector("gate_a", CH, [j])
        return _rnd(x_v[r:r + CH, j * T:(j + 1) * T].astype(F32) + gate * attn)

    def finalize(r):
        x1_at = [pl.ds(_OFF["O"] + j * S + r, FR) for j in range(MT)]
        mean_at, inv_at = pl.ds(_OFF["MX"] + r, FR), pl.ds(_OFF["M"] + r, FR)

        def keep_mean():
            w[mean_at, :] = _mean([w[a, :] for a in x1_at])

        def keep_inv_std():
            w[inv_at, :] = _inv_std([w[a, :] for a in x1_at], w[mean_at, :])

        def output():
            x1 = [w[a, :] for a in x1_at]
            h2 = _norm2(x1, w[mean_at, :], w[inv_at, :],
                        vector("scale_b", FR), vector("shift_b", FR))
            out = [t + g * h for t, g, h in zip(x1, vector("gate_b", FR), h2)]
            out_v[r:r + FR, :] = jnp.concatenate(out, axis=1).astype(BF)
            score = _row_sum([h * v for h, v in zip(h2, vector("w_r", FR))])
            at = pl.ds(_OFF["R"] + r // (8 * T) * 8, 8)
            lane = lax.broadcasted_iota(I32, (8, T), 1)
            tile = w[at, :]
            for t in range(0, FR, 8):
                tile = jnp.where(lane == (r + t) // 8 % T, score[t:t + 8], tile)
            w[at, :] = tile
            if (r + FR) % BQ == 0:
                out_copies[r // BQ].start()

        return [(_FIN_LAG, keep_mean), (2 * _FIN_LAG + 64, keep_inv_std),
                (3 * _FIN_LAG + 128 + _FIN_TILE, output)]

    _head(_SEQ_LAST, w, origin, wo_v.at[(H - 1) % 2], residual=residual, finalize=finalize)

    score = _rnd(w[_OFF["R"]:_OFF["R"] + 16, :])
    bits = pltpu.bitcast(jnp.where(score == 0.0, 0.0, score), I32) >> 16
    rank = jnp.where(bits < 0, -1 - bits, bits + 0x8000)
    rank = jnp.where(score != score, 0, rank)
    sub = lax.broadcasted_iota(I32, (16, T), 0)
    row = (sub >> 3) * (8 * T) + 8 * lax.broadcasted_iota(I32, (16, T), 1) + (sub & 7)
    key = pltpu.bitcast((rank << 11) | (S - 1 - row) | (1 << 29), F32)
    picked = []
    for _ in range(TOPK):
        top = jnp.max(jnp.max(key, axis=0, keepdims=True), axis=1, keepdims=True)
        key = jnp.where(key == top, 0.0, key)
        top = pltpu.bitcast(jnp.broadcast_to(top, (8, T)), I32)
        picked.append(S - 1 - (top[0, 0] & (S - 1)))

    wait(out_copies)

    def gather(at):
        return jnp.concatenate([w[pl.ds(at + r, 1), :] for r in picked], axis=0)

    x1 = [gather(_OFF["O"] + j * S) for j in range(MT)]
    h2 = _norm2(x1, gather(_OFF["MX"]), gather(_OFF["M"]),
                vector("scale_b", 8), vector("shift_b", 8))
    r_sel = _rnd(_row_sum([h * v for h, v in zip(h2, vector("w_r", 8))]))[:, :1]
    x1, h2 = jnp.concatenate(x1, axis=1), jnp.concatenate(h2, axis=1)
    gu = _rnd(jnp.concatenate([_nn(h2.astype(BF), pltpu.bitcast(wgu_t[j], BF))
                               for j in range(2 * F // T)], axis=1))
    g, u = gu[:, :F], gu[:, F:]
    y = _nn((_rnd(g * jax.nn.sigmoid(g)) * u).astype(BF), wd_v[...])
    new = x1 + jnp.concatenate(vector("gate_b", 8), axis=1) * (h2 + y * jax.nn.sigmoid(r_sel))

    groups = [pl.ds(pl.multiple_of((r >> 4) << 4, 16), 16) for r in picked]
    line = lax.broadcasted_iota(I32, (16, M), 0)
    for n, r in enumerate(picked):
        old = out_v[groups[n], :].astype(F32)
        out_v[groups[n], :] = jnp.where(line == (r & 15), new[n:n + 1], old).astype(BF)

    fixes = []
    for n, r in enumerate(picked):
        fresh = True
        for earlier in picked[:n]:
            fresh = jnp.logical_and(fresh, (earlier >> 4) != (r >> 4))
        fixes.append((fresh, pltpu.make_async_copy(
            out_v.at[groups[n]], out_hbm.at[groups[n]], sem_fix.at[n])))
    for fresh, copy in fixes:
        pl.when(fresh)(copy.start)
    for fresh, copy in fixes:
        pl.when(fresh)(copy.wait)


@jax.jit
def pallas_adaLN_cond__compressed_kv_cla__moe_arch_mod__prompt_kernel(
    A_x: jax.Array,
    A_c_kv: jax.Array,
    A_w_q: jax.Array,
    A_w_uk: jax.Array,
    A_w_uv: jax.Array,
    A_w_o: jax.Array,
    B_x: jax.Array,
    B_w_r: jax.Array,
    B_w_gate: jax.Array,
    B_w_up: jax.Array,
    B_w_down: jax.Array,
    c: jax.Array,
    w_mod: jax.Array,
):
    del B_x
    assert A_x.shape == (1, S, M) and A_c_kv.shape == (1, S, C)
    assert A_w_q.shape == (M, H, D) and B_w_gate.shape == (M, F)
    dma = pltpu.SemaphoreType.DMA
    out = pl.pallas_call(
        _kernel,
        in_specs=[pl.BlockSpec(memory_space=pl.ANY)] * 12,
        out_specs=pl.BlockSpec(memory_space=pl.ANY),
        out_shape=jax.ShapeDtypeStruct((S, M), BF),
        scratch_shapes=[
            pltpu.VMEM((_ROWS, T), F32),
            pltpu.VMEM((S, M), BF), pltpu.VMEM((S, C), BF),
            pltpu.VMEM((2, M // 2, 2, 2, D), BF), pltpu.VMEM((2, C // 2, 2, 2, D), BF),
            pltpu.VMEM((2, C // 2, 2, 2, D), BF), pltpu.VMEM((2, D, M), BF),
            pltpu.VMEM((M,), BF),
            pltpu.VMEM((2 * F, M), BF), pltpu.VMEM((2 * F // T, M // 2, T), F32),
            pltpu.VMEM((F, M), BF),
            pltpu.VMEM((1, M), BF),
            pltpu.VMEM((M, 6 * M), BF), pltpu.VMEM((M, T), F32), pltpu.VMEM((6 * MT, 8, T), F32),
            pltpu.VMEM((S, M), BF),
            dma((7,)), dma((S // BQ,)), dma((S // BQ,)), dma((6,)), dma((2,)),
            dma((S // BQ,)), dma((TOPK,)),
        ],
        compiler_params=pltpu.CompilerParams(vmem_limit_bytes=100 * 2 ** 20),
        name="adaln_attn_moe",
    )(A_x[0], A_c_kv[0], A_w_q.reshape(M // 2, 2, H, D), A_w_uk.reshape(C // 2, 2, H, D),
      A_w_uv.reshape(C // 2, 2, H, D), A_w_o, B_w_r,
      B_w_gate.T, B_w_up.T, B_w_down, c, w_mod)
    return out[None]
```

```python
import jax
import jax.numpy as jnp
from jax import lax
import jax.experimental.pallas as pl
import jax.experimental.pallas.tpu as pltpu

BF = jnp.bfloat16
F32 = jnp.float32
I32 = jnp.int32
U32 = jnp.uint32

S = 2048
M = 640
C = 512
H = 32
D = 128
F = 1728
TOPK = 8
EPS = 1e-5
LOG2E = 1.4426950408889634
QSCALE = D ** -0.5 * LOG2E
MASKED = -1e9 * LOG2E

T = 128
BQ = 256
CH = 64
MT = M // T
CT = C // T

_OFF = {}
_ROWS = 0
for _name, _n in (
    ("H", MT * S // 2), ("C", CT * S // 2),
    ("Q", S // 2), ("K", S // 2), ("V", S // 2), ("X", S // 2),
    ("Wq", M // 2), ("Wk", C // 2), ("Wv", C // 2),
    ("S", (S // BQ) ** 2 * BQ), ("SD", S // 2),
    ("MX", S), ("M", S), ("L", S), ("ACC", 3 * BQ), ("PA", S),
    ("O", MT * S), ("D", T), ("R", 16), ("PAD", 8), ("MOD", 5 * MT * 8),
):
    _OFF[_name] = _ROWS
    _ROWS += _n

_SEQ = (
    "q0 k0 q1 k1 q2 v0 A0+A1 A0 q3 q4 B0 A1 k2 v1 q5 B1 A2 B0+A2 q6 q7 v2 k3 "
    "B2 A3 B1+A3 v3 k4 k5 k6 k7 B3 A4 B2+A4 v4 v5 v6 v7 B4 A5 B3+A5 o0 o1 "
    "B5 A6 B4+A6 o2 o3 B6 A7 B5+A7 o4 o5 B6+B7 B7 o6 o7"
)
_SEQ_FIRST = (
    "A0+A1 A0 A1 A2+A3 A2 A3 B0+B1 B0 B1 A4+A5 A4 B2+B3 B2 B3 o0 o1 A5 A6+A7 A6 "
    "B4+B5 B4 B5 o2 o3 A7 o4 o5 B6+B7 B6 B7 o6 o7"
)
_SEQ_LAST = (
    "q0 q1 k0 k1 v0 A0+A1 A0 A1 v1 q2 k2 B0+B1 B0 B1 k3 q3 o0 o1 A2+A3 A2 v2 k4 q4 v3 "
    "B2+A4 B2 A3 q5 k5 o2 B3+A5 B3 A4 v4 q6 k6 o3 B4+A6 B4 A5 v5 q7 k7 o4 "
    "B5+A7 B5 A6 v6 o5 v7 A7 B6 B6+B7 B7 o6 o7"
)
_RES_LAG, _CTX_LAG, _MAX_LAG, _SUM_LAG = 208, 208, 192, 80
import os
_FIN_STEP, _FIN_LAG = eval(os.environ.get('FS','(80, 192)')), int(os.environ.get('FL',176))
FR = int(os.environ.get('FR',16))
_SEQ_LAST=os.environ.get('SL',_SEQ_LAST)
_FIN_TILE = int(os.environ.get('FT',0))


def _slots(seq):
    lanes = []
    for word in seq.split():
        if "+" in word:
            lanes.append(tuple(
                (p[0], int(p[1:]), 2 * int(p[1:]) + 1, T) for p in word.split("+")))
        else:
            k, (i, *part) = word[0], map(int, word[1:].split(":"))
            n = {"q": MT, "k": CT, "v": CT, "o": MT, "A": 2 * i + 1, "B": 2 * i + 1}[k]
            lanes += [((k, i, j, 0),) for j in range(*(part or [n]))]
    assert len(lanes) % 4 == 0
    return [lanes[s:s + 4] for s in range(0, len(lanes), 4)]


def _nt(a, b):
    return lax.dot_general(a, b, (((1,), (1,)), ((), ())), preferred_element_type=F32)


def _nn(a, b):
    return jnp.dot(a, b, preferred_element_type=F32)


def _rnd(x):
    if x.shape[1] == T and x.shape[0] % 16 == 0:
        half = x.shape[0] // 2
        y = _rnd(jnp.concatenate([x[:half], x[half:]], axis=1))
        return jnp.concatenate([y[:, :T], y[:, T:]], axis=0)
    return x.astype(BF).astype(F32)


def _pack(x):
    return pltpu.bitcast(x.astype(BF), F32)


def _select_head(src, slot, r, parity):
    even = pltpu.bitcast(src[slot, r // 2:r // 2 + 8, 0], U32).reshape(8, T)
    odd = pltpu.bitcast(src[slot, r // 2:r // 2 + 8, 1], U32).reshape(8, T)
    down = jnp.asarray(16 * parity, U32)
    word = ((even >> down) & 0xFFFF) | ((odd >> down) << 16)
    return pltpu.bitcast(word, F32)


def _head(seq, w, zero, wo, *, assign=False, next_weights=None, residual=None,
          finalize=None, extras=()):
    def load(r, n):
        return w[r:r + n, :]

    def ordered(r, n):
        head = w[pl.ds(zero + r, 8), :]
        return head if n == 8 else jnp.concatenate([head, load(r + 8, n - 8)], axis=0)

    def store(r, v):
        w[r:r + v.shape[0], :] = v

    def s_row(i, j, t, half):
        if half:
            return _OFF["SD"] + i * T + t - T
        return _OFF["S"] + (i * i + j) * BQ + t

    events = []

    def at(time, rank, fn):
        events.append((time, rank, len(events), fn))

    slots = _slots(seq)
    left = {}
    for slot in slots:
        for lane in slot:
            for k, i, _, t0 in lane:
                for t in range(t0, BQ, CH):
                    left[k, i, t] = left.get((k, i, t), 0) + 1
    has_sum, has_acc, last_use, complete = set(), set(), {}, {}
    pending = {}

    def expect(*tag):
        pending[tag] = pending.get(tag, 0) + 1
        return pending[tag]

    def settled(*tag):
        assert not pending.get(tag), tag

    for s, slot in enumerate(slots):
        base = BQ * s
        jobs = ([(lane[0], -T) for lane in slot if len(lane) == 2]
                + [(lane[0], 0) for lane in slot if len(lane) == 1]
                + [(lane[1], 0) for lane in slot if len(lane) == 2])
        lhs, res, groups = {}, {}, {}
        for job, shift in jobs:
            groups.setdefault((job[0], job[1], shift), []).append(job)
            last_use[job[0]] = base + BQ

        for (k, i, shift), group in groups.items():
            for t in range(0, BQ, CH):
                live = [job for job in group if t >= job[3]]
                if not live:
                    continue

                def fetch(k=k, i=i, t=t, live=live, lhs=lhs, first=(i, t) not in has_sum):
                    r = i * BQ + t
                    if k in "qkv":
                        src = _OFF["H" if k == "q" else "C"] + r // 2
                        for job in live:
                            get = ordered if job == live[0] else load
                            lhs[job, t] = get(src + job[2] * S // 2, CH // 2)
                    elif k in "Ao":
                        settled("q" if k == "A" else "B", i, t)
                        v = ordered(_OFF["Q" if k == "A" else "X"] + r // 2, CH // 2)
                        for job in live:
                            lhs[job, t] = v
                            if k == "A" and job[2] == 2 * i + t // T:
                                lhs["d", job, t] = ordered(_OFF["D"] + t % T, 8)
                    else:
                        settled("A", i, t)
                        settled("m", i, t)
                        settled("l", i, t)
                        expect("l", i, t)
                        m = ordered(_OFF["M"] + r, CH)
                        l = None if first else load(_OFF["L"] + r, CH)
                        for job in live:
                            p = jnp.exp2(load(s_row(i, job[2], t, job[3]), CH) - m)
                            l = p if l is None else l + p
                            lhs[job, t] = p
                        lhs["l", i, t] = l

                at(base + shift + t, 1, fetch)
                if k == "B":
                    has_sum.add((i, t))

                    def keep_sum(i=i, t=t, lhs=lhs):
                        pending["l", i, t] -= 1
                        store(_OFF["L"] + i * BQ + t, lhs["l", i, t])

                    at(base + shift + t + CH - 16 + _SUM_LAG, 0, keep_sum)

        for job, shift in jobs:
            def matmul(job=job, lhs=lhs, res=res):
                k, _, j, t0 = job
                a = jnp.concatenate([lhs[job, t] for t in range(t0, BQ, CH)], axis=0)
                a = a.astype(BF) if k == "B" else pltpu.bitcast(a, BF)
                if k == "o":
                    res[job] = _nn(a, wo[:, j * T:(j + 1) * T])
                    return
                region = {"A": "K", "B": "V"}.get(k, "W" + k)
                if k in "AB":
                    settled(region.lower(), j // 2, (j % 2) * T + T - CH)
                b = pltpu.bitcast(load(_OFF[region] + j * T // 2, T // 2), BF)
                res[job] = _nt(a, b) if k == "A" else _nn(a, b)

            at(base + shift + BQ - CH, 2, matmul)

        for (k, i, shift), group in groups.items():
            for t in range(0, BQ, CH):
                live = [job for job in group if t >= job[3]]
                if not live:
                    continue
                first = (k, i, t) not in has_acc
                has_acc.add((k, i, t))
                left[k, i, t] -= len(live)
                last = left[k, i, t] == 0

                def finish(k=k, i=i, t=t, live=live, lhs=lhs, res=res, first=first, last=last):
                    r = i * BQ + t
                    pending[k, i, t] -= 1
                    assert k == "o" or last == (pending[k, i, t] == 0), (k, i, t)
                    parts = [res[job][t - job[3]:t - job[3] + CH] for job in live]
                    if k == "o":
                        for job, v in zip(live, parts):
                            a = _OFF["O"] + job[2] * S + r
                            v = v if assign else load(a, CH) + v
                            store(a, residual(job[2], r, v) if residual else v)
                    elif k == "A":
                        mx = None if first else load(_OFF["MX"] + r, CH)
                        for job, v in zip(live, parts):
                            if job[2] == 2 * i + t // T:
                                d = lhs["d", job, t]
                                v = jnp.concatenate(
                                    [jnp.where(d <= u, v[u:u + 8], MASKED)
                                     for u in range(0, CH, 8)], axis=0)
                            store(s_row(i, job[2], t, job[3]), v)
                            mx = v if mx is None else jnp.maximum(mx, v)
                        if last:
                            res["m", i, t] = jnp.broadcast_to(
                                jnp.max(mx, axis=1, keepdims=True), (CH, T))
                        else:
                            store(_OFF["MX"] + r, mx)
                    else:
                        a = _OFF["PA"] + r if k == "B" else _OFF["ACC"] + "qkv".index(k) * BQ + t
                        acc = None if first else load(a, CH)
                        for v in parts:
                            acc = v if acc is None else acc + v
                        if not last:
                            store(a, acc)
                        elif k == "B":
                            settled("l", i, t)
                            l = jnp.sum(load(_OFF["L"] + r, CH), axis=1, keepdims=True)
                            store(_OFF["X"] + r // 2, _pack(acc * (1.0 / l)))
                        elif k == "q":
                            store(_OFF["Q"] + r // 2, _pack(acc * QSCALE))
                        else:
                            store(_OFF[k.upper()] + r // 2, _pack(acc))

                ready = base + shift + t + CH - 16 + (_CTX_LAG if k == "B" and last else _RES_LAG)
                when = max(base + shift + BQ, ready)
                expect(k, i, t)
                at(when, 0, finish)
                if k == "o" and last:
                    complete[i * BQ + t] = when
                if k == "A" and last:
                    def keep_max(i=i, t=t, res=res):
                        pending["m", i, t] -= 1
                        store(_OFF["M"] + i * BQ + t, res["m", i, t])

                    expect("m", i, t)
                    at(max(when, ready + _MAX_LAG), 0, keep_max)

    busy = [any(job[0] == "B" for s2 in (max(s - 1, 0), s) for lane in slots[s2] for job in lane)
            for s in range(len(slots))]
    if next_weights:
        todo = [(k, r) for k, n in (("q", M), ("k", C), ("v", C)) for r in range(0, n, 16)]
        calm = [s for s in range(last_use.get("q", 0) // BQ, len(slots) - 2) if not busy[s]]
        for n, (k, r) in enumerate(todo):
            step = BQ * len(calm) * n // len(todo)
            time = BQ * calm[step // BQ] + step % BQ
            assert time >= last_use.get(k, 0)
            at(time, 0, lambda k=k, r=r: next_weights(k, r))
    for time, fn in extras:
        at(time, 0, fn)
    if finalize:
        time = 0
        for r in range(0, S, FR):
            heavy = time // BQ < len(slots) and busy[time // BQ]
            time = max(time + _FIN_STEP[heavy], complete[r // CH * CH])
            for delay, fn in finalize(r):
                at(time + delay, 0, fn)

    for event in sorted(events, key=lambda e: e[:3]):
        event[3]()


def _row_sum(tiles):
    total = tiles[0]
    for tile in tiles[1:]:
        total = total + tile
    return jnp.broadcast_to(jnp.sum(total, axis=1, keepdims=True), total.shape)


def _mean(x1):
    return _row_sum(x1) * (1.0 / M)


def _inv_std(x1, mean):
    var = _row_sum([jnp.square(t - mean) for t in x1]) * (1.0 / M)
    return 1.0 / _rnd(jnp.sqrt(_rnd(_rnd(var) + EPS)))


def _norm2(x1, mean, inv_std, scale, shift):
    mean = _rnd(mean)
    return [_rnd((t - mean) * inv_std * a + b) for t, a, b in zip(x1, scale, shift)]


def _kernel(x_hbm, ckv_hbm, wq_hbm, wk_hbm, wv_hbm, wo_hbm, wr_hbm, wg_hbm, wu_hbm,
            wd_hbm, c_hbm, wmod_hbm, out_hbm,
            w, x_v, ckv_v, wq_v, wk_v, wv_v, wo_v, wr_v, wgu_v, wgu_t, wd_v, c_v,
            wmod_v, silu_v, mod_v, out_v, sem_in, sem_x, sem_c, sem_w, sem_o, sem_out, sem_fix):
    pairs = {"q": wq_v, "k": wk_v, "v": wv_v}
    nb = S // BQ

    def rows(i, n=1):
        return pl.ds(i * BQ, n * BQ)

    def pair_copies(p):
        heads = pl.ds(2 * p, 2)
        return [pltpu.make_async_copy(src.at[:, :, heads, :], dst.at[(p & 1)],
                                      sem_w.at[3 * ((p & 1)) + n])
                for n, (src, dst) in enumerate(((wq_hbm, wq_v), (wk_hbm, wk_v), (wv_hbm, wv_v)))]

    def wo_copy(h):
        return pltpu.make_async_copy(wo_hbm.at[h], wo_v.at[(h & 1)], sem_o.at[(h & 1)])

    def weights_of(h):
        def select(k, r):
            a = _OFF["W" + k] + r // 2
            w[a:a + 8, :] = _select_head(pairs[k], (h >> 1) & 1, r, (h & 1))
        return select

    def weight(k, n):
        return pltpu.bitcast(w[_OFF["W" + k]:_OFF["W" + k] + n // 2, :], BF)

    def put(region, i, v):
        for j in range(v.shape[1] // T):
            a = _OFF[region] + (j * S + i * BQ) // 2
            w[a:a + v.shape[0], :] = v[:, j * T:(j + 1) * T]

    c_copy = pltpu.make_async_copy(c_hbm, c_v, sem_in.at[0])
    early, late = pl.ds(0, 2 * M), pl.ds(2 * M, 4 * M)
    mod_a_copy, mod_b_copy, wg_copy, wu_copy, wd_copy, wr_copy = [
        pltpu.make_async_copy(src, dst, sem_in.at[1 + n]) for n, (src, dst) in enumerate((
            (wmod_hbm.at[:, early], wmod_v.at[:, early]),
            (wmod_hbm.at[:, late], wmod_v.at[:, late]),
            (wg_hbm, wgu_v.at[pl.ds(0, F)]), (wu_hbm, wgu_v.at[pl.ds(F, F)]),
            (wd_hbm, wd_v), (wr_hbm, wr_v)))]

    def block_copies(i):
        return [pltpu.make_async_copy(x_hbm.at[rows(i)], x_v.at[rows(i)], sem_x.at[i]),
                pltpu.make_async_copy(ckv_hbm.at[rows(i)], ckv_v.at[rows(i)], sem_c.at[i])]

    def start(copies):
        for copy in copies:
            copy.start()

    def wait(copies):
        for copy in copies:
            copy.wait()

    start(pair_copies(0) + [c_copy, mod_a_copy])
    w[_OFF["D"]:_OFF["D"] + T, :] = (
        lax.broadcasted_iota(I32, (T, T), 1) - lax.broadcasted_iota(I32, (T, T), 0)).astype(F32)
    w[_OFF["R"]:_OFF["R"] + 16, :] = jnp.zeros((16, T), F32)
    wait(pair_copies(0))
    start(block_copies(0))
    for k, n in (("q", M), ("k", C), ("v", C)):
        for r in range(0, n, 16):
            weights_of(0)(k, r)
    origin = pl.multiple_of(pltpu.bitcast(w[_OFF["R"]:_OFF["R"] + 8, :], I32)[0, 0], 16)
    c_copy.wait()
    c = jnp.broadcast_to(c_v[...].astype(F32), (16, M))
    silu_c = (c * jax.nn.sigmoid(c)).astype(BF)
    silu_v[...] = jnp.concatenate([silu_c.astype(F32)] * (T // 16), axis=0).T
    mod_a_copy.wait()
    start(block_copies(1))
    mod = _rnd(_nn(silu_c, wmod_v[:, early])[:1])
    shift_a, scale_a = mod[:, :M], _rnd(1.0 + mod[:, M:])

    for i in range(nb):
        wait(block_copies(i))
        start(block_copies(i + 2) if i + 2 < nb else
              [wo_copy(i + 2 - nb)] + (pair_copies(1) if i == nb - 1 else []))
        ckv = pltpu.bitcast(ckv_v[rows(i), :], F32)
        put("C", i, ckv)
        put("K", i, _pack(_nn(pltpu.bitcast(ckv, BF), weight("k", C))))
        put("V", i, _pack(_nn(pltpu.bitcast(ckv, BF), weight("v", C))))
        x = x_v[rows(i), :].astype(F32)
        xc = x - jnp.mean(x, axis=1, keepdims=True)
        var = jnp.mean(xc * xc, axis=1, keepdims=True)
        h = _pack(xc * lax.rsqrt(var + EPS) * scale_a + shift_a)
        put("H", i, h)
        h, wq = pltpu.bitcast(h, BF), weight("q", M)
        q = _nn(h[:, :4 * T], wq[:4 * T])
        q += jnp.concatenate([_nn(h[t:t + BQ // 4, 4 * T:], wq[4 * T:])
                              for t in range(0, BQ, BQ // 4)], axis=0)
        put("Q", i, _pack(q * QSCALE))
    wo_copy(0).wait()
    start([wg_copy, wu_copy])

    _head(_SEQ_FIRST, w, origin, wo_v.at[0], assign=True, next_weights=weights_of(1))

    wait([wg_copy, wu_copy])

    def head_step(h, carry):
        wo_copy(h).wait()
        pl.when(h == 2 * MT)(mod_b_copy.wait)

        @pl.when((h & 1) == 1)
        def _():
            for copy in pair_copies((h >> 1) + 1):
                copy.wait()

        wo_copy(h + 1).start()
        for n, copy in enumerate((mod_b_copy, wd_copy, wr_copy)):
            pl.when(h == 2 * n + 1)(copy.start)

        @pl.when(jnp.logical_and((h & 1) == 0, h + 2 < H))
        def _():
            for copy in pair_copies((h >> 1) + 1):
                copy.start()

        pad = pl.ds(_OFF["PAD"], 8)

        def modulation(k):
            lanes, ks = pl.ds(pl.multiple_of((h - 1) * T, T), T), pl.ds(k * T, T)
            part = jnp.sum(silu_v[ks, :] * wmod_v[ks, lanes].astype(F32), axis=0, keepdims=True)
            total = jnp.broadcast_to(part, (8, T)) + (w[pad, :] if k else 0.0)
            w[pad, :] = total
            if k == MT - 1:
                mod_v[h - 1] = total

        def transpose():
            n = jnp.minimum(h - 1, 2 * F // T - 1)
            wgu_t[n] = pltpu.bitcast(wgu_v[pl.ds(pl.multiple_of(n * T, T), T), :].T, F32)
            w[pad, :] = wgu_t[n + origin, :8, :]

        extras = [(T * (k + 1), lambda k=k: modulation(k)) for k in range(MT)]
        _head(_SEQ, w, origin, wo_v.at[(h & 1)], next_weights=weights_of(h + 1),
              extras=extras + [(5 * BQ, transpose)])
        return carry

    assert H - 2 == 6 * MT >= 2 * F // T
    lax.fori_loop(1, H - 1, head_step, 0)

    wait([wo_copy(H - 1), wd_copy, wr_copy])
    vectors = ("gate_a", "shift_b", "scale_b", "gate_b", "w_r")

    def set_vector(name, v):
        for j in range(MT):
            a = _OFF["MOD"] + (vectors.index(name) * MT + j) * 8
            w[a:a + 8, :] = v[:, j * T:(j + 1) * T]

    def vector(name, n, tiles=range(MT)):
        a = _OFF["MOD"] + vectors.index(name) * MT * 8
        return [jnp.concatenate([w[a + 8 * j:a + 8 * j + 8, :]] * (n // 8), axis=0)
                for j in tiles]

    mod = _rnd(jnp.concatenate([mod_v[j] for j in range(2 * MT, 6 * MT)], axis=1))
    set_vector("gate_a", mod[:, :M])
    set_vector("shift_b", mod[:, M:2 * M])
    set_vector("scale_b", _rnd(1.0 + mod[:, 2 * M:3 * M]))
    set_vector("gate_b", mod[:, 3 * M:])
    set_vector("w_r", jnp.broadcast_to(wr_v[...].astype(F32).reshape(1, M), (8, M)))
    out_copies = [pltpu.make_async_copy(out_v.at[rows(i)], out_hbm.at[rows(i)], sem_out.at[i])
                  for i in range(nb)]

    def residual(j, r, attn):
        gate, = vector("gate_a", CH, [j])
        return _rnd(x_v[r:r + CH, j * T:(j + 1) * T].astype(F32) + gate * attn)

    def finalize(r):
        x1_at = [pl.ds(_OFF["O"] + j * S + r, FR) for j in range(MT)]
        mean_at, inv_at = pl.ds(_OFF["MX"] + r, FR), pl.ds(_OFF["M"] + r, FR)

        def keep_mean():
            w[mean_at, :] = _mean([w[a, :] for a in x1_at])

        def keep_inv_std():
            w[inv_at, :] = _inv_std([w[a, :] for a in x1_at], w[mean_at, :])

        def output():
            x1 = [w[a, :] for a in x1_at]
            h2 = _norm2(x1, w[mean_at, :], w[inv_at, :],
                        vector("scale_b", FR), vector("shift_b", FR))
            out = [t + g * h for t, g, h in zip(x1, vector("gate_b", FR), h2)]
            out_v[r:r + FR, :] = jnp.concatenate(out, axis=1).astype(BF)
            score = _row_sum([h * v for h, v in zip(h2, vector("w_r", FR))])
            at = pl.ds(_OFF["R"] + r // (8 * T) * 8, 8)
            lane = lax.broadcasted_iota(I32, (8, T), 1)
            tile = w[at, :]
            for t in range(0, FR, 8):
                tile = jnp.where(lane == (r + t) // 8 % T, score[t:t + 8], tile)
            w[at, :] = tile
            if (r + FR) % BQ == 0:
                out_copies[r // BQ].start()

        return [(_FIN_LAG, keep_mean), (2 * _FIN_LAG + 64, keep_inv_std),
                (3 * _FIN_LAG + 128 + _FIN_TILE, output)]

    _head(_SEQ_LAST, w, origin, wo_v.at[(H - 1) % 2], residual=residual, finalize=finalize)

    score = _rnd(w[_OFF["R"]:_OFF["R"] + 16, :])
    bits = pltpu.bitcast(jnp.where(score == 0.0, 0.0, score), I32) >> 16
    rank = jnp.where(bits < 0, -1 - bits, bits + 0x8000)
    rank = jnp.where(score != score, 0, rank)
    sub = lax.broadcasted_iota(I32, (16, T), 0)
    row = (sub >> 3) * (8 * T) + 8 * lax.broadcasted_iota(I32, (16, T), 1) + (sub & 7)
    key = pltpu.bitcast((rank << 11) | (S - 1 - row) | (1 << 29), F32)
    best = jnp.broadcast_to(jnp.max(key, axis=0, keepdims=True), (T, T))
    place = jnp.sum(jnp.where(best.T > best, 1.0, 0.0), axis=0, keepdims=True)
    chosen = place == lax.broadcasted_iota(I32, (TOPK, T), 0).astype(F32)
    key = jnp.concatenate([jnp.where(chosen, key[n:n + 1], 0.0) for n in range(16)], axis=0)
    key = jnp.broadcast_to(jnp.max(key, axis=1, keepdims=True), key.shape)
    picked = []
    for _ in range(TOPK):
        top = jnp.max(key, axis=0, keepdims=True)
        key = jnp.where(key == top, 0.0, key)
        top = pltpu.bitcast(jnp.broadcast_to(top, (8, T)), I32)
        picked.append(S - 1 - (top[0, 0] & (S - 1)))

    wait(out_copies)

    def gather(at):
        return jnp.concatenate([w[pl.ds(at + r, 1), :] for r in picked], axis=0)

    x1 = [gather(_OFF["O"] + j * S) for j in range(MT)]
    h2 = _norm2(x1, gather(_OFF["MX"]), gather(_OFF["M"]),
                vector("scale_b", 8), vector("shift_b", 8))
    r_sel = _rnd(_row_sum([h * v for h, v in zip(h2, vector("w_r", 8))]))[:, :1]
    x1, h2 = jnp.concatenate(x1, axis=1), jnp.concatenate(h2, axis=1)
    gu = _rnd(jnp.concatenate([_nn(h2.astype(BF), pltpu.bitcast(wgu_t[j], BF))
                               for j in range(2 * F // T)], axis=1))
    g, u = gu[:, :F], gu[:, F:]
    y = _nn((_rnd(g * jax.nn.sigmoid(g)) * u).astype(BF), wd_v[...])
    new = x1 + jnp.concatenate(vector("gate_b", 8), axis=1) * (h2 + y * jax.nn.sigmoid(r_sel))

    groups = [pl.ds(pl.multiple_of((r >> 4) << 4, 16), 16) for r in picked]
    line = lax.broadcasted_iota(I32, (16, M), 0)
    for n, r in enumerate(picked):
        old = out_v[groups[n], :].astype(F32)
        out_v[groups[n], :] = jnp.where(line == (r & 15), new[n:n + 1], old).astype(BF)

    fixes = []
    for n, r in enumerate(picked):
        fresh = True
        for earlier in picked[:n]:
            fresh = jnp.logical_and(fresh, (earlier >> 4) != (r >> 4))
        fixes.append((fresh, pltpu.make_async_copy(
            out_v.at[groups[n]], out_hbm.at[groups[n]], sem_fix.at[n])))
    for fresh, copy in fixes:
        pl.when(fresh)(copy.start)
    for fresh, copy in fixes:
        pl.when(fresh)(copy.wait)


@jax.jit
def pallas_adaLN_cond__compressed_kv_cla__moe_arch_mod__prompt_kernel(
    A_x: jax.Array,
    A_c_kv: jax.Array,
    A_w_q: jax.Array,
    A_w_uk: jax.Array,
    A_w_uv: jax.Array,
    A_w_o: jax.Array,
    B_x: jax.Array,
    B_w_r: jax.Array,
    B_w_gate: jax.Array,
    B_w_up: jax.Array,
    B_w_down: jax.Array,
    c: jax.Array,
    w_mod: jax.Array,
):
    del B_x
    assert A_x.shape == (1, S, M) and A_c_kv.shape == (1, S, C)
    assert A_w_q.shape == (M, H, D) and B_w_gate.shape == (M, F)
    dma = pltpu.SemaphoreType.DMA
    out = pl.pallas_call(
        _kernel,
        in_specs=[pl.BlockSpec(memory_space=pl.ANY)] * 12,
        out_specs=pl.BlockSpec(memory_space=pl.ANY),
        out_shape=jax.ShapeDtypeStruct((S, M), BF),
        scratch_shapes=[
            pltpu.VMEM((_ROWS, T), F32),
            pltpu.VMEM((S, M), BF), pltpu.VMEM((S, C), BF),
            pltpu.VMEM((2, M // 2, 2, 2, D), BF), pltpu.VMEM((2, C // 2, 2, 2, D), BF),
            pltpu.VMEM((2, C // 2, 2, 2, D), BF), pltpu.VMEM((2, D, M), BF),
            pltpu.VMEM((M,), BF),
            pltpu.VMEM((2 * F, M), BF), pltpu.VMEM((2 * F // T, M // 2, T), F32),
            pltpu.VMEM((F, M), BF),
            pltpu.VMEM((1, M), BF),
            pltpu.VMEM((M, 6 * M), BF), pltpu.VMEM((M, T), F32), pltpu.VMEM((6 * MT, 8, T), F32),
            pltpu.VMEM((S, M), BF),
            dma((7,)), dma((S // BQ,)), dma((S // BQ,)), dma((6,)), dma((2,)),
            dma((S // BQ,)), dma((TOPK,)),
        ],
        compiler_params=pltpu.CompilerParams(vmem_limit_bytes=100 * 2 ** 20),
        name="adaln_attn_moe",
    )(A_x[0], A_c_kv[0], A_w_q.reshape(M // 2, 2, H, D), A_w_uk.reshape(C // 2, 2, H, D),
      A_w_uv.reshape(C // 2, 2, H, D), A_w_o, B_w_r,
      B_w_gate.T, B_w_up.T, B_w_down, c, w_mod)
    return out[None]
```

```python
import jax
import jax.numpy as jnp
from jax import lax
import jax.experimental.pallas as pl
import jax.experimental.pallas.tpu as pltpu

BF = jnp.bfloat16
F32 = jnp.float32
I32 = jnp.int32
U32 = jnp.uint32

S = 2048
M = 640
C = 512
H = 32
D = 128
F = 1728
TOPK = 8
EPS = 1e-5
LOG2E = 1.4426950408889634
QSCALE = D ** -0.5 * LOG2E
MASKED = -1e9 * LOG2E

T = 128
BQ = 256
CH = 64
MT = M // T
CT = C // T

_OFF = {}
_ROWS = 0
for _name, _n in (
    ("H", MT * S // 2), ("C", CT * S // 2),
    ("Q", S // 2), ("K", S // 2), ("V", S // 2), ("X", S // 2),
    ("Wq", M // 2), ("Wk", C // 2), ("Wv", C // 2),
    ("S", (S // BQ) ** 2 * BQ), ("SD", S // 2),
    ("MX", S), ("M", S), ("L", S), ("ACC", 3 * BQ), ("PA", S),
    ("O", MT * S), ("D", T), ("R", 16), ("PAD", 8), ("MOD", 5 * MT * 8),
):
    _OFF[_name] = _ROWS
    _ROWS += _n

_SEQ = (
    "q0 k0 q1 k1 q2 v0 A0+A1 A0 q3 q4 B0 A1 k2 v1 q5 B1 A2 B0+A2 q6 q7 v2 k3 "
    "B2 A3 B1+A3 v3 k4 k5 k6 k7 B3 A4 B2+A4 v4 v5 v6 v7 B4 A5 B3+A5 o0 o1 "
    "B5 A6 B4+A6 o2 o3 B6 A7 B5+A7 o4 o5 B6+B7 B7 o6 o7"
)
_SEQ_FIRST = (
    "A0+A1 A0 A1 A2+A3 A2 A3 B0+B1 B0 B1 A4+A5 A4 B2+B3 B2 B3 o0 o1 A5 A6+A7 A6 "
    "B4+B5 B4 B5 o2 o3 A7 o4 o5 B6+B7 B6 B7 o6 o7"
)
_SEQ_LAST = (
    "q0 q1 k0 k1 v0 A0+A1 A0 A1 v1 q2 k2 B0+B1 B0 B1 k3 q3 o0 o1 A2+A3 A2 v2 k4 q4 v3 "
    "B2+A4 B2 A3 q5 k5 o2 B3+A5 B3 A4 v4 q6 k6 o3 B4+A6 B4 A5 v5 q7 k7 o4 "
    "B5+A7 B5 A6 v6 o5 v7 A7 B6 B6+B7 B7 o6 o7"
)
_RES_LAG, _CTX_LAG, _MAX_LAG, _SUM_LAG = 208, 208, 192, 80
import os
_FIN_STEP, _FIN_LAG = eval(os.environ.get('FS','(80, 192)')), int(os.environ.get('FL',176))
FR = int(os.environ.get('FR',16))
_SEQ_LAST=os.environ.get('SL',_SEQ_LAST)
_FIN_TILE = int(os.environ.get('FT',0))


def _slots(seq):
    lanes = []
    for word in seq.split():
        if "+" in word:
            lanes.append(tuple(
                (p[0], int(p[1:]), 2 * int(p[1:]) + 1, T) for p in word.split("+")))
        else:
            k, (i, *part) = word[0], map(int, word[1:].split(":"))
            n = {"q": MT, "k": CT, "v": CT, "o": MT, "A": 2 * i + 1, "B": 2 * i + 1}[k]
            lanes += [((k, i, j, 0),) for j in range(*(part or [n]))]
    assert len(lanes) % 4 == 0
    return [lanes[s:s + 4] for s in range(0, len(lanes), 4)]


def _nt(a, b):
    return lax.dot_general(a, b, (((1,), (1,)), ((), ())), preferred_element_type=F32)


def _nn(a, b):
    return jnp.dot(a, b, preferred_element_type=F32)


def _rnd(x):
    if x.shape[1] == T and x.shape[0] % 16 == 0:
        half = x.shape[0] // 2
        y = _rnd(jnp.concatenate([x[:half], x[half:]], axis=1))
        return jnp.concatenate([y[:, :T], y[:, T:]], axis=0)
    return x.astype(BF).astype(F32)


def _pack(x):
    return pltpu.bitcast(x.astype(BF), F32)


def _select_head(src, slot, r, parity):
    even = pltpu.bitcast(src[slot, r // 2:r // 2 + 8, 0], U32).reshape(8, T)
    odd = pltpu.bitcast(src[slot, r // 2:r // 2 + 8, 1], U32).reshape(8, T)
    down = jnp.asarray(16 * parity, U32)
    word = ((even >> down) & 0xFFFF) | ((odd >> down) << 16)
    return pltpu.bitcast(word, F32)


def _head(seq, w, zero, wo, *, assign=False, next_weights=None, residual=None,
          finalize=None, extras=()):
    def load(r, n):
        return w[r:r + n, :]

    def ordered(r, n):
        head = w[pl.ds(zero + r, 8), :]
        return head if n == 8 else jnp.concatenate([head, load(r + 8, n - 8)], axis=0)

    def store(r, v):
        w[r:r + v.shape[0], :] = v

    def s_row(i, j, t, half):
        if half:
            return _OFF["SD"] + i * T + t - T
        return _OFF["S"] + (i * i + j) * BQ + t

    events = []

    def at(time, rank, fn):
        events.append((time, rank, len(events), fn))

    slots = _slots(seq)
    left = {}
    for slot in slots:
        for lane in slot:
            for k, i, _, t0 in lane:
                for t in range(t0, BQ, CH):
                    left[k, i, t] = left.get((k, i, t), 0) + 1
    has_sum, has_acc, last_use, complete = set(), set(), {}, {}
    pending = {}

    def expect(*tag):
        pending[tag] = pending.get(tag, 0) + 1
        return pending[tag]

    def settled(*tag):
        assert not pending.get(tag), tag

    for s, slot in enumerate(slots):
        base = BQ * s
        jobs = ([(lane[0], -T) for lane in slot if len(lane) == 2]
                + [(lane[0], 0) for lane in slot if len(lane) == 1]
                + [(lane[1], 0) for lane in slot if len(lane) == 2])
        lhs, res, groups = {}, {}, {}
        for job, shift in jobs:
            groups.setdefault((job[0], job[1], shift), []).append(job)
            last_use[job[0]] = base + BQ

        for (k, i, shift), group in groups.items():
            for t in range(0, BQ, CH):
                live = [job for job in group if t >= job[3]]
                if not live:
                    continue

                def fetch(k=k, i=i, t=t, live=live, lhs=lhs, first=(i, t) not in has_sum):
                    r = i * BQ + t
                    if k in "qkv":
                        src = _OFF["H" if k == "q" else "C"] + r // 2
                        for job in live:
                            get = ordered if job == live[0] else load
                            lhs[job, t] = get(src + job[2] * S // 2, CH // 2)
                    elif k in "Ao":
                        settled("q" if k == "A" else "B", i, t)
                        v = ordered(_OFF["Q" if k == "A" else "X"] + r // 2, CH // 2)
                        for job in live:
                            lhs[job, t] = v
                            if k == "A" and job[2] == 2 * i + t // T:
                                lhs["d", job, t] = ordered(_OFF["D"] + t % T, 8)
                    else:
                        settled("A", i, t)
                        settled("m", i, t)
                        settled("l", i, t)
                        expect("l", i, t)
                        m = ordered(_OFF["M"] + r, CH)
                        l = None if first else load(_OFF["L"] + r, CH)
                        for job in live:
                            p = jnp.exp2(load(s_row(i, job[2], t, job[3]), CH) - m)
                            l = p if l is None else l + p
                            lhs[job, t] = p
                        lhs["l", i, t] = l

                at(base + shift + t, 1, fetch)
                if k == "B":
                    has_sum.add((i, t))

                    def keep_sum(i=i, t=t, lhs=lhs):
                        pending["l", i, t] -= 1
                        store(_OFF["L"] + i * BQ + t, lhs["l", i, t])

                    at(base + shift + t + CH - 16 + _SUM_LAG, 0, keep_sum)

        for job, shift in jobs:
            def matmul(job=job, lhs=lhs, res=res):
                k, _, j, t0 = job
                a = jnp.concatenate([lhs[job, t] for t in range(t0, BQ, CH)], axis=0)
                a = a.astype(BF) if k == "B" else pltpu.bitcast(a, BF)
                if k == "o":
                    res[job] = _nn(a, wo[:, j * T:(j + 1) * T])
                    return
                region = {"A": "K", "B": "V"}.get(k, "W" + k)
                if k in "AB":
                    settled(region.lower(), j // 2, (j % 2) * T + T - CH)
                b = pltpu.bitcast(load(_OFF[region] + j * T // 2, T // 2), BF)
                res[job] = _nt(a, b) if k == "A" else _nn(a, b)

            at(base + shift + BQ - CH, 2, matmul)

        for (k, i, shift), group in groups.items():
            for t in range(0, BQ, CH):
                live = [job for job in group if t >= job[3]]
                if not live:
                    continue
                first = (k, i, t) not in has_acc
                has_acc.add((k, i, t))
                left[k, i, t] -= len(live)
                last = left[k, i, t] == 0

                def finish(k=k, i=i, t=t, live=live, lhs=lhs, res=res, first=first, last=last):
                    r = i * BQ + t
                    pending[k, i, t] -= 1
                    assert k == "o" or last == (pending[k, i, t] == 0), (k, i, t)
                    parts = [res[job][t - job[3]:t - job[3] + CH] for job in live]
                    if k == "o":
                        for job, v in zip(live, parts):
                            a = _OFF["O"] + job[2] * S + r
                            v = v if assign else load(a, CH) + v
                            store(a, residual(job[2], r, v) if residual else v)
                    elif k == "A":
                        mx = None if first else load(_OFF["MX"] + r, CH)
                        for job, v in zip(live, parts):
                            if job[2] == 2 * i + t // T:
                                d = lhs["d", job, t]
                                v = jnp.concatenate(
                                    [jnp.where(d <= u, v[u:u + 8], MASKED)
                                     for u in range(0, CH, 8)], axis=0)
                            store(s_row(i, job[2], t, job[3]), v)
                            mx = v if mx is None else jnp.maximum(mx, v)
                        if last:
                            res["m", i, t] = jnp.broadcast_to(
                                jnp.max(mx, axis=1, keepdims=True), (CH, T))
                        else:
                            store(_OFF["MX"] + r, mx)
                    else:
                        a = _OFF["PA"] + r if k == "B" else _OFF["ACC"] + "qkv".index(k) * BQ + t
                        acc = None if first else load(a, CH)
                        for v in parts:
                            acc = v if acc is None else acc + v
                        if not last:
                            store(a, acc)
                        elif k == "B":
                            settled("l", i, t)
                            l = jnp.sum(load(_OFF["L"] + r, CH), axis=1, keepdims=True)
                            store(_OFF["X"] + r // 2, _pack(acc * (1.0 / l)))
                        elif k == "q":
                            store(_OFF["Q"] + r // 2, _pack(acc * QSCALE))
                        else:
                            store(_OFF[k.upper()] + r // 2, _pack(acc))

                ready = base + shift + t + CH - 16 + (_CTX_LAG if k == "B" and last else _RES_LAG)
                when = max(base + shift + BQ, ready)
                expect(k, i, t)
                at(when, 0, finish)
                if k == "o" and last:
                    complete[i * BQ + t] = when
                if k == "A" and last:
                    def keep_max(i=i, t=t, res=res):
                        pending["m", i, t] -= 1
                        store(_OFF["M"] + i * BQ + t, res["m", i, t])

                    expect("m", i, t)
                    at(max(when, ready + _MAX_LAG), 0, keep_max)

    busy = [any(job[0] == "B" for s2 in (max(s - 1, 0), s) for lane in slots[s2] for job in lane)
            for s in range(len(slots))]
    if next_weights:
        todo = [(k, r) for k, n in (("q", M), ("k", C), ("v", C)) for r in range(0, n, 16)]
        calm = [s for s in range(last_use.get("q", 0) // BQ, len(slots) - 2) if not busy[s]]
        for n, (k, r) in enumerate(todo):
            step = BQ * len(calm) * n // len(todo)
            time = BQ * calm[step // BQ] + step % BQ
            assert time >= last_use.get(k, 0)
            at(time, 0, lambda k=k, r=r: next_weights(k, r))
    for time, fn in extras:
        at(time, 0, fn)
    if finalize:
        time = 0
        for r in range(0, S, FR):
            heavy = time // BQ < len(slots) and busy[time // BQ]
            time = max(time + _FIN_STEP[heavy], complete[r // CH * CH])
            for delay, fn in finalize(r):
                at(time + delay, 0, fn)

    for event in sorted(events, key=lambda e: e[:3]):
        event[3]()


def _row_sum(tiles):
    total = tiles[0]
    for tile in tiles[1:]:
        total = total + tile
    return jnp.broadcast_to(jnp.sum(total, axis=1, keepdims=True), total.shape)


def _mean(x1):
    return _row_sum(x1) * (1.0 / M)


def _inv_std(x1, mean):
    var = _row_sum([jnp.square(t - mean) for t in x1]) * (1.0 / M)
    return 1.0 / _rnd(jnp.sqrt(_rnd(_rnd(var) + EPS)))


def _norm2(x1, mean, inv_std, scale, shift):
    mean = _rnd(mean)
    return [_rnd((t - mean) * inv_std * a + b) for t, a, b in zip(x1, scale, shift)]


def _kernel(x_hbm, ckv_hbm, wq_hbm, wk_hbm, wv_hbm, wo_hbm, wr_hbm, wg_hbm, wu_hbm,
            wd_hbm, c_hbm, wmod_hbm, out_hbm,
            w, x_v, ckv_v, wq_v, wk_v, wv_v, wo_v, wr_v, wgu_v, wgu_t, wd_v, c_v,
            wmod_v, silu_v, mod_v, out_v, sem_in, sem_x, sem_c, sem_w, sem_o, sem_out, sem_fix):
    pairs = {"q": wq_v, "k": wk_v, "v": wv_v}
    nb = S // BQ

    def rows(i, n=1):
        return pl.ds(i * BQ, n * BQ)

    def pair_copies(p):
        heads = pl.ds(2 * p, 2)
        return [pltpu.make_async_copy(src.at[:, :, heads, :], dst.at[(p & 1)],
                                      sem_w.at[3 * ((p & 1)) + n])
                for n, (src, dst) in enumerate(((wq_hbm, wq_v), (wk_hbm, wk_v), (wv_hbm, wv_v)))]

    wo_first, wo_next, wo_rest = [
        pltpu.make_async_copy(wo_hbm.at[heads], wo_v.at[heads], sem_o.at[n])
        for n, heads in enumerate((pl.ds(0, 1), pl.ds(1, 2 * MT - 1), pl.ds(2 * MT, H - 2 * MT)))]

    def weights_of(h):
        def select(k, r):
            a = _OFF["W" + k] + r // 2
            w[a:a + 8, :] = _select_head(pairs[k], (h >> 1) & 1, r, (h & 1))
        return select

    def weight(k, n):
        return pltpu.bitcast(w[_OFF["W" + k]:_OFF["W" + k] + n // 2, :], BF)

    def put(region, i, v):
        for j in range(v.shape[1] // T):
            a = _OFF[region] + (j * S + i * BQ) // 2
            w[a:a + v.shape[0], :] = v[:, j * T:(j + 1) * T]

    c_copy = pltpu.make_async_copy(c_hbm, c_v, sem_in.at[0])
    early, late = pl.ds(0, 2 * M), pl.ds(2 * M, 4 * M)
    mod_a_copy, mod_b_copy, wg_copy, wu_copy, wd_copy, wr_copy = [
        pltpu.make_async_copy(src, dst, sem_in.at[1 + n]) for n, (src, dst) in enumerate((
            (wmod_hbm.at[:, early], wmod_v.at[:, early]),
            (wmod_hbm.at[:, late], wmod_v.at[:, late]),
            (wg_hbm, wgu_v.at[pl.ds(0, F)]), (wu_hbm, wgu_v.at[pl.ds(F, F)]),
            (wd_hbm, wd_v), (wr_hbm, wr_v)))]

    def block_copies(i):
        return [pltpu.make_async_copy(x_hbm.at[rows(i)], x_v.at[rows(i)], sem_x.at[i]),
                pltpu.make_async_copy(ckv_hbm.at[rows(i)], ckv_v.at[rows(i)], sem_c.at[i])]

    def start(copies):
        for copy in copies:
            copy.start()

    def wait(copies):
        for copy in copies:
            copy.wait()

    start(pair_copies(0) + [c_copy, mod_a_copy])
    w[_OFF["D"]:_OFF["D"] + T, :] = (
        lax.broadcasted_iota(I32, (T, T), 1) - lax.broadcasted_iota(I32, (T, T), 0)).astype(F32)
    w[_OFF["R"]:_OFF["R"] + 16, :] = jnp.zeros((16, T), F32)
    wait(pair_copies(0))
    start(block_copies(0))
    for k, n in (("q", M), ("k", C), ("v", C)):
        for r in range(0, n, 16):
            weights_of(0)(k, r)
    origin = pl.multiple_of(pltpu.bitcast(w[_OFF["R"]:_OFF["R"] + 8, :], I32)[0, 0], 16)
    c_copy.wait()
    c = jnp.broadcast_to(c_v[...].astype(F32), (16, M))
    silu_c = (c * jax.nn.sigmoid(c)).astype(BF)
    silu_v[...] = jnp.concatenate([silu_c.astype(F32)] * (T // 16), axis=0).T
    mod_a_copy.wait()
    start(block_copies(1))
    mod = _rnd(_nn(silu_c, wmod_v[:, early])[:1])
    shift_a, scale_a = mod[:, :M], _rnd(1.0 + mod[:, M:])

    for i in range(nb):
        wait(block_copies(i))
        start(block_copies(i + 2) if i + 2 < nb else
              pair_copies(1) if i == nb - 1 else [wo_first])
        ckv = pltpu.bitcast(ckv_v[rows(i), :], F32)
        put("C", i, ckv)
        put("K", i, _pack(_nn(pltpu.bitcast(ckv, BF), weight("k", C))))
        put("V", i, _pack(_nn(pltpu.bitcast(ckv, BF), weight("v", C))))
        x = x_v[rows(i), :].astype(F32)
        xc = x - jnp.mean(x, axis=1, keepdims=True)
        var = jnp.mean(xc * xc, axis=1, keepdims=True)
        h = _pack(xc * lax.rsqrt(var + EPS) * scale_a + shift_a)
        put("H", i, h)
        h, wq = pltpu.bitcast(h, BF), weight("q", M)
        q = _nn(h[:, :4 * T], wq[:4 * T])
        q += jnp.concatenate([_nn(h[t:t + BQ // 4, 4 * T:], wq[4 * T:])
                              for t in range(0, BQ, BQ // 4)], axis=0)
        put("Q", i, _pack(q * QSCALE))
    wo_first.wait()
    start([wo_next, wg_copy])

    _head(_SEQ_FIRST, w, origin, wo_v.at[0], assign=True, next_weights=weights_of(1))

    wait([wo_next, wg_copy])
    start([mod_b_copy, wo_rest, wu_copy])

    def head_step(h, carry):
        pl.when(h == 2 * MT)(lambda: wait([mod_b_copy, wo_rest, wu_copy]))

        @pl.when((h & 1) == 1)
        def _():
            for copy in pair_copies((h >> 1) + 1):
                copy.wait()

        pl.when(h == 3)(lambda: start([wd_copy, wr_copy]))

        @pl.when(jnp.logical_and((h & 1) == 0, h + 2 < H))
        def _():
            for copy in pair_copies((h >> 1) + 1):
                copy.start()

        pad = pl.ds(_OFF["PAD"], 8)

        def modulation(k):
            lanes, ks = pl.ds(pl.multiple_of((h - 1) * T, T), T), pl.ds(k * T, T)
            part = jnp.sum(silu_v[ks, :] * wmod_v[ks, lanes].astype(F32), axis=0, keepdims=True)
            total = jnp.broadcast_to(part, (8, T)) + (w[pad, :] if k else 0.0)
            w[pad, :] = total
            if k == MT - 1:
                mod_v[h - 1] = total

        def transpose():
            n = jnp.minimum(h - 1, 2 * F // T - 1)
            wgu_t[n] = pltpu.bitcast(wgu_v[pl.ds(pl.multiple_of(n * T, T), T), :].T, F32)
            w[pad, :] = wgu_t[n + origin, :8, :]

        extras = [(T * (k + 1), lambda k=k: modulation(k)) for k in range(MT)]
        _head(_SEQ, w, origin, wo_v.at[h], next_weights=weights_of(h + 1),
              extras=extras + [(5 * BQ, transpose)])
        return carry

    assert H - 2 == 6 * MT >= 2 * F // T
    lax.fori_loop(1, H - 1, head_step, 0)

    wait([wd_copy, wr_copy])
    vectors = ("gate_a", "shift_b", "scale_b", "gate_b", "w_r")

    def set_vector(name, v):
        for j in range(MT):
            a = _OFF["MOD"] + (vectors.index(name) * MT + j) * 8
            w[a:a + 8, :] = v[:, j * T:(j + 1) * T]

    def vector(name, n, tiles=range(MT)):
        a = _OFF["MOD"] + vectors.index(name) * MT * 8
        return [jnp.concatenate([w[a + 8 * j:a + 8 * j + 8, :]] * (n // 8), axis=0)
                for j in tiles]

    mod = _rnd(jnp.concatenate([mod_v[j] for j in range(2 * MT, 6 * MT)], axis=1))
    set_vector("gate_a", mod[:, :M])
    set_vector("shift_b", mod[:, M:2 * M])
    set_vector("scale_b", _rnd(1.0 + mod[:, 2 * M:3 * M]))
    set_vector("gate_b", mod[:, 3 * M:])
    set_vector("w_r", jnp.broadcast_to(wr_v[...].astype(F32).reshape(1, M), (8, M)))
    out_copies = [pltpu.make_async_copy(out_v.at[rows(i)], out_hbm.at[rows(i)], sem_out.at[i])
                  for i in range(nb)]

    def residual(j, r, attn):
        gate, = vector("gate_a", CH, [j])
        return _rnd(x_v[r:r + CH, j * T:(j + 1) * T].astype(F32) + gate * attn)

    def finalize(r):
        x1_at = [pl.ds(_OFF["O"] + j * S + r, FR) for j in range(MT)]
        mean_at, inv_at = pl.ds(_OFF["MX"] + r, FR), pl.ds(_OFF["M"] + r, FR)

        def keep_mean():
            w[mean_at, :] = _mean([w[a, :] for a in x1_at])

        def keep_inv_std():
            w[inv_at, :] = _inv_std([w[a, :] for a in x1_at], w[mean_at, :])

        def output():
            x1 = [w[a, :] for a in x1_at]
            h2 = _norm2(x1, w[mean_at, :], w[inv_at, :],
                        vector("scale_b", FR), vector("shift_b", FR))
            out = [t + g * h for t, g, h in zip(x1, vector("gate_b", FR), h2)]
            out_v[r:r + FR, :] = jnp.concatenate(out, axis=1).astype(BF)
            score = _row_sum([h * v for h, v in zip(h2, vector("w_r", FR))])
            at = pl.ds(_OFF["R"] + r // (8 * T) * 8, 8)
            lane = lax.broadcasted_iota(I32, (8, T), 1)
            tile = w[at, :]
            for t in range(0, FR, 8):
                tile = jnp.where(lane == (r + t) // 8 % T, score[t:t + 8], tile)
            w[at, :] = tile
            if (r + FR) % BQ == 0:
                out_copies[r // BQ].start()

        return [(_FIN_LAG, keep_mean), (2 * _FIN_LAG + 64, keep_inv_std),
                (3 * _FIN_LAG + 128 + _FIN_TILE, output)]

    _head(_SEQ_LAST, w, origin, wo_v.at[H - 1], residual=residual, finalize=finalize)

    score = _rnd(w[_OFF["R"]:_OFF["R"] + 16, :])
    bits = pltpu.bitcast(jnp.where(score == 0.0, 0.0, score), I32) >> 16
    rank = jnp.where(bits < 0, -1 - bits, bits + 0x8000)
    rank = jnp.where(score != score, 0, rank)
    sub = lax.broadcasted_iota(I32, (16, T), 0)
    row = (sub >> 3) * (8 * T) + 8 * lax.broadcasted_iota(I32, (16, T), 1) + (sub & 7)
    key = pltpu.bitcast((rank << 11) | (S - 1 - row) | (1 << 29), F32)
    best = jnp.broadcast_to(jnp.max(key, axis=0, keepdims=True), (T, T))
    place = jnp.sum(jnp.where(best.T > best, 1.0, 0.0), axis=0, keepdims=True)
    chosen = place == lax.broadcasted_iota(I32, (TOPK, T), 0).astype(F32)
    key = jnp.concatenate([jnp.where(chosen, key[n:n + 1], 0.0) for n in range(16)], axis=0)
    key = jnp.broadcast_to(jnp.max(key, axis=1, keepdims=True), key.shape)
    picked = []
    for _ in range(TOPK):
        top = jnp.max(key, axis=0, keepdims=True)
        key = jnp.where(key == top, 0.0, key)
        top = pltpu.bitcast(jnp.broadcast_to(top, (8, T)), I32)
        picked.append(S - 1 - (top[0, 0] & (S - 1)))

    wait(out_copies)

    def gather(at):
        return jnp.concatenate([w[pl.ds(at + r, 1), :] for r in picked], axis=0)

    x1 = [gather(_OFF["O"] + j * S) for j in range(MT)]
    h2 = _norm2(x1, gather(_OFF["MX"]), gather(_OFF["M"]),
                vector("scale_b", 8), vector("shift_b", 8))
    r_sel = _rnd(_row_sum([h * v for h, v in zip(h2, vector("w_r", 8))]))[:, :1]
    x1, h2 = jnp.concatenate(x1, axis=1), jnp.concatenate(h2, axis=1)
    gu = _rnd(jnp.concatenate([_nn(h2.astype(BF), pltpu.bitcast(wgu_t[j], BF))
                               for j in range(2 * F // T)], axis=1))
    g, u = gu[:, :F], gu[:, F:]
    y = _nn((_rnd(g * jax.nn.sigmoid(g)) * u).astype(BF), wd_v[...])
    new = x1 + jnp.concatenate(vector("gate_b", 8), axis=1) * (h2 + y * jax.nn.sigmoid(r_sel))

    groups = [pl.ds(pl.multiple_of((r >> 4) << 4, 16), 16) for r in picked]
    line = lax.broadcasted_iota(I32, (16, M), 0)
    for n, r in enumerate(picked):
        old = out_v[groups[n], :].astype(F32)
        out_v[groups[n], :] = jnp.where(line == (r & 15), new[n:n + 1], old).astype(BF)

    fixes = []
    for n, r in enumerate(picked):
        fresh = True
        for earlier in picked[:n]:
            fresh = jnp.logical_and(fresh, (earlier >> 4) != (r >> 4))
        fixes.append((fresh, pltpu.make_async_copy(
            out_v.at[groups[n]], out_hbm.at[groups[n]], sem_fix.at[n])))
    for fresh, copy in fixes:
        pl.when(fresh)(copy.start)
    for fresh, copy in fixes:
        pl.when(fresh)(copy.wait)


@jax.jit
def pallas_adaLN_cond__compressed_kv_cla__moe_arch_mod__prompt_kernel(
    A_x: jax.Array,
    A_c_kv: jax.Array,
    A_w_q: jax.Array,
    A_w_uk: jax.Array,
    A_w_uv: jax.Array,
    A_w_o: jax.Array,
    B_x: jax.Array,
    B_w_r: jax.Array,
    B_w_gate: jax.Array,
    B_w_up: jax.Array,
    B_w_down: jax.Array,
    c: jax.Array,
    w_mod: jax.Array,
):
    del B_x
    assert A_x.shape == (1, S, M) and A_c_kv.shape == (1, S, C)
    assert A_w_q.shape == (M, H, D) and B_w_gate.shape == (M, F)
    dma = pltpu.SemaphoreType.DMA
    out = pl.pallas_call(
        _kernel,
        in_specs=[pl.BlockSpec(memory_space=pl.ANY)] * 12,
        out_specs=pl.BlockSpec(memory_space=pl.ANY),
        out_shape=jax.ShapeDtypeStruct((S, M), BF),
        scratch_shapes=[
            pltpu.VMEM((_ROWS, T), F32),
            pltpu.VMEM((S, M), BF), pltpu.VMEM((S, C), BF),
            pltpu.VMEM((2, M // 2, 2, 2, D), BF), pltpu.VMEM((2, C // 2, 2, 2, D), BF),
            pltpu.VMEM((2, C // 2, 2, 2, D), BF), pltpu.VMEM((H, D, M), BF),
            pltpu.VMEM((M,), BF),
            pltpu.VMEM((2 * F, M), BF), pltpu.VMEM((2 * F // T, M // 2, T), F32),
            pltpu.VMEM((F, M), BF),
            pltpu.VMEM((1, M), BF),
            pltpu.VMEM((M, 6 * M), BF), pltpu.VMEM((M, T), F32), pltpu.VMEM((6 * MT, 8, T), F32),
            pltpu.VMEM((S, M), BF),
            dma((7,)), dma((S // BQ,)), dma((S // BQ,)), dma((6,)), dma((3,)),
            dma((S // BQ,)), dma((TOPK,)),
        ],
        compiler_params=pltpu.CompilerParams(vmem_limit_bytes=100 * 2 ** 20),
        name="adaln_attn_moe",
    )(A_x[0], A_c_kv[0], A_w_q.reshape(M // 2, 2, H, D), A_w_uk.reshape(C // 2, 2, H, D),
      A_w_uv.reshape(C // 2, 2, H, D), A_w_o, B_w_r,
      B_w_gate.T, B_w_up.T, B_w_down, c, w_mod)
    return out[None]
```

```python
import jax
import jax.numpy as jnp
from jax import lax
import jax.experimental.pallas as pl
import jax.experimental.pallas.tpu as pltpu

BF = jnp.bfloat16
F32 = jnp.float32
I32 = jnp.int32
U32 = jnp.uint32

S = 2048
M = 640
C = 512
H = 32
D = 128
F = 1728
TOPK = 8
EPS = 1e-5
LOG2E = 1.4426950408889634
QSCALE = D ** -0.5 * LOG2E
MASKED = -1e9 * LOG2E

T = 128
BQ = 256
CH = 64
MT = M // T
CT = C // T

_OFF = {}
_ROWS = 0
for _name, _n in (
    ("H", MT * S // 2), ("C", CT * S // 2),
    ("Q", S // 2), ("K", S // 2), ("V", S // 2), ("X", S // 2),
    ("Wq", M // 2), ("Wk", C // 2), ("Wv", C // 2),
    ("S", (S // BQ) ** 2 * BQ), ("SD", S // 2),
    ("MX", S), ("M", S), ("L", S), ("ACC", 3 * BQ), ("PA", S),
    ("O", MT * S), ("D", T), ("R", 16), ("PAD", 8), ("MOD", 5 * MT * 8),
):
    _OFF[_name] = _ROWS
    _ROWS += _n

_SEQ = (
    "q0 k0 q1 k1 q2 v0 A0+A1 A0 q3 q4 B0 A1 k2 v1 q5 B1 A2 B0+A2 q6 q7 v2 k3 "
    "B2 A3 B1+A3 v3 k4 k5 k6 k7 B3 A4 B2+A4 v4 v5 v6 v7 B4 A5 B3+A5 o0 o1 "
    "B5 A6 B4+A6 o2 o3 B6 A7 B5+A7 o4 o5 B6+B7 B7 o6 o7"
)
_SEQ_FIRST = (
    "A0+A1 A0 A1 A2+A3 A2 A3 B0+B1 B0 B1 A4+A5 A4 B2+B3 B2 B3 o0 o1 A5 A6+A7 A6 "
    "B4+B5 B4 B5 o2 o3 A7 o4 o5 B6+B7 B6 B7 o6 o7"
)
_SEQ_LAST = (
    "q0 q1 k0 k1 v0 A0+A1 A0 A1 v1 q2 k2 B0+B1 B0 B1 k3 q3 o0 o1 A2+A3 A2 v2 k4 q4 v3 "
    "B2+A4 B2 A3 q5 k5 o2 B3+A5 B3 A4 v4 q6 k6 o3 B4+A6 B4 A5 v5 q7 k7 o4 "
    "B5+A7 B5 A6 v6 o5 v7 A7 B6 B6+B7 B7 o6 o7"
)
_RES_LAG, _CTX_LAG, _MAX_LAG, _SUM_LAG = 208, 208, 192, 80
FR = 16
_FIN_STEP, _FIN_LAG = (80, 192), 176


def _slots(seq):
    lanes = []
    for word in seq.split():
        if "+" in word:
            lanes.append(tuple(
                (p[0], int(p[1:]), 2 * int(p[1:]) + 1, T) for p in word.split("+")))
        else:
            k, i = word[0], int(word[1:])
            n = {"q": MT, "k": CT, "v": CT, "o": MT, "A": 2 * i + 1, "B": 2 * i + 1}[k]
            lanes += [((k, i, j, 0),) for j in range(n)]
    assert len(lanes) % 4 == 0
    return [lanes[s:s + 4] for s in range(0, len(lanes), 4)]


def _nt(a, b):
    return lax.dot_general(a, b, (((1,), (1,)), ((), ())), preferred_element_type=F32)


def _nn(a, b):
    return jnp.dot(a, b, preferred_element_type=F32)


def _rnd(x):
    if x.shape[1] == T and x.shape[0] % 16 == 0:
        half = x.shape[0] // 2
        y = _rnd(jnp.concatenate([x[:half], x[half:]], axis=1))
        return jnp.concatenate([y[:, :T], y[:, T:]], axis=0)
    return x.astype(BF).astype(F32)


def _pack(x):
    return pltpu.bitcast(x.astype(BF), F32)


def _select_head(src, slot, r, parity):
    even = pltpu.bitcast(src[slot, r // 2:r // 2 + 8, 0], U32).reshape(8, T)
    odd = pltpu.bitcast(src[slot, r // 2:r // 2 + 8, 1], U32).reshape(8, T)
    down = jnp.asarray(16 * parity, U32)
    word = ((even >> down) & 0xFFFF) | ((odd >> down) << 16)
    return pltpu.bitcast(word, F32)


def _head(seq, w, zero, wo, *, assign=False, next_weights=None, residual=None,
          finalize=None, extras=()):
    def load(r, n):
        return w[r:r + n, :]

    def ordered(r, n):
        head = w[pl.ds(zero + r, 8), :]
        return head if n == 8 else jnp.concatenate([head, load(r + 8, n - 8)], axis=0)

    def store(r, v):
        w[r:r + v.shape[0], :] = v

    def s_row(i, j, t, half):
        if half:
            return _OFF["SD"] + i * T + t - T
        return _OFF["S"] + (i * i + j) * BQ + t

    events = []

    def at(time, rank, fn):
        events.append((time, rank, len(events), fn))

    slots = _slots(seq)
    left = {}
    for slot in slots:
        for lane in slot:
            for k, i, _, t0 in lane:
                for t in range(t0, BQ, CH):
                    left[k, i, t] = left.get((k, i, t), 0) + 1
    has_sum, has_acc, last_use, complete = set(), set(), {}, {}
    pending = {}

    def expect(*tag):
        pending[tag] = pending.get(tag, 0) + 1

    def settled(*tag):
        assert not pending.get(tag), tag

    for s, slot in enumerate(slots):
        base = BQ * s
        jobs = ([(lane[0], -T) for lane in slot if len(lane) == 2]
                + [(lane[0], 0) for lane in slot if len(lane) == 1]
                + [(lane[1], 0) for lane in slot if len(lane) == 2])
        lhs, res, groups = {}, {}, {}
        for job, shift in jobs:
            groups.setdefault((job[0], job[1], shift), []).append(job)
            last_use[job[0]] = base + BQ

        for (k, i, shift), group in groups.items():
            for t in range(0, BQ, CH):
                live = [job for job in group if t >= job[3]]
                if not live:
                    continue

                def fetch(k=k, i=i, t=t, live=live, lhs=lhs, first=(i, t) not in has_sum):
                    r = i * BQ + t
                    if k in "qkv":
                        src = _OFF["H" if k == "q" else "C"] + r // 2
                        for job in live:
                            get = ordered if job == live[0] else load
                            lhs[job, t] = get(src + job[2] * S // 2, CH // 2)
                    elif k in "Ao":
                        settled("q" if k == "A" else "B", i, t)
                        v = ordered(_OFF["Q" if k == "A" else "X"] + r // 2, CH // 2)
                        for job in live:
                            lhs[job, t] = v
                            if k == "A" and job[2] == 2 * i + t // T:
                                lhs["d", job, t] = ordered(_OFF["D"] + t % T, 8)
                    else:
                        settled("A", i, t)
                        settled("m", i, t)
                        settled("l", i, t)
                        expect("l", i, t)
                        m = ordered(_OFF["M"] + r, CH)
                        l = None if first else load(_OFF["L"] + r, CH)
                        for job in live:
                            p = jnp.exp2(load(s_row(i, job[2], t, job[3]), CH) - m)
                            l = p if l is None else l + p
                            lhs[job, t] = p
                        lhs["l", i, t] = l

                at(base + shift + t, 1, fetch)
                if k == "B":
                    has_sum.add((i, t))

                    def keep_sum(i=i, t=t, lhs=lhs):
                        pending["l", i, t] -= 1
                        store(_OFF["L"] + i * BQ + t, lhs["l", i, t])

                    at(base + shift + t + CH - 16 + _SUM_LAG, 0, keep_sum)

        for job, shift in jobs:
            def matmul(job=job, lhs=lhs, res=res):
                k, _, j, t0 = job
                a = jnp.concatenate([lhs[job, t] for t in range(t0, BQ, CH)], axis=0)
                a = a.astype(BF) if k == "B" else pltpu.bitcast(a, BF)
                if k == "o":
                    res[job] = _nn(a, wo[:, j * T:(j + 1) * T])
                    return
                region = {"A": "K", "B": "V"}.get(k, "W" + k)
                if k in "AB":
                    settled(region.lower(), j // 2, (j % 2) * T + T - CH)
                b = pltpu.bitcast(load(_OFF[region] + j * T // 2, T // 2), BF)
                res[job] = _nt(a, b) if k == "A" else _nn(a, b)

            at(base + shift + BQ - CH, 2, matmul)

        for (k, i, shift), group in groups.items():
            for t in range(0, BQ, CH):
                live = [job for job in group if t >= job[3]]
                if not live:
                    continue
                first = (k, i, t) not in has_acc
                has_acc.add((k, i, t))
                left[k, i, t] -= len(live)
                last = left[k, i, t] == 0

                def finish(k=k, i=i, t=t, live=live, lhs=lhs, res=res, first=first, last=last):
                    r = i * BQ + t
                    pending[k, i, t] -= 1
                    assert k == "o" or last == (pending[k, i, t] == 0), (k, i, t)
                    parts = [res[job][t - job[3]:t - job[3] + CH] for job in live]
                    if k == "o":
                        for job, v in zip(live, parts):
                            a = _OFF["O"] + job[2] * S + r
                            v = v if assign else load(a, CH) + v
                            store(a, residual(job[2], r, v) if residual else v)
                    elif k == "A":
                        mx = None if first else load(_OFF["MX"] + r, CH)
                        for job, v in zip(live, parts):
                            if job[2] == 2 * i + t // T:
                                d = lhs["d", job, t]
                                v = jnp.concatenate(
                                    [jnp.where(d <= u, v[u:u + 8], MASKED)
                                     for u in range(0, CH, 8)], axis=0)
                            store(s_row(i, job[2], t, job[3]), v)
                            mx = v if mx is None else jnp.maximum(mx, v)
                        if last:
                            res["m", i, t] = jnp.broadcast_to(
                                jnp.max(mx, axis=1, keepdims=True), (CH, T))
                        else:
                            store(_OFF["MX"] + r, mx)
                    else:
                        a = _OFF["PA"] + r if k == "B" else _OFF["ACC"] + "qkv".index(k) * BQ + t
                        acc = None if first else load(a, CH)
                        for v in parts:
                            acc = v if acc is None else acc + v
                        if not last:
                            store(a, acc)
                        elif k == "B":
                            settled("l", i, t)
                            l = jnp.sum(load(_OFF["L"] + r, CH), axis=1, keepdims=True)
                            store(_OFF["X"] + r // 2, _pack(acc * (1.0 / l)))
                        elif k == "q":
                            store(_OFF["Q"] + r // 2, _pack(acc * QSCALE))
                        else:
                            store(_OFF[k.upper()] + r // 2, _pack(acc))

                ready = base + shift + t + CH - 16 + (_CTX_LAG if k == "B" and last else _RES_LAG)
                when = max(base + shift + BQ, ready)
                expect(k, i, t)
                at(when, 0, finish)
                if k == "o" and last:
                    complete[i * BQ + t] = when
                if k == "A" and last:
                    def keep_max(i=i, t=t, res=res):
                        pending["m", i, t] -= 1
                        store(_OFF["M"] + i * BQ + t, res["m", i, t])

                    expect("m", i, t)
                    at(max(when, ready + _MAX_LAG), 0, keep_max)

    busy = [any(job[0] == "B" for s2 in (max(s - 1, 0), s) for lane in slots[s2] for job in lane)
            for s in range(len(slots))]
    if next_weights:
        todo = [(k, r) for k, n in (("q", M), ("k", C), ("v", C)) for r in range(0, n, 16)]
        calm = [s for s in range(last_use.get("q", 0) // BQ, len(slots) - 2) if not busy[s]]
        for n, (k, r) in enumerate(todo):
            step = BQ * len(calm) * n // len(todo)
            time = BQ * calm[step // BQ] + step % BQ
            assert time >= last_use.get(k, 0)
            at(time, 0, lambda k=k, r=r: next_weights(k, r))
    for time, fn in extras:
        at(time, 0, fn)
    if finalize:
        time = 0
        for r in range(0, S, FR):
            heavy = time // BQ < len(slots) and busy[time // BQ]
            time = max(time + _FIN_STEP[heavy], complete[r // CH * CH])
            for delay, fn in finalize(r):
                at(time + delay, 0, fn)

    for event in sorted(events, key=lambda e: e[:3]):
        event[3]()


def _row_sum(tiles):
    total = tiles[0]
    for tile in tiles[1:]:
        total = total + tile
    return jnp.broadcast_to(jnp.sum(total, axis=1, keepdims=True), total.shape)


def _mean(x1):
    return _row_sum(x1) * (1.0 / M)


def _inv_std(x1, mean):
    var = _row_sum([jnp.square(t - mean) for t in x1]) * (1.0 / M)
    return 1.0 / _rnd(jnp.sqrt(_rnd(_rnd(var) + EPS)))


def _norm2(x1, mean, inv_std, scale, shift):
    mean = _rnd(mean)
    return [_rnd((t - mean) * inv_std * a + b) for t, a, b in zip(x1, scale, shift)]


def _kernel(x_hbm, ckv_hbm, wq_hbm, wk_hbm, wv_hbm, wo_hbm, wr_hbm, wg_hbm, wu_hbm,
            wd_hbm, c_hbm, wmod_hbm, out_hbm,
            w, x_v, ckv_v, wq_v, wk_v, wv_v, wo_v, wr_v, wgu_v, wgu_t, wd_v, c_v,
            wmod_v, silu_v, mod_v, out_v, sem_in, sem_x, sem_c, sem_w, sem_o, sem_out, sem_fix):
    pairs = {"q": wq_v, "k": wk_v, "v": wv_v}
    nb = S // BQ

    def rows(i):
        return pl.ds(i * BQ, BQ)

    def pair_copies(p):
        heads = pl.ds(2 * p, 2)
        return [pltpu.make_async_copy(src.at[:, :, heads, :], dst.at[p & 1],
                                      sem_w.at[3 * (p & 1) + n])
                for n, (src, dst) in enumerate(((wq_hbm, wq_v), (wk_hbm, wk_v), (wv_hbm, wv_v)))]

    wo_first, wo_next, wo_rest = [
        pltpu.make_async_copy(wo_hbm.at[heads], wo_v.at[heads], sem_o.at[n])
        for n, heads in enumerate((pl.ds(0, 1), pl.ds(1, 2 * MT - 1), pl.ds(2 * MT, H - 2 * MT)))]

    def weights_of(h):
        def select(k, r):
            a = _OFF["W" + k] + r // 2
            w[a:a + 8, :] = _select_head(pairs[k], (h >> 1) & 1, r, h & 1)
        return select

    def weight(k, n):
        return pltpu.bitcast(w[_OFF["W" + k]:_OFF["W" + k] + n // 2, :], BF)

    def put(region, i, v):
        for j in range(v.shape[1] // T):
            a = _OFF[region] + (j * S + i * BQ) // 2
            w[a:a + v.shape[0], :] = v[:, j * T:(j + 1) * T]

    c_copy = pltpu.make_async_copy(c_hbm, c_v, sem_in.at[0])
    mod_copies = [pltpu.make_async_copy(wmod_hbm.at[:, pl.ds(n * M, M)], wmod_v.at[n],
                                        sem_in.at[1 + n]) for n in range(6)]
    wg_copy, wu_copy, wd_copy, wr_copy = [
        pltpu.make_async_copy(src, dst, sem_in.at[7 + n]) for n, (src, dst) in enumerate((
            (wg_hbm, wgu_v.at[pl.ds(0, F)]), (wu_hbm, wgu_v.at[pl.ds(F, F)]),
            (wd_hbm, wd_v), (wr_hbm, wr_v)))]

    def block_copies(i):
        return [pltpu.make_async_copy(x_hbm.at[rows(i)], x_v.at[rows(i)], sem_x.at[i]),
                pltpu.make_async_copy(ckv_hbm.at[rows(i)], ckv_v.at[rows(i)], sem_c.at[i])]

    def start(copies):
        for copy in copies:
            copy.start()

    def wait(copies):
        for copy in copies:
            copy.wait()

    start(pair_copies(0) + [c_copy] + mod_copies[:2])
    w[_OFF["D"]:_OFF["D"] + T, :] = (
        lax.broadcasted_iota(I32, (T, T), 1) - lax.broadcasted_iota(I32, (T, T), 0)).astype(F32)
    w[_OFF["R"]:_OFF["R"] + 16, :] = jnp.zeros((16, T), F32)
    wait(pair_copies(0))
    start(block_copies(0))
    for k, n in (("q", M), ("k", C), ("v", C)):
        for r in range(0, n, 16):
            weights_of(0)(k, r)
    origin = pl.multiple_of(pltpu.bitcast(w[_OFF["R"]:_OFF["R"] + 8, :], I32)[0, 0], 16)
    c_copy.wait()
    c = jnp.broadcast_to(c_v[...].astype(F32), (16, M))
    silu_c = (c * jax.nn.sigmoid(c)).astype(BF)
    silu_v[...] = jnp.concatenate([silu_c.astype(F32)] * (T // 16), axis=0).T
    mod_copies[0].wait()
    start(block_copies(1))
    shift_a = _rnd(_nn(silu_c, wmod_v[0])[:1])
    mod_copies[1].wait()
    scale_a = _rnd(1.0 + _rnd(_nn(silu_c, wmod_v[1])[:1]))

    for i in range(nb):
        wait(block_copies(i))
        start(block_copies(i + 2) if i + 2 < nb else
              pair_copies(1) if i == nb - 1 else [wo_first])
        ckv = pltpu.bitcast(ckv_v[rows(i), :], F32)
        put("C", i, ckv)
        put("K", i, _pack(_nn(pltpu.bitcast(ckv, BF), weight("k", C))))
        put("V", i, _pack(_nn(pltpu.bitcast(ckv, BF), weight("v", C))))
        x = x_v[rows(i), :].astype(F32)
        xc = x - jnp.mean(x, axis=1, keepdims=True)
        var = jnp.mean(xc * xc, axis=1, keepdims=True)
        h = _pack(xc * lax.rsqrt(var + EPS) * scale_a + shift_a)
        put("H", i, h)
        h, wq = pltpu.bitcast(h, BF), weight("q", M)
        q = _nn(h[:, :4 * T], wq[:4 * T])
        q += jnp.concatenate([_nn(h[t:t + BQ // 4, 4 * T:], wq[4 * T:])
                              for t in range(0, BQ, BQ // 4)], axis=0)
        put("Q", i, _pack(q * QSCALE))
    wo_first.wait()
    start([wo_next, wg_copy])

    _head(_SEQ_FIRST, w, origin, wo_v.at[0], assign=True, next_weights=weights_of(1))

    wait([wo_next, wg_copy])
    start(mod_copies[2:] + [wo_rest, wu_copy])

    def head_step(h, carry):
        pl.when(h == 2 * MT)(lambda: wait(mod_copies[2:] + [wo_rest, wu_copy]))

        pl.when((h & 1) == 1)(lambda: wait(pair_copies((h >> 1) + 1)))
        pl.when(h == 3)(lambda: start([wd_copy, wr_copy]))
        pl.when(jnp.logical_and((h & 1) == 0, h + 2 < H))(
            lambda: start(pair_copies((h >> 1) + 1)))

        pad = pl.ds(_OFF["PAD"], 8)

        def modulation(k):
            lanes = pl.ds(pl.multiple_of(lax.rem(h - 1, MT) * T, T), T)
            tile = wmod_v[lax.div(h - 1, MT), pl.ds(k * T, T), lanes].astype(F32)
            part = jnp.sum(silu_v[pl.ds(k * T, T), :] * tile, axis=0, keepdims=True)
            total = jnp.broadcast_to(part, (8, T)) + (w[pad, :] if k else 0.0)
            w[pad, :] = total
            if k == MT - 1:
                mod_v[h - 1] = total

        def transpose():
            n = jnp.minimum(h - 1, 2 * F // T - 1)
            wgu_t[n] = pltpu.bitcast(wgu_v[pl.ds(pl.multiple_of(n * T, T), T), :].T, F32)
            w[pad, :] = wgu_t[n + origin, :8, :]

        extras = [(T * (k + 1), lambda k=k: modulation(k)) for k in range(MT)]
        _head(_SEQ, w, origin, wo_v.at[h], next_weights=weights_of(h + 1),
              extras=extras + [(5 * BQ, transpose)])
        return carry

    assert H - 2 == 6 * MT >= 2 * F // T
    lax.fori_loop(1, H - 1, head_step, 0)

    wait([wd_copy, wr_copy])
    vectors = ("gate_a", "shift_b", "scale_b", "gate_b", "w_r")

    def set_vector(name, v):
        for j in range(MT):
            a = _OFF["MOD"] + (vectors.index(name) * MT + j) * 8
            w[a:a + 8, :] = v[:, j * T:(j + 1) * T]

    def vector(name, n, tiles=range(MT)):
        a = _OFF["MOD"] + vectors.index(name) * MT * 8
        return [jnp.concatenate([w[a + 8 * j:a + 8 * j + 8, :]] * (n // 8), axis=0)
                for j in tiles]

    mod = _rnd(jnp.concatenate([mod_v[j] for j in range(2 * MT, 6 * MT)], axis=1))
    set_vector("gate_a", mod[:, :M])
    set_vector("shift_b", mod[:, M:2 * M])
    set_vector("scale_b", _rnd(1.0 + mod[:, 2 * M:3 * M]))
    set_vector("gate_b", mod[:, 3 * M:])
    set_vector("w_r", jnp.broadcast_to(wr_v[...].astype(F32).reshape(1, M), (8, M)))
    out_copies = [pltpu.make_async_copy(out_v.at[rows(i)], out_hbm.at[rows(i)], sem_out.at[i])
                  for i in range(nb)]

    def residual(j, r, attn):
        gate, = vector("gate_a", CH, [j])
        return _rnd(x_v[r:r + CH, j * T:(j + 1) * T].astype(F32) + gate * attn)

    def finalize(r):
        x1_at = [pl.ds(_OFF["O"] + j * S + r, FR) for j in range(MT)]
        mean_at, inv_at = pl.ds(_OFF["MX"] + r, FR), pl.ds(_OFF["M"] + r, FR)

        def keep_mean():
            w[mean_at, :] = _mean([w[a, :] for a in x1_at])

        def keep_inv_std():
            w[inv_at, :] = _inv_std([w[a, :] for a in x1_at], w[mean_at, :])

        def output():
            x1 = [w[a, :] for a in x1_at]
            h2 = _norm2(x1, w[mean_at, :], w[inv_at, :],
                        vector("scale_b", FR), vector("shift_b", FR))
            out = [t + g * h for t, g, h in zip(x1, vector("gate_b", FR), h2)]
            out_v[r:r + FR, :] = jnp.concatenate(out, axis=1).astype(BF)
            score = _row_sum([h * v for h, v in zip(h2, vector("w_r", FR))])
            at = pl.ds(_OFF["R"] + r // (8 * T) * 8, 8)
            lane = lax.broadcasted_iota(I32, (8, T), 1)
            tile = w[at, :]
            for t in range(0, FR, 8):
                tile = jnp.where(lane == (r + t) // 8 % T, score[t:t + 8], tile)
            w[at, :] = tile
            if (r + FR) % BQ == 0:
                out_copies[r // BQ].start()

        return [(_FIN_LAG, keep_mean), (2 * _FIN_LAG + 64, keep_inv_std),
                (3 * _FIN_LAG + 128, output)]

    _head(_SEQ_LAST, w, origin, wo_v.at[H - 1], residual=residual, finalize=finalize)

    score = _rnd(w[_OFF["R"]:_OFF["R"] + 16, :])
    bits = pltpu.bitcast(jnp.where(score == 0.0, 0.0, score), I32) >> 16
    rank = jnp.where(bits < 0, -1 - bits, bits + 0x8000)
    rank = jnp.where(score != score, 0, rank)
    sub = lax.broadcasted_iota(I32, (16, T), 0)
    row = (sub >> 3) * (8 * T) + 8 * lax.broadcasted_iota(I32, (16, T), 1) + (sub & 7)
    key = pltpu.bitcast((rank << 11) | (S - 1 - row) | (1 << 29), F32)
    best = jnp.broadcast_to(jnp.max(key, axis=0, keepdims=True), (T, T))
    place = jnp.sum(jnp.where(best.T > best, 1.0, 0.0), axis=0, keepdims=True)
    chosen = place == lax.broadcasted_iota(I32, (TOPK, T), 0).astype(F32)
    key = jnp.concatenate([jnp.where(chosen, key[n:n + 1], 0.0) for n in range(16)], axis=0)
    key = jnp.broadcast_to(jnp.max(key, axis=1, keepdims=True), key.shape)
    picked = []
    for _ in range(TOPK):
        top = jnp.max(key, axis=0, keepdims=True)
        key = jnp.where(key == top, 0.0, key)
        top = pltpu.bitcast(jnp.broadcast_to(top, (8, T)), I32)
        picked.append(S - 1 - (top[0, 0] & (S - 1)))

    wait(out_copies)

    def gather(at):
        return jnp.concatenate([w[pl.ds(at + r, 1), :] for r in picked], axis=0)

    x1 = [gather(_OFF["O"] + j * S) for j in range(MT)]
    h2 = _norm2(x1, gather(_OFF["MX"]), gather(_OFF["M"]),
                vector("scale_b", 8), vector("shift_b", 8))
    r_sel = _rnd(_row_sum([h * v for h, v in zip(h2, vector("w_r", 8))]))[:, :1]
    x1, h2 = jnp.concatenate(x1, axis=1), jnp.concatenate(h2, axis=1)
    gu = _rnd(jnp.concatenate([_nn(h2.astype(BF), pltpu.bitcast(wgu_t[j], BF))
                               for j in range(2 * F // T)], axis=1))
    g, u = gu[:, :F], gu[:, F:]
    y = _nn((_rnd(g * jax.nn.sigmoid(g)) * u).astype(BF), wd_v[...])
    new = x1 + jnp.concatenate(vector("gate_b", 8), axis=1) * (h2 + y * jax.nn.sigmoid(r_sel))

    groups = [pl.ds(pl.multiple_of((r >> 4) << 4, 16), 16) for r in picked]
    line = lax.broadcasted_iota(I32, (16, M), 0)
    for n, r in enumerate(picked):
        old = out_v[groups[n], :].astype(F32)
        out_v[groups[n], :] = jnp.where(line == (r & 15), new[n:n + 1], old).astype(BF)

    fixes = []
    for n, r in enumerate(picked):
        fresh = True
        for earlier in picked[:n]:
            fresh = jnp.logical_and(fresh, (earlier >> 4) != (r >> 4))
        fixes.append((fresh, pltpu.make_async_copy(
            out_v.at[groups[n]], out_hbm.at[groups[n]], sem_fix.at[n])))
    for fresh, copy in fixes:
        pl.when(fresh)(copy.start)
    for fresh, copy in fixes:
        pl.when(fresh)(copy.wait)


@jax.jit
def pallas_adaLN_cond__compressed_kv_cla__moe_arch_mod__prompt_kernel(
    A_x: jax.Array,
    A_c_kv: jax.Array,
    A_w_q: jax.Array,
    A_w_uk: jax.Array,
    A_w_uv: jax.Array,
    A_w_o: jax.Array,
    B_x: jax.Array,
    B_w_r: jax.Array,
    B_w_gate: jax.Array,
    B_w_up: jax.Array,
    B_w_down: jax.Array,
    c: jax.Array,
    w_mod: jax.Array,
):
    del B_x
    assert A_x.shape == (1, S, M) and A_c_kv.shape == (1, S, C)
    assert A_w_q.shape == (M, H, D) and B_w_gate.shape == (M, F)
    dma = pltpu.SemaphoreType.DMA
    out = pl.pallas_call(
        _kernel,
        in_specs=[pl.BlockSpec(memory_space=pl.ANY)] * 12,
        out_specs=pl.BlockSpec(memory_space=pl.ANY),
        out_shape=jax.ShapeDtypeStruct((S, M), BF),
        scratch_shapes=[
            pltpu.VMEM((_ROWS, T), F32),
            pltpu.VMEM((S, M), BF), pltpu.VMEM((S, C), BF),
            pltpu.VMEM((2, M // 2, 2, 2, D), BF), pltpu.VMEM((2, C // 2, 2, 2, D), BF),
            pltpu.VMEM((2, C // 2, 2, 2, D), BF), pltpu.VMEM((H, D, M), BF),
            pltpu.VMEM((M,), BF),
            pltpu.VMEM((2 * F, M), BF), pltpu.VMEM((2 * F // T, M // 2, T), F32),
            pltpu.VMEM((F, M), BF),
            pltpu.VMEM((1, M), BF),
            pltpu.VMEM((6, M, M), BF), pltpu.VMEM((M, T), F32), pltpu.VMEM((6 * MT, 8, T), F32),
            pltpu.VMEM((S, M), BF),
            dma((11,)), dma((S // BQ,)), dma((S // BQ,)), dma((6,)), dma((3,)),
            dma((S // BQ,)), dma((TOPK,)),
        ],
        compiler_params=pltpu.CompilerParams(vmem_limit_bytes=100 * 2 ** 20),
        name="adaln_attn_moe",
    )(A_x[0], A_c_kv[0], A_w_q.reshape(M // 2, 2, H, D), A_w_uk.reshape(C // 2, 2, H, D),
      A_w_uv.reshape(C // 2, 2, H, D), A_w_o, B_w_r,
      B_w_gate.T, B_w_up.T, B_w_down, c, w_mod)
    return out[None]
```

```python
import jax
import jax.numpy as jnp
from jax import lax
import jax.experimental.pallas as pl
import jax.experimental.pallas.tpu as pltpu

BF = jnp.bfloat16
F32 = jnp.float32
I32 = jnp.int32
U32 = jnp.uint32

S = 2048
M = 640
C = 512
H = 32
D = 128
F = 1728
TOPK = 8
EPS = 1e-5
LOG2E = 1.4426950408889634
QSCALE = D ** -0.5 * LOG2E
MASKED = -1e9 * LOG2E

T = 128
BQ = 256
CH = 64
MT = M // T
CT = C // T

_OFF = {}
_ROWS = 0
for _name, _n in (
    ("H", MT * S // 2), ("C", CT * S // 2),
    ("Q", S // 2), ("K", S // 2), ("V", S // 2), ("X", S // 2),
    ("Wq", M // 2), ("Wk", C // 2), ("Wv", C // 2),
    ("K2", S // 2), ("V2", S // 2), ("Wq2", M // 2), ("Wk2", C // 2), ("Wv2", C // 2),
    ("S", (S // BQ) ** 2 * BQ), ("SD", S // 2),
    ("MX", S), ("M", S), ("L", S), ("ACC", 3 * BQ), ("PA", S),
    ("O", MT * S), ("D", T), ("R", 32), ("PAD", 8), ("MOD", 7 * MT * 8),
):
    _OFF[_name] = _ROWS
    _ROWS += _n

_SEQ = (
    "q0 k0 q1 k1 q2 v0 A0+A1 A0 q3 q4 B0 A1 k2 v1 q5 B1 A2 B0+A2 q6 q7 v2 k3 "
    "B2 A3 B1+A3 v3 k4 k5 k6 k7 B3 A4 B2+A4 v4 v5 v6 v7 B4 A5 B3+A5 o0 o1 "
    "B5 A6 B4+A6 o2 o3 B6 A7 B5+A7 o4 o5 B6+B7 B7 o6 o7"
)
_SEQ_FIRST = (
    "A0+A1 A0 A1 A2+A3 A2 A3 B0+B1 B0 B1 A4+A5 A4 B2+B3 B2 B3 o0 o1 A5 A6+A7 A6 "
    "B4+B5 B4 B5 o2 o3 A7 o4 o5 B6+B7 B6 B7 o6 o7"
)
_SEQ_LAST = (
    "q0 q1 q2 A0+A1 A0 A1 q3 q4 B0+B1 B0 B1 A2+A3 A2 o0 o1 B2 A3 B2+A4 q5 o2 B3+A5 B3 "
    "A4 q6 o3 B4+A6 B4 A5 q7 o4 B5+A7 B5 A6 o5 A7 B6 B6+B7 B7 o6 o7"
)
_RES_LAG, _CTX_LAG, _MAX_LAG, _SUM_LAG = 208, 208, 192, 80
FR = 16
_FIN_STEP, _FIN_LAG = (64, 128), 192


def _slots(seq):
    lanes = []
    for word in seq.split():
        if "+" in word:
            lanes.append(tuple(
                (p[0], int(p[1:]), 2 * int(p[1:]) + 1, T) for p in word.split("+")))
        else:
            k, i = word[0], int(word[1:])
            n = {"q": MT, "k": CT, "v": CT, "o": MT, "A": 2 * i + 1, "B": 2 * i + 1}[k]
            lanes += [((k, i, j, 0),) for j in range(n)]
    assert len(lanes) % 4 == 0
    return [lanes[s:s + 4] for s in range(0, len(lanes), 4)]


def _nt(a, b):
    return lax.dot_general(a, b, (((1,), (1,)), ((), ())), preferred_element_type=F32)


def _nn(a, b):
    return jnp.dot(a, b, preferred_element_type=F32)


def _rnd(x):
    if x.shape[1] == T and x.shape[0] % 16 == 0:
        half = x.shape[0] // 2
        y = _rnd(jnp.concatenate([x[:half], x[half:]], axis=1))
        return jnp.concatenate([y[:, :T], y[:, T:]], axis=0)
    return x.astype(BF).astype(F32)


def _pack(x):
    return pltpu.bitcast(x.astype(BF), F32)


def _select_head(even, odd, parity):
    down = jnp.asarray(16 * parity, U32)
    return pltpu.bitcast(((even >> down) & 0xFFFF) | ((odd >> down) << 16), F32)


def _head(seq, w, zero, wo, *, assign=False, next_weights=None, residual=None,
          finalize=None, extras=(), suffix=""):
    def load(r, n):
        return w[r:r + n, :]

    def ordered(r, n):
        head = w[pl.ds(zero + r, 8), :]
        return head if n == 8 else jnp.concatenate([head, load(r + 8, n - 8)], axis=0)

    def store(r, v):
        w[r:r + v.shape[0], :] = v

    def s_row(i, j, t, half):
        if half:
            return _OFF["SD"] + i * T + t - T
        return _OFF["S"] + (i * i + j) * BQ + t

    events = []

    def at(time, rank, fn):
        events.append((time, rank, len(events), fn))

    slots = _slots(seq)
    left = {}
    for slot in slots:
        for lane in slot:
            for k, i, _, t0 in lane:
                for t in range(t0, BQ, CH):
                    left[k, i, t] = left.get((k, i, t), 0) + 1
    has_sum, has_acc, last_use, complete = set(), set(), {}, {}
    pending = {}

    def expect(*tag):
        pending[tag] = pending.get(tag, 0) + 1

    def settled(*tag):
        assert not pending.get(tag), tag

    for s, slot in enumerate(slots):
        base = BQ * s
        jobs = ([(lane[0], -T) for lane in slot if len(lane) == 2]
                + [(lane[0], 0) for lane in slot if len(lane) == 1]
                + [(lane[1], 0) for lane in slot if len(lane) == 2])
        lhs, res, groups = {}, {}, {}
        for job, shift in jobs:
            groups.setdefault((job[0], job[1], shift), []).append(job)
            last_use[job[0]] = base + BQ

        for (k, i, shift), group in groups.items():
            for t in range(0, BQ, CH):
                live = [job for job in group if t >= job[3]]
                if not live:
                    continue

                def fetch(k=k, i=i, t=t, live=live, lhs=lhs, first=(i, t) not in has_sum):
                    r = i * BQ + t
                    if k in "qkv":
                        src = _OFF["H" if k == "q" else "C"] + r // 2
                        for job in live:
                            get = ordered if job == live[0] else load
                            lhs[job, t] = get(src + job[2] * S // 2, CH // 2)
                    elif k in "Ao":
                        settled("q" if k == "A" else "B", i, t)
                        v = ordered(_OFF["Q" if k == "A" else "X"] + r // 2, CH // 2)
                        for job in live:
                            lhs[job, t] = v
                            if k == "A" and job[2] == 2 * i + t // T:
                                lhs["d", job, t] = ordered(_OFF["D"] + t % T, 8)
                    else:
                        settled("A", i, t)
                        settled("m", i, t)
                        settled("l", i, t)
                        expect("l", i, t)
                        m = ordered(_OFF["M"] + r, CH)
                        l = None if first else load(_OFF["L"] + r, CH)
                        for job in live:
                            p = jnp.exp2(load(s_row(i, job[2], t, job[3]), CH) - m)
                            l = p if l is None else l + p
                            lhs[job, t] = p
                        lhs["l", i, t] = l

                at(base + shift + t, 1, fetch)
                if k == "B":
                    has_sum.add((i, t))

                    def keep_sum(i=i, t=t, lhs=lhs):
                        pending["l", i, t] -= 1
                        store(_OFF["L"] + i * BQ + t, lhs["l", i, t])

                    at(base + shift + t + CH - 16 + _SUM_LAG, 0, keep_sum)

        for job, shift in jobs:
            def matmul(job=job, lhs=lhs, res=res):
                k, _, j, t0 = job
                a = jnp.concatenate([lhs[job, t] for t in range(t0, BQ, CH)], axis=0)
                a = a.astype(BF) if k == "B" else pltpu.bitcast(a, BF)
                if k == "o":
                    res[job] = _nn(a, wo[:, j * T:(j + 1) * T])
                    return
                region = {"A": "K", "B": "V"}.get(k, "W" + k)
                if k in "AB":
                    settled(region.lower(), j // 2, (j % 2) * T + T - CH)
                b = pltpu.bitcast(load(_OFF[region + suffix] + j * T // 2, T // 2), BF)
                res[job] = _nt(a, b) if k == "A" else _nn(a, b)

            at(base + shift + BQ - CH, 2, matmul)

        for (k, i, shift), group in groups.items():
            for t in range(0, BQ, CH):
                live = [job for job in group if t >= job[3]]
                if not live:
                    continue
                first = (k, i, t) not in has_acc
                has_acc.add((k, i, t))
                left[k, i, t] -= len(live)
                last = left[k, i, t] == 0

                def finish(k=k, i=i, t=t, live=live, lhs=lhs, res=res, first=first, last=last):
                    r = i * BQ + t
                    pending[k, i, t] -= 1
                    assert k == "o" or last == (pending[k, i, t] == 0), (k, i, t)
                    parts = [res[job][t - job[3]:t - job[3] + CH] for job in live]
                    if k == "o":
                        for job, v in zip(live, parts):
                            a = _OFF["O"] + job[2] * S + r
                            v = v if assign else load(a, CH) + v
                            store(a, residual(job[2], r, v) if residual else v)
                    elif k == "A":
                        mx = None if first else load(_OFF["MX"] + r, CH)
                        for job, v in zip(live, parts):
                            if job[2] == 2 * i + t // T:
                                d = lhs["d", job, t]
                                v = jnp.concatenate(
                                    [jnp.where(d <= u, v[u:u + 8], MASKED)
                                     for u in range(0, CH, 8)], axis=0)
                            store(s_row(i, job[2], t, job[3]), v)
                            mx = v if mx is None else jnp.maximum(mx, v)
                        if last:
                            res["m", i, t] = jnp.broadcast_to(
                                jnp.max(mx, axis=1, keepdims=True), (CH, T))
                        else:
                            store(_OFF["MX"] + r, mx)
                    else:
                        a = _OFF["PA"] + r if k == "B" else _OFF["ACC"] + "qkv".index(k) * BQ + t
                        acc = None if first else load(a, CH)
                        for v in parts:
                            acc = v if acc is None else acc + v
                        if not last:
                            store(a, acc)
                        elif k == "B":
                            settled("l", i, t)
                            l = jnp.sum(load(_OFF["L"] + r, CH), axis=1, keepdims=True)
                            store(_OFF["X"] + r // 2, _pack(acc * (1.0 / l)))
                        elif k == "q":
                            store(_OFF["Q"] + r // 2, _pack(acc * QSCALE))
                        else:
                            store(_OFF[k.upper() + suffix] + r // 2, _pack(acc))

                ready = base + shift + t + CH - 16 + (_CTX_LAG if k == "B" and last else _RES_LAG)
                when = max(base + shift + BQ, ready)
                expect(k, i, t)
                at(when, 0, finish)
                if k == "o" and last:
                    complete[i * BQ + t] = when
                if k == "A" and last:
                    def keep_max(i=i, t=t, res=res):
                        pending["m", i, t] -= 1
                        store(_OFF["M"] + i * BQ + t, res["m", i, t])

                    expect("m", i, t)
                    at(max(when, ready + _MAX_LAG), 0, keep_max)

    busy = [any(job[0] == "B" for s2 in (max(s - 1, 0), s) for lane in slots[s2] for job in lane)
            for s in range(len(slots))]
    if next_weights:
        todo = [(k, r) for k, n in (("q", M), ("k", C), ("v", C)) for r in range(0, n, 16)]
        calm = [s for s in range(last_use.get("q", 0) // BQ, len(slots) - 2) if not busy[s]]
        for n, (k, r) in enumerate(todo):
            step = BQ * len(calm) * n // len(todo)
            time = BQ * calm[step // BQ] + step % BQ
            assert time >= last_use.get(k, 0)
            at(time, 0, lambda k=k, r=r: next_weights(k, r))
    for time, fn in extras:
        at(time, 0, fn)
    if finalize:
        time = 0
        for r in range(0, S, FR):
            heavy = time // BQ < len(slots) and busy[time // BQ]
            time = max(time + _FIN_STEP[heavy], complete[r // CH * CH])
            for delay, fn in finalize(r):
                at(time + delay, 0, fn)

    for event in sorted(events, key=lambda e: e[:3]):
        event[3]()


def _row_sum(tiles):
    total = tiles[0]
    for tile in tiles[1:]:
        total = total + tile
    return jnp.broadcast_to(jnp.sum(total, axis=1, keepdims=True), total.shape)


def _kernel(x_hbm, ckv_hbm, wq_hbm, wk_hbm, wv_hbm, wo_hbm, wr_hbm, wg_hbm, wu_hbm,
            wd_hbm, c_hbm, wmod_hbm, out_hbm,
            w, x_v, ckv_v, wq_v, wk_v, wv_v, wo_v, wr_v, wgu_v, wgu_t, wd_v, c_v,
            wmod_v, silu_v, mod_v, rows_v, out_v, sem_in, sem_x, sem_c, sem_w, sem_o, sem_out, sem_fix):
    pairs = {"q": wq_v, "k": wk_v, "v": wv_v}
    nb = S // BQ

    def rows(i):
        return pl.ds(i * BQ, BQ)

    def pair_copies(p):
        heads = pl.ds(2 * p, 2)
        return [pltpu.make_async_copy(src.at[:, :, heads, :], dst.at[p & 1],
                                      sem_w.at[3 * (p & 1) + n])
                for n, (src, dst) in enumerate(((wq_hbm, wq_v), (wk_hbm, wk_v), (wv_hbm, wv_v)))]

    wo_first, wo_next, wo_rest = [
        pltpu.make_async_copy(wo_hbm.at[heads], wo_v.at[heads], sem_o.at[n])
        for n, heads in enumerate((pl.ds(0, 1), pl.ds(1, 2 * MT - 1), pl.ds(2 * MT, H - 2 * MT)))]

    def pair_rows(k, slot, r):
        return [pltpu.bitcast(pairs[k][slot, r // 2:r // 2 + 8, odd], U32).reshape(8, T)
                for odd in range(2)]

    def weights_of(h):
        def select(k, r):
            a = _OFF["W" + k] + r // 2
            w[a:a + 8, :] = _select_head(*pair_rows(k, (h >> 1) & 1, r), h & 1)
        return select

    def weight(k, n):
        return pltpu.bitcast(w[_OFF["W" + k]:_OFF["W" + k] + n // 2, :], BF)

    def put(region, i, v):
        for j in range(v.shape[1] // T):
            a = _OFF[region] + (j * S + i * BQ) // 2
            w[a:a + v.shape[0], :] = v[:, j * T:(j + 1) * T]

    c_copy = pltpu.make_async_copy(c_hbm, c_v, sem_in.at[0])
    mod_copies = [pltpu.make_async_copy(wmod_hbm.at[:, pl.ds(n * M, M)], wmod_v.at[n],
                                        sem_in.at[1 + n]) for n in range(6)]
    wg_copy, wu_copy, wd_copy, wr_copy = [
        pltpu.make_async_copy(src, dst, sem_in.at[7 + n]) for n, (src, dst) in enumerate((
            (wg_hbm, wgu_v.at[pl.ds(0, F)]), (wu_hbm, wgu_v.at[pl.ds(F, F)]),
            (wd_hbm, wd_v), (wr_hbm, wr_v)))]

    x_copies = [pltpu.make_async_copy(x_hbm.at[rows(i)], x_v.at[rows(i)], sem_x.at[i])
                for i in range(nb)]
    ckv_groups = ((0,), (1, 2), (3, 4, 5), (6, 7))
    ckv_copies = [
        pltpu.make_async_copy(ckv_hbm.at[pl.ds(g[0] * BQ, len(g) * BQ)],
                              ckv_v.at[pl.ds(g[0] * BQ, len(g) * BQ)], sem_c.at[n])
        for n, g in enumerate(ckv_groups)]

    def start(copies):
        for copy in copies:
            copy.start()

    def wait(copies):
        for copy in copies:
            copy.wait()

    def select_both(k, rs):
        for r in rs:
            rows_v[r:r + 8, :], rows_v[r + 8:r + 16, :] = pair_rows(k, 0, r)
            both = rows_v[r:r + 8, :], rows_v[r + 8:r + 16, :]
            for parity, name in enumerate(("W" + k, "W" + k + "2")):
                w[pl.ds(_OFF[name] + r // 2, 8), :] = _select_head(*both, parity)

    def project(name, i, base=0):
        ckv = jnp.concatenate(
            [w[pl.ds(base + (_OFF["C"] + (j * S + i * BQ) // 2), BQ // 2), :]
             for j in range(CT)], axis=1)
        put(name.upper(), i, _pack(_nn(pltpu.bitcast(ckv, BF), weight(name, C))))

    def take_ckv(n):
        for i in ckv_groups[n]:
            put("C", i, pltpu.bitcast(ckv_v[rows(i), :], F32))
        return [(name, i) for name in ("k", "k2", "v", "v2") for i in ckv_groups[n]]

    wq_copy, wk_copy, wv_copy = pair_copies(0)
    start([wk_copy, ckv_copies[0], wv_copy])
    w[_OFF["D"]:_OFF["D"] + T, :] = (
        lax.broadcasted_iota(I32, (T, T), 1) - lax.broadcasted_iota(I32, (T, T), 0)).astype(F32)
    w[_OFF["R"]:_OFF["R"] + 32, :] = jnp.zeros((32, T), F32)
    wk_copy.wait()
    ckv_copies[1].start()
    select_both("k", range(0, C, 16))
    origin = pl.multiple_of(pltpu.bitcast(w[_OFF["R"]:_OFF["R"] + 8, :], I32)[0, 0], 16)
    wait([ckv_copies[0], wv_copy])
    start([wq_copy, ckv_copies[2], c_copy])
    select_both("v", range(0, C, 16))
    for unit in take_ckv(0):
        project(*unit)
    ckv_copies[1].wait()
    start(mod_copies[:2])
    for unit in take_ckv(1):
        project(*unit)
    wait([ckv_copies[2], c_copy])
    start(x_copies[:2])
    for unit in take_ckv(2):
        project(*unit)
    c = jnp.broadcast_to(c_v[...].astype(F32), (16, M))
    silu_c = (c * jax.nn.sigmoid(c)).astype(BF)
    silu_v[...] = jnp.concatenate([silu_c.astype(F32)] * (T // 16), axis=0).T
    wait(mod_copies[:2] + [wq_copy])
    start([ckv_copies[3], x_copies[2]])
    shift_a = _rnd(_nn(silu_c, wmod_v[0])[:1])
    scale_a = _rnd(1.0 + _rnd(_nn(silu_c, wmod_v[1])[:1]))
    select_both("q", range(0, M, 16))

    needed = [x_copies[:1], x_copies[1:2], [x_copies[2], ckv_copies[3]], x_copies[3:4],
              x_copies[4:6], [], x_copies[6:], []]
    more = [x_copies[3:4], x_copies[4:5], x_copies[5:7], [x_copies[7]] + pair_copies(1),
            [wo_first], [], [], []]
    for i in range(nb):
        wait(needed[i])
        start(more[i])
        if i == 2:
            todo = take_ckv(3)
        if i in (2, 3):
            project(*todo[i - 2])
        if i >= 2:
            project(*todo[i])
        x = x_v[rows(i), :].astype(F32)
        xc = x - jnp.mean(x, axis=1, keepdims=True)
        var = jnp.mean(xc * xc, axis=1, keepdims=True)
        h = _pack(xc * lax.rsqrt(var + EPS) * scale_a + shift_a)
        put("H", i, h)
        h, wq = pltpu.bitcast(h, BF), weight("q", M)
        q = _nn(h[:, :4 * T], wq[:4 * T])
        q += jnp.concatenate([_nn(h[t:t + BQ // 4, 4 * T:], wq[4 * T:])
                              for t in range(0, BQ, BQ // 4)], axis=0)
        put("Q", i, _pack(q * QSCALE))
    wait([wo_first] + pair_copies(1))
    start([wo_next, wg_copy])

    _head(_SEQ_FIRST, w, origin, wo_v.at[0], assign=True, next_weights=weights_of(2))

    wait([wo_next, wg_copy])
    start(mod_copies[2:] + [wu_copy])

    def head_step(h, carry):
        pl.when(h == 2 * MT)(lambda: wait(mod_copies[2:] + [wo_rest, wu_copy]))

        pl.when(jnp.logical_and((h & 1) == 1, h + 1 < H))(
            lambda: wait(pair_copies((h >> 1) + 1)))
        pl.when(h == 3)(lambda: start([wo_rest, wd_copy, wr_copy]))
        pl.when(jnp.logical_and((h & 1) == 0, h + 2 < H))(
            lambda: start(pair_copies((h >> 1) + 1)))

        pad = pl.ds(_OFF["PAD"], 8)

        def modulation(k):
            lanes = pl.ds(pl.multiple_of(lax.rem(h - 2, MT) * T, T), T)
            tile = wmod_v[lax.div(h - 2, MT), pl.ds(k * T, T), lanes].astype(F32)
            part = jnp.sum(silu_v[pl.ds(k * T, T), :] * tile, axis=0, keepdims=True)
            total = jnp.broadcast_to(part, (8, T)) + (w[pad, :] if k else 0.0)
            w[pad, :] = total
            if k == MT - 1:
                mod_v[h - 2] = total

        def transpose():
            n = jnp.minimum(h - 2, 2 * F // T - 1)
            wgu_t[n] = pltpu.bitcast(wgu_v[pl.ds(pl.multiple_of(n * T, T), T), :].T, F32)
            w[pad, :] = wgu_t[n + origin, :8, :]

        extras = [(T * (k + 1), lambda k=k: modulation(k)) for k in range(MT)]
        _head(_SEQ, w, origin, wo_v.at[h], next_weights=weights_of(h + 1),
              extras=extras + [(5 * BQ, transpose)])
        return carry

    assert H - 2 == 6 * MT >= 2 * F // T
    lax.fori_loop(2, H, head_step, 0)

    wait([wd_copy, wr_copy])
    vectors = ("gate_a", "shift_b", "scale_b", "gate_b", "route", "gain", "bias")

    def set_vector(name, v):
        for j in range(MT):
            a = _OFF["MOD"] + (vectors.index(name) * MT + j) * 8
            w[a:a + 8, :] = v[:, j * T:(j + 1) * T]

    def vector(name, n, tiles=range(MT)):
        a = _OFF["MOD"] + vectors.index(name) * MT * 8
        return [jnp.concatenate([w[a + 8 * j:a + 8 * j + 8, :]] * (n // 8), axis=0)
                for j in tiles]

    mod = _rnd(jnp.concatenate([mod_v[j] for j in range(2 * MT, 6 * MT)], axis=1))
    shift_b, scale_b, gate_b = mod[:, M:2 * M], _rnd(1.0 + mod[:, 2 * M:3 * M]), mod[:, 3 * M:]
    w_r = jnp.broadcast_to(wr_v[...].astype(F32).reshape(1, M), (8, M))
    for name, v in zip(vectors, (mod[:, :M], shift_b, scale_b, gate_b, scale_b * w_r,
                                 gate_b * scale_b, gate_b * shift_b)):
        set_vector(name, v)
    out_copies = [pltpu.make_async_copy(out_v.at[rows(i)], out_hbm.at[rows(i)], sem_out.at[i])
                  for i in range(nb)]

    def residual(j, r, attn):
        gate, = vector("gate_a", CH, [j])
        return x_v[r:r + CH, j * T:(j + 1) * T].astype(F32) + gate * attn

    def finalize(r):
        x1_at = [pl.ds(_OFF["O"] + j * S + r, FR) for j in range(MT)]
        mean_at, inv_at = pl.ds(_OFF["MX"] + r, FR), pl.ds(_OFF["M"] + r, FR)

        def keep_mean():
            w[mean_at, :] = _row_sum([w[a, :] for a in x1_at]) * (1.0 / M)

        def keep_moments():
            mean = w[mean_at, :]
            centred = [w[a, :] - mean for a in x1_at]
            var = _row_sum([d * d for d in centred]) * (1.0 / M)
            dot = _row_sum([d * v for d, v in zip(centred, vector("route", FR))])
            w[inv_at, :] = lax.rsqrt(var + EPS)
            lane = lax.broadcasted_iota(I32, (8, T), 1)
            for n, v in enumerate((var, dot)):
                at = pl.ds(_OFF["R"] + 16 * n + r // (8 * T) * 8, 8)
                tile = w[at, :]
                for t in range(0, FR, 8):
                    tile = jnp.where(lane == (r + t) // 8 % T, v[t:t + 8], tile)
                w[at, :] = tile

        def output():
            mean, inv_std = w[mean_at, :], w[inv_at, :]
            out = [(w[a, :] - mean) * inv_std * g + (w[a, :] + b)
                   for a, g, b in zip(x1_at, vector("gain", FR), vector("bias", FR))]
            out_v[r:r + FR, :] = jnp.concatenate(out, axis=1).astype(BF)
            if r < S - 2 * BQ:
                w[pl.ds(_OFF["PAD"], 8), :] = pltpu.bitcast(
                    out_v[pl.ds(origin + r, 16), :T], F32)
            if (r + FR) % BQ == 0:
                out_copies[r // BQ].start()

        return [(_FIN_LAG, keep_mean), (2 * _FIN_LAG + 64, keep_moments),
                (2 * _FIN_LAG + 128, output)]

    _head(_SEQ_LAST, w, origin, wo_v.at[1], residual=residual, finalize=finalize,
          suffix="2")

    var, dot = w[_OFF["R"]:_OFF["R"] + 16, :], w[_OFF["R"] + 16:_OFF["R"] + 32, :]
    offset = jnp.sum((shift_b * w_r)[:1], axis=1, keepdims=True)
    score = _rnd(dot / _rnd(jnp.sqrt(_rnd(_rnd(var) + EPS))) + offset)
    bits = pltpu.bitcast(jnp.where(score == 0.0, 0.0, score), I32) >> 16
    rank = jnp.where(bits < 0, -1 - bits, bits + 0x8000)
    rank = jnp.where(score != score, 0, rank)
    sub = lax.broadcasted_iota(I32, (16, T), 0)
    row = (sub >> 3) * (8 * T) + 8 * lax.broadcasted_iota(I32, (16, T), 1) + (sub & 7)
    key = pltpu.bitcast((rank << 11) | (S - 1 - row) | (1 << 29), F32)
    best = jnp.broadcast_to(jnp.max(key, axis=0, keepdims=True), (T, T))
    place = jnp.sum(jnp.where(best.T > best, 1.0, 0.0), axis=0, keepdims=True)
    chosen = place == lax.broadcasted_iota(I32, (TOPK, T), 0).astype(F32)
    key = jnp.concatenate([jnp.where(chosen, key[n:n + 1], 0.0) for n in range(16)], axis=0)
    key = jnp.broadcast_to(jnp.max(key, axis=1, keepdims=True), key.shape)
    picked = []
    for _ in range(TOPK):
        top = jnp.max(key, axis=0, keepdims=True)
        key = jnp.where(key == top, 0.0, key)
        top = pltpu.bitcast(jnp.broadcast_to(top, (8, T)), I32)
        picked.append(S - 1 - (top[0, 0] & (S - 1)))

    wait(out_copies[:-2])

    def gather(at):
        return jnp.concatenate([w[pl.ds(at + r, 1), :] for r in picked], axis=0)

    x1 = [gather(_OFF["O"] + j * S) for j in range(MT)]
    mean, inv_std = gather(_OFF["MX"]), gather(_OFF["M"])
    h2 = [_rnd((t - mean) * inv_std * a + b)
          for t, a, b in zip(x1, vector("scale_b", 8), vector("shift_b", 8))]
    x1, h2 = jnp.concatenate(x1, axis=1), jnp.concatenate(h2, axis=1)
    r_sel = jnp.sum(h2 * w_r, axis=1, keepdims=True)
    gu = _rnd(jnp.concatenate([_nn(h2.astype(BF), pltpu.bitcast(wgu_t[j], BF))
                               for j in range(2 * F // T)], axis=1))
    g, u = gu[:, :F], gu[:, F:]
    y = _nn((_rnd(g * jax.nn.sigmoid(g)) * u).astype(BF), wd_v[...])
    new = x1 + jnp.concatenate(vector("gate_b", 8), axis=1) * (h2 + y * jax.nn.sigmoid(r_sel))

    wait(out_copies[-2:])
    groups = [pl.ds(pl.multiple_of((r >> 4) << 4, 16), 16) for r in picked]
    line = lax.broadcasted_iota(I32, (16, M), 0)
    for n, r in enumerate(picked):
        old = out_v[groups[n], :].astype(F32)
        out_v[groups[n], :] = jnp.where(line == (r & 15), new[n:n + 1], old).astype(BF)

    fixes = []
    for n, r in enumerate(picked):
        fresh = True
        for earlier in picked[:n]:
            fresh = jnp.logical_and(fresh, (earlier >> 4) != (r >> 4))
        fixes.append((fresh, pltpu.make_async_copy(
            out_v.at[groups[n]], out_hbm.at[groups[n]], sem_fix.at[n])))
    for fresh, copy in fixes:
        pl.when(fresh)(copy.start)
    for fresh, copy in fixes:
        pl.when(fresh)(copy.wait)


@jax.jit
def pallas_adaLN_cond__compressed_kv_cla__moe_arch_mod__prompt_kernel(
    A_x: jax.Array,
    A_c_kv: jax.Array,
    A_w_q: jax.Array,
    A_w_uk: jax.Array,
    A_w_uv: jax.Array,
    A_w_o: jax.Array,
    B_x: jax.Array,
    B_w_r: jax.Array,
    B_w_gate: jax.Array,
    B_w_up: jax.Array,
    B_w_down: jax.Array,
    c: jax.Array,
    w_mod: jax.Array,
):
    del B_x
    assert A_x.shape == (1, S, M) and A_c_kv.shape == (1, S, C)
    assert A_w_q.shape == (M, H, D) and B_w_gate.shape == (M, F)
    dma = pltpu.SemaphoreType.DMA
    out = pl.pallas_call(
        _kernel,
        in_specs=[pl.BlockSpec(memory_space=pl.ANY)] * 12,
        out_specs=pl.BlockSpec(memory_space=pl.ANY),
        out_shape=jax.ShapeDtypeStruct((S, M), BF),
        scratch_shapes=[
            pltpu.VMEM((_ROWS, T), F32),
            pltpu.VMEM((S, M), BF), pltpu.VMEM((S, C), BF),
            pltpu.VMEM((2, M // 2, 2, 2, D), BF), pltpu.VMEM((2, C // 2, 2, 2, D), BF),
            pltpu.VMEM((2, C // 2, 2, 2, D), BF), pltpu.VMEM((H, D, M), BF),
            pltpu.VMEM((M,), BF),
            pltpu.VMEM((2 * F, M), BF), pltpu.VMEM((2 * F // T, M // 2, T), F32),
            pltpu.VMEM((F, M), BF),
            pltpu.VMEM((1, M), BF),
            pltpu.VMEM((6, M, M), BF), pltpu.VMEM((M, T), F32), pltpu.VMEM((6 * MT, 8, T), F32),
            pltpu.VMEM((M, T), U32),
            pltpu.VMEM((S, M), BF),
            dma((11,)), dma((S // BQ,)), dma((S // BQ // 2,)), dma((6,)), dma((3,)),
            dma((S // BQ,)), dma((TOPK,)),
        ],
        compiler_params=pltpu.CompilerParams(vmem_limit_bytes=100 * 2 ** 20),
        name="adaln_attn_moe",
    )(A_x[0], A_c_kv[0], A_w_q.reshape(M // 2, 2, H, D), A_w_uk.reshape(C // 2, 2, H, D),
      A_w_uv.reshape(C // 2, 2, H, D), A_w_o, B_w_r,
      B_w_gate.T, B_w_up.T, B_w_down, c, w_mod)
    return out[None]
```

```python
import jax
import jax.numpy as jnp
from jax import lax
import jax.experimental.pallas as pl
import jax.experimental.pallas.tpu as pltpu

BF = jnp.bfloat16
F32 = jnp.float32
I32 = jnp.int32
U32 = jnp.uint32

S = 2048
M = 640
C = 512
H = 32
D = 128
F = 1728
TOPK = 8
EPS = 1e-5
LOG2E = 1.4426950408889634
QSCALE = D ** -0.5 * LOG2E
MASKED = -1e9 * LOG2E

T = 128
BQ = 256
CH = 64
MT = M // T
CT = C // T

_OFF = {}
_ROWS = 0
for _name, _n in (
    ("H", MT * S // 2), ("C", CT * S // 2),
    ("Q", S // 2), ("K", S // 2), ("V", S // 2), ("X", S // 2),
    ("Wq", M // 2), ("Wk", C // 2), ("Wv", C // 2),
    ("Q2", S // 2), ("K2", S // 2), ("V2", S // 2), ("Wq2", M // 2), ("Wk2", C // 2), ("Wv2", C // 2),
    ("S", (S // BQ) ** 2 * BQ), ("SD", S // 2),
    ("MX", S), ("M", S), ("L", S), ("ACC", 3 * BQ), ("PA", S),
    ("O", MT * S), ("D", T), ("R", 32), ("PAD", 8), ("MOD", 7 * MT * 8),
):
    _OFF[_name] = _ROWS
    _ROWS += _n

_SEQ = (
    "q0 k0 q1 k1 q2 v0 A0+A1 A0 q3 q4 B0 A1 k2 v1 q5 B1 A2 B0+A2 q6 q7 v2 k3 "
    "B2 A3 B1+A3 v3 k4 k5 k6 k7 B3 A4 B2+A4 v4 v5 v6 v7 B4 A5 B3+A5 o0 o1 "
    "B5 A6 B4+A6 o2 o3 B6 A7 B5+A7 o4 o5 B6+B7 B7 o6 o7"
)
_SEQ_FIRST = (
    "A0+A1 A0 A1 A2+A3 A2 A3 B0+B1 B0 B1 A4+A5 A4 B2+B3 B2 B3 o0 o1 A5 A6+A7 A6 "
    "B4+B5 B4 B5 o2 o3 A7 o4 o5 B6+B7 B6 B7 o6 o7"
)
_SEQ_LAST = (
    "A0+A1 A0 A1 A2+A3 A2 q4 B0+B1 B0 B1 A3 o0 o1 B2 B2+A4 q5 o2 B3+A5 B3 "
    "A4 q6 o3 B4+A6 B4 A5 q7 o4 B5+A7 B5 A6 o5 A7 B6 B6+B7 B7 o6 o7"
)
_RES_LAG, _CTX_LAG, _MAX_LAG, _SUM_LAG = 208, 208, 192, 80
FR = 16
_FIN_STEP, _FIN_LAG = (64, 128), 192


def _slots(seq):
    lanes = []
    for word in seq.split():
        if "+" in word:
            lanes.append(tuple(
                (p[0], int(p[1:]), 2 * int(p[1:]) + 1, T) for p in word.split("+")))
        else:
            k, i = word[0], int(word[1:])
            n = {"q": MT, "k": CT, "v": CT, "o": MT, "A": 2 * i + 1, "B": 2 * i + 1}[k]
            lanes += [((k, i, j, 0),) for j in range(n)]
    assert len(lanes) % 4 == 0
    return [lanes[s:s + 4] for s in range(0, len(lanes), 4)]


def _nt(a, b):
    return lax.dot_general(a, b, (((1,), (1,)), ((), ())), preferred_element_type=F32)


def _nn(a, b):
    return jnp.dot(a, b, preferred_element_type=F32)


def _rnd(x):
    if x.shape[1] == T and x.shape[0] % 16 == 0:
        half = x.shape[0] // 2
        y = _rnd(jnp.concatenate([x[:half], x[half:]], axis=1))
        return jnp.concatenate([y[:, :T], y[:, T:]], axis=0)
    return x.astype(BF).astype(F32)


def _pack(x):
    return pltpu.bitcast(x.astype(BF), F32)


def _select_head(even, odd, parity):
    down = jnp.asarray(16 * parity, U32)
    return pltpu.bitcast(((even >> down) & 0xFFFF) | ((odd >> down) << 16), F32)


def _head(seq, w, zero, wo, *, assign=False, next_weights=None, residual=None,
          finalize=None, extras=(), suffix=""):
    def load(r, n):
        return w[r:r + n, :]

    def ordered(r, n):
        head = w[pl.ds(zero + r, 8), :]
        return head if n == 8 else jnp.concatenate([head, load(r + 8, n - 8)], axis=0)

    def store(r, v):
        w[r:r + v.shape[0], :] = v

    def s_row(i, j, t, half):
        if half:
            return _OFF["SD"] + i * T + t - T
        return _OFF["S"] + (i * i + j) * BQ + t

    events = []

    def at(time, rank, fn):
        events.append((time, rank, len(events), fn))

    slots = _slots(seq)
    left = {}
    for slot in slots:
        for lane in slot:
            for k, i, _, t0 in lane:
                for t in range(t0, BQ, CH):
                    left[k, i, t] = left.get((k, i, t), 0) + 1
    has_sum, has_acc, last_use, complete = set(), set(), {}, {}
    pending = {}

    def expect(*tag):
        pending[tag] = pending.get(tag, 0) + 1

    def settled(*tag):
        assert not pending.get(tag), tag

    for s, slot in enumerate(slots):
        base = BQ * s
        jobs = ([(lane[0], -T) for lane in slot if len(lane) == 2]
                + [(lane[0], 0) for lane in slot if len(lane) == 1]
                + [(lane[1], 0) for lane in slot if len(lane) == 2])
        lhs, res, groups = {}, {}, {}
        for job, shift in jobs:
            groups.setdefault((job[0], job[1], shift), []).append(job)
            last_use[job[0]] = base + BQ

        for (k, i, shift), group in groups.items():
            for t in range(0, BQ, CH):
                live = [job for job in group if t >= job[3]]
                if not live:
                    continue

                def fetch(k=k, i=i, t=t, live=live, lhs=lhs, first=(i, t) not in has_sum):
                    r = i * BQ + t
                    if k in "qkv":
                        src = _OFF["H" if k == "q" else "C"] + r // 2
                        for job in live:
                            get = ordered if job == live[0] else load
                            lhs[job, t] = get(src + job[2] * S // 2, CH // 2)
                    elif k in "Ao":
                        settled("q" if k == "A" else "B", i, t)
                        v = ordered(_OFF["Q" + suffix if k == "A" else "X"] + r // 2, CH // 2)
                        for job in live:
                            lhs[job, t] = v
                            if k == "A" and job[2] == 2 * i + t // T:
                                lhs["d", job, t] = ordered(_OFF["D"] + t % T, 8)
                    else:
                        settled("A", i, t)
                        settled("m", i, t)
                        settled("l", i, t)
                        expect("l", i, t)
                        m = ordered(_OFF["M"] + r, CH)
                        l = None if first else load(_OFF["L"] + r, CH)
                        for job in live:
                            p = jnp.exp2(load(s_row(i, job[2], t, job[3]), CH) - m)
                            l = p if l is None else l + p
                            lhs[job, t] = p
                        lhs["l", i, t] = l

                at(base + shift + t, 1, fetch)
                if k == "B":
                    has_sum.add((i, t))

                    def keep_sum(i=i, t=t, lhs=lhs):
                        pending["l", i, t] -= 1
                        store(_OFF["L"] + i * BQ + t, lhs["l", i, t])

                    at(base + shift + t + CH - 16 + _SUM_LAG, 0, keep_sum)

        for job, shift in jobs:
            def matmul(job=job, lhs=lhs, res=res):
                k, _, j, t0 = job
                a = jnp.concatenate([lhs[job, t] for t in range(t0, BQ, CH)], axis=0)
                a = a.astype(BF) if k == "B" else pltpu.bitcast(a, BF)
                if k == "o":
                    res[job] = _nn(a, wo[:, j * T:(j + 1) * T])
                    return
                region = {"A": "K", "B": "V"}.get(k, "W" + k)
                if k in "AB":
                    settled(region.lower(), j // 2, (j % 2) * T + T - CH)
                b = pltpu.bitcast(load(_OFF[region + suffix] + j * T // 2, T // 2), BF)
                res[job] = _nt(a, b) if k == "A" else _nn(a, b)

            at(base + shift + BQ - CH, 2, matmul)

        for (k, i, shift), group in groups.items():
            for t in range(0, BQ, CH):
                live = [job for job in group if t >= job[3]]
                if not live:
                    continue
                first = (k, i, t) not in has_acc
                has_acc.add((k, i, t))
                left[k, i, t] -= len(live)
                last = left[k, i, t] == 0

                def finish(k=k, i=i, t=t, live=live, lhs=lhs, res=res, first=first, last=last):
                    r = i * BQ + t
                    pending[k, i, t] -= 1
                    assert k == "o" or last == (pending[k, i, t] == 0), (k, i, t)
                    parts = [res[job][t - job[3]:t - job[3] + CH] for job in live]
                    if k == "o":
                        for job, v in zip(live, parts):
                            a = _OFF["O"] + job[2] * S + r
                            v = v if assign else load(a, CH) + v
                            store(a, residual(job[2], r, v) if residual else v)
                    elif k == "A":
                        mx = None if first else load(_OFF["MX"] + r, CH)
                        for job, v in zip(live, parts):
                            if job[2] == 2 * i + t // T:
                                d = lhs["d", job, t]
                                v = jnp.concatenate(
                                    [jnp.where(d <= u, v[u:u + 8], MASKED)
                                     for u in range(0, CH, 8)], axis=0)
                            store(s_row(i, job[2], t, job[3]), v)
                            mx = v if mx is None else jnp.maximum(mx, v)
                        if last:
                            res["m", i, t] = jnp.broadcast_to(
                                jnp.max(mx, axis=1, keepdims=True), (CH, T))
                        else:
                            store(_OFF["MX"] + r, mx)
                    else:
                        a = _OFF["PA"] + r if k == "B" else _OFF["ACC"] + "qkv".index(k) * BQ + t
                        acc = None if first else load(a, CH)
                        for v in parts:
                            acc = v if acc is None else acc + v
                        if not last:
                            store(a, acc)
                        elif k == "B":
                            settled("l", i, t)
                            l = jnp.sum(load(_OFF["L"] + r, CH), axis=1, keepdims=True)
                            store(_OFF["X"] + r // 2, _pack(acc * (1.0 / l)))
                        elif k == "q":
                            store(_OFF["Q" + suffix] + r // 2, _pack(acc * QSCALE))
                        else:
                            store(_OFF[k.upper() + suffix] + r // 2, _pack(acc))

                ready = base + shift + t + CH - 16 + (_CTX_LAG if k == "B" and last else _RES_LAG)
                when = max(base + shift + BQ, ready)
                expect(k, i, t)
                at(when, 0, finish)
                if k == "o" and last:
                    complete[i * BQ + t] = when
                if k == "A" and last:
                    def keep_max(i=i, t=t, res=res):
                        pending["m", i, t] -= 1
                        store(_OFF["M"] + i * BQ + t, res["m", i, t])

                    expect("m", i, t)
                    at(max(when, ready + _MAX_LAG), 0, keep_max)

    busy = [any(job[0] == "B" for s2 in (max(s - 1, 0), s) for lane in slots[s2] for job in lane)
            for s in range(len(slots))]
    if next_weights:
        todo = [(k, r) for k, n in (("q", M), ("k", C), ("v", C)) for r in range(0, n, 16)]
        calm = [s for s in range(last_use.get("q", 0) // BQ, len(slots) - 2) if not busy[s]]
        for n, (k, r) in enumerate(todo):
            step = BQ * len(calm) * n // len(todo)
            time = BQ * calm[step // BQ] + step % BQ
            assert time >= last_use.get(k, 0)
            at(time, 0, lambda k=k, r=r: next_weights(k, r))
    for time, fn in extras:
        at(time, 0, fn)
    if finalize:
        time = 0
        for r in range(0, S, FR):
            heavy = time // BQ < len(slots) and busy[time // BQ]
            time = max(time + _FIN_STEP[heavy], complete[r // CH * CH])
            for delay, fn in finalize(r):
                at(time + delay, 0, fn)

    for event in sorted(events, key=lambda e: e[:3]):
        event[3]()


def _row_sum(tiles):
    total = tiles[0]
    for tile in tiles[1:]:
        total = total + tile
    return jnp.broadcast_to(jnp.sum(total, axis=1, keepdims=True), total.shape)


def _kernel(x_hbm, ckv_hbm, wq_hbm, wk_hbm, wv_hbm, wo_hbm, wr_hbm, wg_hbm, wu_hbm,
            wd_hbm, c_hbm, wmod_hbm, out_hbm,
            w, x_v, ckv_v, wq_v, wk_v, wv_v, wo_v, wr_v, wgu_v, wgu_t, wd_v, c_v,
            wmod_v, silu_v, mod_v, rows_v, out_v, sem_a, sem_b, sem_m, sem_w):
    pairs = {"q": wq_v, "k": wk_v, "v": wv_v}
    nb = S // BQ

    def rows(i):
        return pl.ds(i * BQ, BQ)

    def pair_copies(p):
        return [pltpu.make_async_copy(src.at[:, :, pl.ds(2 * p, 2), :], dst.at[p],
                                      sem_w.at[n])
                for n, (src, dst) in enumerate(((wq_hbm, wq_v), (wk_hbm, wk_v), (wv_hbm, wv_v)))]

    def later_pairs_wait():
        for n, dst in enumerate((wq_v, wk_v, wv_v)):
            rest = dst.at[pl.ds(3, H // 2 - 3)]
            pltpu.make_async_copy(rest, rest, sem_w.at[n]).wait()

    def pair_rows(k, slot, r):
        return [pltpu.bitcast(pairs[k][slot, r // 2:r // 2 + 8, odd], U32).reshape(8, T)
                for odd in range(2)]

    def weights_of(h):
        def select(k, r):
            a = _OFF["W" + k] + r // 2
            w[a:a + 8, :] = _select_head(*pair_rows(k, h >> 1, r), h & 1)
        return select

    def weight(k, n):
        return pltpu.bitcast(w[_OFF["W" + k]:_OFF["W" + k] + n // 2, :], BF)

    def put(region, i, v):
        for j in range(v.shape[1] // T):
            a = _OFF[region] + (j * S + i * BQ) // 2
            w[a:a + v.shape[0], :] = v[:, j * T:(j + 1) * T]

    c_copy = pltpu.make_async_copy(c_hbm, c_v, sem_m.at[2])
    mod_copies = [pltpu.make_async_copy(wmod_hbm.at[:, pl.ds(n * M, M)], wmod_v.at[n],
                                        (sem_m if n < 2 else sem_a).at[n]) for n in range(6)]
    wo_first, wo_next, wo_rest = [
        pltpu.make_async_copy(wo_hbm.at[heads], wo_v.at[heads], sem) for heads, sem in (
            (pl.ds(0, 1), sem_b.at[0]), (pl.ds(1, 4), sem_b.at[1]), (pl.ds(5, H - 5), sem_b.at[2]))]
    wg_copy = pltpu.make_async_copy(wg_hbm, wgu_v.at[pl.ds(0, F)], sem_b.at[3])
    wu_copy = pltpu.make_async_copy(wu_hbm, wgu_v.at[pl.ds(F, F)], sem_a.at[0])
    wd_copy = pltpu.make_async_copy(wd_hbm, wd_v, sem_a.at[1])
    wr_copy = pltpu.make_async_copy(wr_hbm, wr_v, sem_a.at[6])
    x_copies = [pltpu.make_async_copy(x_hbm.at[rows(i)], x_v.at[rows(i)], sem_a.at[i])
                for i in range(nb)]
    ckv_groups = ((0,), (1, 2), (3, 4, 5), (6, 7))
    ckv_copies = [
        pltpu.make_async_copy(ckv_hbm.at[pl.ds(g[0] * BQ, len(g) * BQ)],
                              ckv_v.at[pl.ds(g[0] * BQ, len(g) * BQ)], sem_b.at[n])
        for n, g in enumerate(ckv_groups)]

    def start(copies):
        for copy in copies:
            copy.start()

    def wait(copies):
        for copy in copies:
            copy.wait()

    def select_both(k, rs):
        for r in rs:
            rows_v[r:r + 8, :], rows_v[r + 8:r + 16, :] = pair_rows(k, 0, r)
            both = rows_v[r:r + 8, :], rows_v[r + 8:r + 16, :]
            for parity, name in enumerate(("W" + k, "W" + k + "2")):
                w[pl.ds(_OFF[name] + r // 2, 8), :] = _select_head(*both, parity)

    def project(name, i, src=None):
        region, n = ("H", M) if name[0] == "q" else ("C", C)
        if src is None:
            src = jnp.concatenate([w[pl.ds(_OFF[region] + (j * S + i * BQ) // 2, BQ // 2), :]
                                   for j in range(n // T)], axis=1)
        a, b = pltpu.bitcast(src, BF), weight(name, n)
        out = _nn(a[:, :4 * T], b[:4 * T])
        if name[0] == "q":
            out += jnp.concatenate([_nn(a[t:t + BQ // 4, 4 * T:], b[4 * T:])
                                    for t in range(0, BQ, BQ // 4)], axis=0)
            out *= QSCALE
        put(name.upper(), i, _pack(out))

    def take_ckv(n):
        for i in ckv_groups[n]:
            put("C", i, pltpu.bitcast(ckv_v[rows(i), :], F32))
        return [(name, i) for name in ("k", "k2", "v", "v2") for i in ckv_groups[n]]

    wq_copy, wk_copy, wv_copy = pair_copies(0)
    start([wk_copy, ckv_copies[0], wv_copy])
    w[_OFF["D"]:_OFF["D"] + T, :] = (
        lax.broadcasted_iota(I32, (T, T), 1) - lax.broadcasted_iota(I32, (T, T), 0)).astype(F32)
    w[_OFF["R"]:_OFF["R"] + 32, :] = jnp.zeros((32, T), F32)
    wk_copy.wait()
    ckv_copies[1].start()
    select_both("k", range(0, C, 16))
    origin = pl.multiple_of(pltpu.bitcast(w[_OFF["R"]:_OFF["R"] + 8, :], I32)[0, 0], 16)
    wait([ckv_copies[0], wv_copy])
    start([wq_copy, ckv_copies[2], c_copy])
    select_both("v", range(0, C, 16))
    for unit in take_ckv(0):
        project(*unit)
    ckv_copies[1].wait()
    start(mod_copies[:2])
    for unit in take_ckv(1):
        project(*unit)
    wait([ckv_copies[2], c_copy])
    start(x_copies[:2])
    for unit in take_ckv(2):
        project(*unit)
    c = jnp.broadcast_to(c_v[...].astype(F32), (16, M))
    silu_c = (c * jax.nn.sigmoid(c)).astype(BF)
    silu_v[...] = jnp.concatenate([silu_c.astype(F32)] * (T // 16), axis=0).T
    wait(mod_copies[:2] + [wq_copy])
    start([ckv_copies[3], x_copies[2]])
    shift_a = _rnd(_nn(silu_c, wmod_v[0])[:1])
    scale_a = _rnd(1.0 + _rnd(_nn(silu_c, wmod_v[1])[:1]))
    select_both("q", range(0, M, 16))

    needed = [x_copies[:1], x_copies[1:2], [x_copies[2], ckv_copies[3]], x_copies[3:4],
              x_copies[4:6], [], x_copies[6:], []]
    more = [x_copies[3:4], x_copies[4:5], x_copies[5:7], [x_copies[7]] + pair_copies(1),
            [wo_first], [], [], []]
    for i in range(nb):
        wait(needed[i])
        start(more[i])
        if i == 2:
            todo = take_ckv(3)
        if i in (2, 3):
            project(*todo[i - 2])
        if i >= 2:
            project(*todo[i])
        if i in (1, 4, 5, 6):
            project("q2", (1, 4, 5, 6).index(i))
        x = x_v[rows(i), :].astype(F32)
        xc = x - jnp.mean(x, axis=1, keepdims=True)
        var = jnp.mean(xc * xc, axis=1, keepdims=True)
        h = _pack(xc * lax.rsqrt(var + EPS) * scale_a + shift_a)
        put("H", i, h)
        project("q", i, h)
    wait([wo_first] + pair_copies(1))
    start(pair_copies(2) + [wo_next, wg_copy])

    _head(_SEQ_FIRST, w, origin, wo_v.at[0], assign=True, next_weights=weights_of(2))

    wait(pair_copies(2) + [wo_next, wg_copy])
    for p in range(3, H // 2):
        start(pair_copies(p))
    start(mod_copies[2:] + [wo_rest, wu_copy, wd_copy, wr_copy])

    def head_step(h, carry):
        @pl.when(h == 5)
        def _():
            later_pairs_wait()
            wait(mod_copies[2:] + [wo_rest, wu_copy])

        pad = pl.ds(_OFF["PAD"], 8)

        def modulation(k):
            lanes = pl.ds(pl.multiple_of(lax.rem(h - 2, MT) * T, T), T)
            tile = wmod_v[lax.div(h - 2, MT), pl.ds(k * T, T), lanes].astype(F32)
            part = jnp.sum(silu_v[pl.ds(k * T, T), :] * tile, axis=0, keepdims=True)
            total = jnp.broadcast_to(part, (8, T)) + (w[pad, :] if k else 0.0)
            w[pad, :] = total
            if k == MT - 1:
                mod_v[h - 2] = total

        def transpose():
            n = jnp.minimum(h - 2, 2 * F // T - 1)
            wgu_t[n] = pltpu.bitcast(wgu_v[pl.ds(pl.multiple_of(n * T, T), T), :].T, F32)
            w[pad, :] = wgu_t[n + origin, :8, :]

        extras = [(T * (k + 1), lambda k=k: modulation(k)) for k in range(MT)]
        _head(_SEQ, w, origin, wo_v.at[h], next_weights=weights_of(jnp.minimum(h + 1, H - 1)),
              extras=extras + [(5 * BQ, transpose)])
        return carry

    assert H - 2 == 6 * MT >= 2 * F // T
    lax.fori_loop(2, H, head_step, 0)

    wait([wd_copy, wr_copy])
    vectors = ("gate_a", "shift_b", "scale_b", "gate_b", "route", "gain", "bias")

    def set_vector(name, v):
        for j in range(MT):
            a = _OFF["MOD"] + (vectors.index(name) * MT + j) * 8
            w[a:a + 8, :] = v[:, j * T:(j + 1) * T]

    def vector(name, n, tiles=range(MT)):
        a = _OFF["MOD"] + vectors.index(name) * MT * 8
        return [jnp.concatenate([w[a + 8 * j:a + 8 * j + 8, :]] * (n // 8), axis=0)
                for j in tiles]

    mod = _rnd(jnp.concatenate([mod_v[j] for j in range(2 * MT, 6 * MT)], axis=1))
    shift_b, scale_b, gate_b = mod[:, M:2 * M], _rnd(1.0 + mod[:, 2 * M:3 * M]), mod[:, 3 * M:]
    w_r = jnp.broadcast_to(wr_v[...].astype(F32).reshape(1, M), (8, M))
    for name, v in zip(vectors, (mod[:, :M], shift_b, scale_b, gate_b, scale_b * w_r,
                                 gate_b * scale_b, gate_b * shift_b)):
        set_vector(name, v)
    out_copies = [pltpu.make_async_copy(out_v.at[rows(i)], out_hbm.at[rows(i)], sem_a.at[i])
                  for i in range(nb)]

    def residual(j, r, attn):
        gate, = vector("gate_a", CH, [j])
        return x_v[r:r + CH, j * T:(j + 1) * T].astype(F32) + gate * attn

    def finalize(r):
        x1_at = [pl.ds(_OFF["O"] + j * S + r, FR) for j in range(MT)]
        mean_at, inv_at = pl.ds(_OFF["MX"] + r, FR), pl.ds(_OFF["M"] + r, FR)

        def keep_mean():
            w[mean_at, :] = _row_sum([w[a, :] for a in x1_at]) * (1.0 / M)

        def keep_moments():
            mean = w[mean_at, :]
            centred = [w[a, :] - mean for a in x1_at]
            var = _row_sum([d * d for d in centred]) * (1.0 / M)
            dot = _row_sum([d * v for d, v in zip(centred, vector("route", FR))])
            w[inv_at, :] = lax.rsqrt(var + EPS)
            lane = lax.broadcasted_iota(I32, (8, T), 1)
            for n, v in enumerate((var, dot)):
                at = pl.ds(_OFF["R"] + 16 * n + r // (8 * T) * 8, 8)
                tile = w[at, :]
                for t in range(0, FR, 8):
                    tile = jnp.where(lane == (r + t) // 8 % T, v[t:t + 8], tile)
                w[at, :] = tile

        def output():
            mean, inv_std = w[mean_at, :], w[inv_at, :]
            out = [(w[a, :] - mean) * inv_std * g + (w[a, :] + b)
                   for a, g, b in zip(x1_at, vector("gain", FR), vector("bias", FR))]
            out_v[r:r + FR, :] = jnp.concatenate(out, axis=1).astype(BF)
            if r < S - 2 * BQ:
                w[pl.ds(_OFF["PAD"], 8), :] = pltpu.bitcast(
                    out_v[pl.ds(origin + r, 16), :T], F32)
            if (r + FR) % BQ == 0:
                out_copies[r // BQ].start()

        return [(_FIN_LAG, keep_mean), (2 * _FIN_LAG + 64, keep_moments),
                (2 * _FIN_LAG + 128, output)]

    _head(_SEQ_LAST, w, origin, wo_v.at[1], residual=residual, finalize=finalize,
          suffix="2")

    var, dot = w[_OFF["R"]:_OFF["R"] + 16, :], w[_OFF["R"] + 16:_OFF["R"] + 32, :]
    offset = jnp.sum((shift_b * w_r)[:1], axis=1, keepdims=True)
    score = _rnd(dot / _rnd(jnp.sqrt(_rnd(_rnd(var) + EPS))) + offset)
    bits = pltpu.bitcast(jnp.where(score == 0.0, 0.0, score), I32) >> 16
    rank = jnp.where(bits < 0, -1 - bits, bits + 0x8000)
    rank = jnp.where(score != score, 0, rank)
    sub = lax.broadcasted_iota(I32, (16, T), 0)
    row = (sub >> 3) * (8 * T) + 8 * lax.broadcasted_iota(I32, (16, T), 1) + (sub & 7)
    key = pltpu.bitcast((rank << 11) | (S - 1 - row) | (1 << 29), F32)
    best = jnp.broadcast_to(jnp.max(key, axis=0, keepdims=True), (T, T))
    place = jnp.sum(jnp.where(best.T > best, 1.0, 0.0), axis=0, keepdims=True)
    chosen = place == lax.broadcasted_iota(I32, (TOPK, T), 0).astype(F32)
    key = jnp.concatenate([jnp.where(chosen, key[n:n + 1], 0.0) for n in range(16)], axis=0)
    key = jnp.broadcast_to(jnp.max(key, axis=1, keepdims=True), key.shape)
    picked = []
    for _ in range(TOPK):
        top = jnp.max(key, axis=0, keepdims=True)
        key = jnp.where(key == top, 0.0, key)
        top = pltpu.bitcast(jnp.broadcast_to(top, (8, T)), I32)
        picked.append(S - 1 - (top[0, 0] & (S - 1)))

    wait(out_copies[:-2])

    def gather(at):
        return jnp.concatenate([w[pl.ds(at + r, 1), :] for r in picked], axis=0)

    x1 = [gather(_OFF["O"] + j * S) for j in range(MT)]
    mean, inv_std = gather(_OFF["MX"]), gather(_OFF["M"])
    h2 = [_rnd((t - mean) * inv_std * a + b)
          for t, a, b in zip(x1, vector("scale_b", 8), vector("shift_b", 8))]
    x1, h2 = jnp.concatenate(x1, axis=1), jnp.concatenate(h2, axis=1)
    r_sel = jnp.sum(h2 * w_r, axis=1, keepdims=True)
    gu = _rnd(jnp.concatenate([_nn(h2.astype(BF), pltpu.bitcast(wgu_t[j], BF))
                               for j in range(2 * F // T)], axis=1))
    g, u = gu[:, :F], gu[:, F:]
    hidden = (_rnd(g * jax.nn.sigmoid(g)) * u).astype(BF)
    wait(out_copies[-2:])
    y = _nn(hidden, wd_v[...])
    new = x1 + jnp.concatenate(vector("gate_b", 8), axis=1) * (h2 + y * jax.nn.sigmoid(r_sel))

    groups = [pl.ds(pl.multiple_of((r >> 4) << 4, 16), 16) for r in picked]
    line = lax.broadcasted_iota(I32, (16, M), 0)
    for n, r in enumerate(picked):
        old = out_v[groups[n], :].astype(F32)
        out_v[groups[n], :] = jnp.where(line == (r & 15), new[n:n + 1], old).astype(BF)

    fixes = []
    for n, r in enumerate(picked):
        fresh = True
        for earlier in picked[:n]:
            fresh = jnp.logical_and(fresh, (earlier >> 4) != (r >> 4))
        fixes.append((fresh, pltpu.make_async_copy(
            out_v.at[groups[n]], out_hbm.at[groups[n]], sem_a.at[n])))
    for fresh, copy in fixes:
        pl.when(fresh)(copy.start)
    for fresh, copy in fixes:
        pl.when(fresh)(copy.wait)


@jax.jit
def pallas_adaLN_cond__compressed_kv_cla__moe_arch_mod__prompt_kernel(
    A_x: jax.Array,
    A_c_kv: jax.Array,
    A_w_q: jax.Array,
    A_w_uk: jax.Array,
    A_w_uv: jax.Array,
    A_w_o: jax.Array,
    B_x: jax.Array,
    B_w_r: jax.Array,
    B_w_gate: jax.Array,
    B_w_up: jax.Array,
    B_w_down: jax.Array,
    c: jax.Array,
    w_mod: jax.Array,
):
    del B_x
    assert A_x.shape == (1, S, M) and A_c_kv.shape == (1, S, C)
    assert A_w_q.shape == (M, H, D) and B_w_gate.shape == (M, F)
    dma = pltpu.SemaphoreType.DMA
    out = pl.pallas_call(
        _kernel,
        in_specs=[pl.BlockSpec(memory_space=pl.ANY)] * 12,
        out_specs=pl.BlockSpec(memory_space=pl.ANY),
        out_shape=jax.ShapeDtypeStruct((S, M), BF),
        scratch_shapes=[
            pltpu.VMEM((_ROWS, T), F32),
            pltpu.VMEM((S, M), BF), pltpu.VMEM((S, C), BF),
            pltpu.VMEM((H // 2, M // 2, 2, 2, D), BF), pltpu.VMEM((H // 2, C // 2, 2, 2, D), BF),
            pltpu.VMEM((H // 2, C // 2, 2, 2, D), BF), pltpu.VMEM((H, D, M), BF),
            pltpu.VMEM((M,), BF),
            pltpu.VMEM((2 * F, M), BF), pltpu.VMEM((2 * F // T, M // 2, T), F32),
            pltpu.VMEM((F, M), BF),
            pltpu.VMEM((1, M), BF),
            pltpu.VMEM((6, M, M), BF), pltpu.VMEM((M, T), F32), pltpu.VMEM((6 * MT, 8, T), F32),
            pltpu.VMEM((M, T), U32),
            pltpu.VMEM((S, M), BF),
            dma((8,)), dma((4,)), dma((3,)), dma((3,)),
        ],
        compiler_params=pltpu.CompilerParams(vmem_limit_bytes=100 * 2 ** 20),
        name="adaln_attn_moe",
    )(A_x[0], A_c_kv[0], A_w_q.reshape(M // 2, 2, H, D), A_w_uk.reshape(C // 2, 2, H, D),
      A_w_uv.reshape(C // 2, 2, H, D), A_w_o, B_w_r,
      B_w_gate.T, B_w_up.T, B_w_down, c, w_mod)
    return out[None]
```

```python
import jax
import jax.numpy as jnp
from jax import lax
import jax.experimental.pallas as pl
import jax.experimental.pallas.tpu as pltpu

BF = jnp.bfloat16
F32 = jnp.float32
I32 = jnp.int32
U32 = jnp.uint32

S = 2048
M = 640
C = 512
H = 32
D = 128
F = 1728
TOPK = 8
EPS = 1e-5
LOG2E = 1.4426950408889634
QSCALE = D ** -0.5 * LOG2E
MASKED = -1e9 * LOG2E

T = 128
BQ = 256
CH = 64
MT = M // T
CT = C // T

_OFF = {}
_ROWS = 0
for _name, _n in (
    ("H", MT * S // 2), ("C", CT * S // 2),
    ("Q", S // 2), ("K", S // 2), ("V", S // 2), ("X", S // 2),
    ("Wq", M // 2), ("Wk", C // 2), ("Wv", C // 2),
    ("Q2", S // 2), ("K2", S // 2), ("V2", S // 2), ("Wq2", M // 2), ("Wk2", C // 2), ("Wv2", C // 2),
    ("S", (S // BQ) ** 2 * BQ), ("SD", S // 2),
    ("MX", S), ("M", S), ("L", S), ("ACC", 3 * BQ), ("PA", S),
    ("O", MT * S), ("D", T), ("R", 32), ("PAD", 8), ("MOD", 7 * MT * 8),
):
    _OFF[_name] = _ROWS
    _ROWS += _n

_SEQ = (
    "q0 k0 q1 k1 q2 v0 A0+A1 A0 q3 q4 B0 A1 k2 v1 q5 B1 A2 B0+A2 q6 q7 v2 k3 "
    "B2 A3 B1+A3 v3 k4 k5 k6 k7 B3 A4 B2+A4 v4 v5 v6 v7 B4 A5 B3+A5 o0 o1 "
    "B5 A6 B4+A6 o2 o3 B6 A7 B5+A7 o4 o5 B6+B7 B7 o6 o7"
)
_SEQ_FIRST = (
    "A0+A1 A0 A1 A2+A3 A2 A3 B0+B1 B0 B1 A4+A5 A4 B2+B3 B2 B3 o0 o1 A5 A6+A7 A6 "
    "B4+B5 B4 B5 o2 o3 A7 o4 o5 B6+B7 B6 B7 o6 o7"
)
_SEQ_LAST = (
    "A0+A1 A0 A1 A2+A3 A2 q4 B0+B1 B0 B1 A3 o0 o1 B2 B2+A4 q5 o2 B3+A5 B3 "
    "A4 q6 o3 B4+A6 B4 A5 q7 o4 B5+A7 B5 A6 o5 A7 B6 B6+B7 B7 o6 o7"
)
_RES_LAG, _CTX_LAG, _MAX_LAG, _SUM_LAG = 208, 208, 192, 80
FR = 16
_FIN_STEP, _FIN_LAG = (64, 128), 192


def _slots(seq):
    lanes = []
    for word in seq.split():
        if "+" in word:
            lanes.append(tuple(
                (p[0], int(p[1:]), 2 * int(p[1:]) + 1, T) for p in word.split("+")))
        else:
            k, i = word[0], int(word[1:])
            n = {"q": MT, "k": CT, "v": CT, "o": MT, "A": 2 * i + 1, "B": 2 * i + 1}[k]
            lanes += [((k, i, j, 0),) for j in range(n)]
    assert len(lanes) % 4 == 0
    return [lanes[s:s + 4] for s in range(0, len(lanes), 4)]


def _nt(a, b):
    return lax.dot_general(a, b, (((1,), (1,)), ((), ())), preferred_element_type=F32)


def _nn(a, b):
    return jnp.dot(a, b, preferred_element_type=F32)


def _rnd(x):
    return x.astype(BF).astype(F32)


def _pack(x):
    return pltpu.bitcast(x.astype(BF), F32)


def _select_head(even, odd, parity):
    down = jnp.asarray(16 * parity, U32)
    return pltpu.bitcast(((even >> down) & 0xFFFF) | ((odd >> down) << 16), F32)


def _head(seq, w, zero, wo, *, assign=False, next_weights=None, residual=None,
          finalize=None, extras=(), suffix=""):
    def load(r, n):
        return w[r:r + n, :]

    def ordered(r, n):
        head = w[pl.ds(zero + r, 8), :]
        return head if n == 8 else jnp.concatenate([head, load(r + 8, n - 8)], axis=0)

    def store(r, v):
        w[r:r + v.shape[0], :] = v

    def s_row(i, j, t, half):
        if half:
            return _OFF["SD"] + i * T + t - T
        return _OFF["S"] + (i * i + j) * BQ + t

    events = []

    def at(time, rank, fn):
        events.append((time, rank, len(events), fn))

    slots = _slots(seq)
    left = {}
    for slot in slots:
        for lane in slot:
            for k, i, _, t0 in lane:
                for t in range(t0, BQ, CH):
                    left[k, i, t] = left.get((k, i, t), 0) + 1
    has_sum, has_acc, last_use, complete = set(), set(), {}, {}
    pending = {}

    def expect(*tag):
        pending[tag] = pending.get(tag, 0) + 1

    def settled(*tag):
        assert not pending.get(tag), tag

    for s, slot in enumerate(slots):
        base = BQ * s
        jobs = ([(lane[0], -T) for lane in slot if len(lane) == 2]
                + [(lane[0], 0) for lane in slot if len(lane) == 1]
                + [(lane[1], 0) for lane in slot if len(lane) == 2])
        lhs, res, groups = {}, {}, {}
        for job, shift in jobs:
            groups.setdefault((job[0], job[1], shift), []).append(job)
            last_use[job[0]] = base + BQ

        for (k, i, shift), group in groups.items():
            for t in range(0, BQ, CH):
                live = [job for job in group if t >= job[3]]
                if not live:
                    continue

                def fetch(k=k, i=i, t=t, live=live, lhs=lhs, first=(i, t) not in has_sum):
                    r = i * BQ + t
                    if k in "qkv":
                        src = _OFF["H" if k == "q" else "C"] + r // 2
                        for job in live:
                            get = ordered if job == live[0] else load
                            lhs[job, t] = get(src + job[2] * S // 2, CH // 2)
                    elif k in "Ao":
                        settled("q" if k == "A" else "B", i, t)
                        v = ordered(_OFF["Q" + suffix if k == "A" else "X"] + r // 2, CH // 2)
                        for job in live:
                            lhs[job, t] = v
                            if k == "A" and job[2] == 2 * i + t // T:
                                lhs["d", job, t] = ordered(_OFF["D"] + t % T, 8)
                    else:
                        settled("A", i, t)
                        settled("m", i, t)
                        settled("l", i, t)
                        expect("l", i, t)
                        m = ordered(_OFF["M"] + r, CH)
                        l = None if first else load(_OFF["L"] + r, CH)
                        for job in live:
                            p = jnp.exp2(load(s_row(i, job[2], t, job[3]), CH) - m)
                            l = p if l is None else l + p
                            lhs[job, t] = p
                        lhs["l", i, t] = l

                at(base + shift + t, 1, fetch)
                if k == "B":
                    has_sum.add((i, t))

                    def keep_sum(i=i, t=t, lhs=lhs):
                        pending["l", i, t] -= 1
                        store(_OFF["L"] + i * BQ + t, lhs["l", i, t])

                    at(base + shift + t + CH - 16 + _SUM_LAG, 0, keep_sum)

        for job, shift in jobs:
            def matmul(job=job, lhs=lhs, res=res):
                k, _, j, t0 = job
                a = jnp.concatenate([lhs[job, t] for t in range(t0, BQ, CH)], axis=0)
                a = a.astype(BF) if k == "B" else pltpu.bitcast(a, BF)
                if k == "o":
                    res[job] = _nn(a, wo[:, j * T:(j + 1) * T])
                    return
                region = {"A": "K", "B": "V"}.get(k, "W" + k)
                if k in "AB":
                    settled(region.lower(), j // 2, (j % 2) * T + T - CH)
                b = pltpu.bitcast(load(_OFF[region + suffix] + j * T // 2, T // 2), BF)
                res[job] = _nt(a, b) if k == "A" else _nn(a, b)

            at(base + shift + BQ - CH, 2, matmul)

        for (k, i, shift), group in groups.items():
            for t in range(0, BQ, CH):
                live = [job for job in group if t >= job[3]]
                if not live:
                    continue
                first = (k, i, t) not in has_acc
                has_acc.add((k, i, t))
                left[k, i, t] -= len(live)
                last = left[k, i, t] == 0

                def finish(k=k, i=i, t=t, live=live, lhs=lhs, res=res, first=first, last=last):
                    r = i * BQ + t
                    pending[k, i, t] -= 1
                    assert k == "o" or last == (pending[k, i, t] == 0), (k, i, t)
                    parts = [res[job][t - job[3]:t - job[3] + CH] for job in live]
                    if k == "o":
                        for job, v in zip(live, parts):
                            a = _OFF["O"] + job[2] * S + r
                            v = v if assign else load(a, CH) + v
                            store(a, residual(job[2], r, v) if residual else v)
                    elif k == "A":
                        mx = None if first else load(_OFF["MX"] + r, CH)
                        for job, v in zip(live, parts):
                            if job[2] == 2 * i + t // T:
                                d = lhs["d", job, t]
                                v = jnp.concatenate(
                                    [jnp.where(d <= u, v[u:u + 8], MASKED)
                                     for u in range(0, CH, 8)], axis=0)
                            store(s_row(i, job[2], t, job[3]), v)
                            mx = v if mx is None else jnp.maximum(mx, v)
                        if last:
                            res["m", i, t] = jnp.broadcast_to(
                                jnp.max(mx, axis=1, keepdims=True), (CH, T))
                        else:
                            store(_OFF["MX"] + r, mx)
                    else:
                        a = _OFF["PA"] + r if k == "B" else _OFF["ACC"] + "qkv".index(k) * BQ + t
                        acc = None if first else load(a, CH)
                        for v in parts:
                            acc = v if acc is None else acc + v
                        if not last:
                            store(a, acc)
                        elif k == "B":
                            settled("l", i, t)
                            l = jnp.sum(load(_OFF["L"] + r, CH), axis=1, keepdims=True)
                            store(_OFF["X"] + r // 2, _pack(acc * (1.0 / l)))
                        elif k == "q":
                            store(_OFF["Q" + suffix] + r // 2, _pack(acc * QSCALE))
                        else:
                            store(_OFF[k.upper() + suffix] + r // 2, _pack(acc))

                ready = base + shift + t + CH - 16 + (_CTX_LAG if k == "B" and last else _RES_LAG)
                when = max(base + shift + BQ, ready)
                expect(k, i, t)
                at(when, 0, finish)
                if k == "o" and last:
                    complete[i * BQ + t] = when
                if k == "A" and last:
                    def keep_max(i=i, t=t, res=res):
                        pending["m", i, t] -= 1
                        store(_OFF["M"] + i * BQ + t, res["m", i, t])

                    expect("m", i, t)
                    at(max(when, ready + _MAX_LAG), 0, keep_max)

    busy = [any(job[0] == "B" for s2 in (max(s - 1, 0), s) for lane in slots[s2] for job in lane)
            for s in range(len(slots))]
    if next_weights:
        todo = [(k, r) for k, n in (("q", M), ("k", C), ("v", C)) for r in range(0, n, 16)]
        calm = [s for s in range(last_use.get("q", 0) // BQ, len(slots) - 2) if not busy[s]]
        for n, (k, r) in enumerate(todo):
            step = BQ * len(calm) * n // len(todo)
            time = BQ * calm[step // BQ] + step % BQ
            assert time >= last_use.get(k, 0)
            at(time, 0, lambda k=k, r=r: next_weights(k, r))
    for time, fn in extras:
        at(time, 0, fn)
    if finalize:
        time = 0
        for r in range(0, S, FR):
            heavy = time // BQ < len(slots) and busy[time // BQ]
            time = max(time + _FIN_STEP[heavy], complete[r // CH * CH])
            for delay, fn in finalize(r):
                at(time + delay, 0, fn)

    for event in sorted(events, key=lambda e: e[:3]):
        event[3]()


def _row_sum(tiles):
    total = tiles[0]
    for tile in tiles[1:]:
        total = total + tile
    return jnp.broadcast_to(jnp.sum(total, axis=1, keepdims=True), total.shape)


def _kernel(x_hbm, ckv_hbm, wq_hbm, wk_hbm, wv_hbm, wo_hbm, wr_hbm, wg_hbm, wu_hbm,
            wd_hbm, c_hbm, wmod_hbm, out_hbm,
            w, x_v, ckv_v, wq_v, wk_v, wv_v, wo_v, wr_v, wgu_v, wgu_t, wd_v, c_v,
            wmod_v, silu_v, mod_v, rows_v, out_v, sem_a, sem_b, sem_m, sem_w):
    pairs = {"q": wq_v, "k": wk_v, "v": wv_v}
    nb = S // BQ

    def rows(i):
        return pl.ds(i * BQ, BQ)

    def pair_copies(p):
        return [pltpu.make_async_copy(src.at[:, :, pl.ds(2 * p, 2), :], dst.at[p], sem_w.at[n])
                for n, (src, dst) in enumerate(((wq_hbm, wq_v), (wk_hbm, wk_v), (wv_hbm, wv_v)))]

    def later_pairs_wait():
        for n, dst in enumerate((wq_v, wk_v, wv_v)):
            rest = dst.at[pl.ds(3, H // 2 - 3)]
            pltpu.make_async_copy(rest, rest, sem_w.at[n]).wait()

    def pair_rows(k, slot, r):
        return [pltpu.bitcast(pairs[k][slot, r // 2:r // 2 + 8, odd], U32).reshape(8, T)
                for odd in range(2)]

    def weights_of(h):
        def select(k, r):
            a = _OFF["W" + k] + r // 2
            w[a:a + 8, :] = _select_head(*pair_rows(k, h >> 1, r), h & 1)
        return select

    def weight(k, n):
        return pltpu.bitcast(w[_OFF["W" + k]:_OFF["W" + k] + n // 2, :], BF)

    def put(region, i, v):
        for j in range(v.shape[1] // T):
            a = _OFF[region] + (j * S + i * BQ) // 2
            w[a:a + v.shape[0], :] = v[:, j * T:(j + 1) * T]

    c_copy = pltpu.make_async_copy(c_hbm, c_v, sem_m.at[2])
    mod_copies = [pltpu.make_async_copy(wmod_hbm.at[:, pl.ds(n * M, M)], wmod_v.at[n],
                                        (sem_m if n < 2 else sem_a).at[n]) for n in range(6)]
    wo_first, wo_next, wo_rest = [
        pltpu.make_async_copy(wo_hbm.at[heads], wo_v.at[heads], sem) for heads, sem in (
            (pl.ds(0, 1), sem_b.at[0]), (pl.ds(1, 4), sem_b.at[1]), (pl.ds(5, H - 5), sem_b.at[2]))]
    wg_copy = pltpu.make_async_copy(wg_hbm, wgu_v.at[pl.ds(0, F)], sem_b.at[3])
    wu_copy = pltpu.make_async_copy(wu_hbm, wgu_v.at[pl.ds(F, F)], sem_a.at[0])
    wd_copy = pltpu.make_async_copy(wd_hbm, wd_v, sem_a.at[1])
    wr_copy = pltpu.make_async_copy(wr_hbm, wr_v, sem_a.at[6])
    x_copies = [pltpu.make_async_copy(x_hbm.at[rows(i)], x_v.at[rows(i)], sem_a.at[i])
                for i in range(nb)]
    ckv_groups = ((0,), (1, 2), (3, 4, 5), (6, 7))
    ckv_copies = [
        pltpu.make_async_copy(ckv_hbm.at[pl.ds(g[0] * BQ, len(g) * BQ)],
                              ckv_v.at[pl.ds(g[0] * BQ, len(g) * BQ)], sem_b.at[n])
        for n, g in enumerate(ckv_groups)]

    def start(copies):
        for copy in copies:
            copy.start()

    def wait(copies):
        for copy in copies:
            copy.wait()

    def select_both(k, rs):
        for r in rs:
            rows_v[r:r + 8, :], rows_v[r + 8:r + 16, :] = pair_rows(k, 0, r)
            both = rows_v[r:r + 8, :], rows_v[r + 8:r + 16, :]
            for parity, name in enumerate(("W" + k, "W" + k + "2")):
                w[pl.ds(_OFF[name] + r // 2, 8), :] = _select_head(*both, parity)

    def project(name, i, src=None):
        region, n = ("H", M) if name[0] == "q" else ("C", C)
        if src is None:
            src = jnp.concatenate([w[pl.ds(_OFF[region] + (j * S + i * BQ) // 2, BQ // 2), :]
                                   for j in range(n // T)], axis=1)
        a, b = pltpu.bitcast(src, BF), weight(name, n)
        out = _nn(a[:, :4 * T], b[:4 * T])
        if name[0] == "q":
            out += jnp.concatenate([_nn(a[t:t + BQ // 4, 4 * T:], b[4 * T:])
                                    for t in range(0, BQ, BQ // 4)], axis=0)
            out *= QSCALE
        put(name.upper(), i, _pack(out))

    def take_ckv(n):
        for i in ckv_groups[n]:
            put("C", i, pltpu.bitcast(ckv_v[rows(i), :], F32))
        return [(name, i) for name in ("k", "k2", "v", "v2") for i in ckv_groups[n]]

    wq_copy, wk_copy, wv_copy = pair_copies(0)
    start([wk_copy, ckv_copies[0], wv_copy])
    w[_OFF["D"]:_OFF["D"] + T, :] = (
        lax.broadcasted_iota(I32, (T, T), 1) - lax.broadcasted_iota(I32, (T, T), 0)).astype(F32)
    w[_OFF["R"]:_OFF["R"] + 32, :] = jnp.zeros((32, T), F32)
    wk_copy.wait()
    ckv_copies[1].start()
    select_both("k", range(0, C, 16))
    origin = pl.multiple_of(pltpu.bitcast(w[_OFF["R"]:_OFF["R"] + 8, :], I32)[0, 0], 16)
    wait([ckv_copies[0], wv_copy])
    start([wq_copy, ckv_copies[2], c_copy])
    select_both("v", range(0, C, 16))
    for unit in take_ckv(0):
        project(*unit)
    ckv_copies[1].wait()
    start(mod_copies[:2])
    for unit in take_ckv(1):
        project(*unit)
    wait([ckv_copies[2], c_copy])
    start(x_copies[:2])
    for unit in take_ckv(2):
        project(*unit)
    c = jnp.broadcast_to(c_v[...].astype(F32), (16, M))
    silu_c = (c * jax.nn.sigmoid(c)).astype(BF)
    silu_v[...] = jnp.concatenate([silu_c.astype(F32)] * (T // 16), axis=0).T
    wait(mod_copies[:2] + [wq_copy])
    start([ckv_copies[3], x_copies[2]])
    shift_a = _rnd(_nn(silu_c, wmod_v[0])[:1])
    scale_a = _rnd(1.0 + _rnd(_nn(silu_c, wmod_v[1])[:1]))
    select_both("q", range(0, M, 16))

    needed = [x_copies[:1], x_copies[1:2], [x_copies[2], ckv_copies[3]], x_copies[3:4],
              x_copies[4:6], [], x_copies[6:], []]
    more = [x_copies[3:4], x_copies[4:5], x_copies[5:7], [x_copies[7]] + pair_copies(1),
            [wo_first], [], [], []]
    for i in range(nb):
        wait(needed[i])
        start(more[i])
        if i == 2:
            todo = take_ckv(3)
        if i in (2, 3):
            project(*todo[i - 2])
        if i >= 2:
            project(*todo[i])
        if i in (1, 4, 5, 6):
            project("q2", (1, 4, 5, 6).index(i))
        x = x_v[rows(i), :].astype(F32)
        xc = x - jnp.mean(x, axis=1, keepdims=True)
        var = jnp.mean(xc * xc, axis=1, keepdims=True)
        h = _pack(xc * lax.rsqrt(var + EPS) * scale_a + shift_a)
        put("H", i, h)
        project("q", i, h)
    wait([wo_first] + pair_copies(1))
    start(pair_copies(2) + [wo_next, wg_copy])

    _head(_SEQ_FIRST, w, origin, wo_v.at[0], assign=True, next_weights=weights_of(2))

    wait(pair_copies(2) + [wo_next, wg_copy])
    for p in range(3, H // 2):
        start(pair_copies(p))
    start(mod_copies[2:] + [wo_rest, wu_copy, wd_copy, wr_copy])

    def head_step(h, carry):
        @pl.when(h == 5)
        def _():
            later_pairs_wait()
            wait(mod_copies[2:] + [wo_rest, wu_copy])

        pad = pl.ds(_OFF["PAD"], 8)

        def modulation(k):
            lanes = pl.ds(pl.multiple_of(lax.rem(h - 2, MT) * T, T), T)
            tile = wmod_v[lax.div(h - 2, MT), pl.ds(k * T, T), lanes].astype(F32)
            part = jnp.sum(silu_v[pl.ds(k * T, T), :] * tile, axis=0, keepdims=True)
            total = jnp.broadcast_to(part, (8, T)) + (w[pad, :] if k else 0.0)
            w[pad, :] = total
            if k == MT - 1:
                mod_v[h - 2] = total

        def transpose():
            n = jnp.minimum(h - 2, 2 * F // T - 1)
            wgu_t[n] = pltpu.bitcast(wgu_v[pl.ds(pl.multiple_of(n * T, T), T), :].T, F32)
            w[pad, :] = wgu_t[n + origin, :8, :]

        extras = [(T * (k + 1), lambda k=k: modulation(k)) for k in range(MT)]
        _head(_SEQ, w, origin, wo_v.at[h], next_weights=weights_of(jnp.minimum(h + 1, H - 1)),
              extras=extras + [(5 * BQ, transpose)])
        return carry

    assert H - 2 == 6 * MT >= 2 * F // T
    lax.fori_loop(2, H, head_step, 0)

    wait([wd_copy, wr_copy])
    vectors = ("gate_a", "shift_b", "scale_b", "gate_b", "route", "gain", "bias")

    def set_vector(name, v):
        for j in range(MT):
            a = _OFF["MOD"] + (vectors.index(name) * MT + j) * 8
            w[a:a + 8, :] = v[:, j * T:(j + 1) * T]

    def vector(name, n, tiles=range(MT)):
        a = _OFF["MOD"] + vectors.index(name) * MT * 8
        return [jnp.concatenate([w[a + 8 * j:a + 8 * j + 8, :]] * (n // 8), axis=0)
                for j in tiles]

    mod = _rnd(jnp.concatenate([mod_v[j] for j in range(2 * MT, 6 * MT)], axis=1))
    shift_b, scale_b, gate_b = mod[:, M:2 * M], _rnd(1.0 + mod[:, 2 * M:3 * M]), mod[:, 3 * M:]
    w_r = jnp.broadcast_to(wr_v[...].astype(F32).reshape(1, M), (8, M))
    for name, v in zip(vectors, (mod[:, :M], shift_b, scale_b, gate_b, scale_b * w_r,
                                 gate_b * scale_b, gate_b * shift_b)):
        set_vector(name, v)
    out_copies = [pltpu.make_async_copy(out_v.at[rows(i)], out_hbm.at[rows(i)], sem_a.at[i])
                  for i in range(nb)]

    def residual(j, r, attn):
        gate, = vector("gate_a", CH, [j])
        return x_v[r:r + CH, j * T:(j + 1) * T].astype(F32) + gate * attn

    def finalize(r):
        x1_at = [pl.ds(_OFF["O"] + j * S + r, FR) for j in range(MT)]
        mean_at, inv_at = pl.ds(_OFF["MX"] + r, FR), pl.ds(_OFF["M"] + r, FR)

        def keep_mean():
            w[mean_at, :] = _row_sum([w[a, :] for a in x1_at]) * (1.0 / M)

        def keep_moments():
            mean = w[mean_at, :]
            centred = [w[a, :] - mean for a in x1_at]
            var = _row_sum([d * d for d in centred]) * (1.0 / M)
            dot = _row_sum([d * v for d, v in zip(centred, vector("route", FR))])
            w[inv_at, :] = lax.rsqrt(var + EPS)
            lane = lax.broadcasted_iota(I32, (8, T), 1)
            for n, v in enumerate((var, dot)):
                at = pl.ds(_OFF["R"] + 16 * n + r // (8 * T) * 8, 8)
                tile = w[at, :]
                for t in range(0, FR, 8):
                    tile = jnp.where(lane == (r + t) // 8 % T, v[t:t + 8], tile)
                w[at, :] = tile

        def output():
            mean, inv_std = w[mean_at, :], w[inv_at, :]
            out = [(w[a, :] - mean) * inv_std * g + (w[a, :] + b)
                   for a, g, b in zip(x1_at, vector("gain", FR), vector("bias", FR))]
            out_v[r:r + FR, :] = jnp.concatenate(out, axis=1).astype(BF)
            if r < S - 2 * BQ:
                w[pl.ds(_OFF["PAD"], 8), :] = pltpu.bitcast(
                    out_v[pl.ds(origin + r, 16), :T], F32)
            if (r + FR) % BQ == 0:
                out_copies[r // BQ].start()

        return [(_FIN_LAG, keep_mean), (2 * _FIN_LAG + 64, keep_moments),
                (2 * _FIN_LAG + 128, output)]

    _head(_SEQ_LAST, w, origin, wo_v.at[1], residual=residual, finalize=finalize,
          suffix="2")

    var, dot = w[_OFF["R"]:_OFF["R"] + 16, :], w[_OFF["R"] + 16:_OFF["R"] + 32, :]
    offset = jnp.sum((shift_b * w_r)[:1], axis=1, keepdims=True)
    score = _rnd(dot / _rnd(jnp.sqrt(_rnd(_rnd(var) + EPS))) + offset)
    bits = pltpu.bitcast(jnp.where(score == 0.0, 0.0, score), I32) >> 16
    rank = jnp.where(bits < 0, -1 - bits, bits + 0x8000)
    rank = jnp.where(score != score, 0, rank)
    sub = lax.broadcasted_iota(I32, (16, T), 0)
    row = (sub >> 3) * (8 * T) + 8 * lax.broadcasted_iota(I32, (16, T), 1) + (sub & 7)
    key = pltpu.bitcast((rank << 11) | (S - 1 - row) | (1 << 29), F32)
    best = jnp.broadcast_to(jnp.max(key, axis=0, keepdims=True), (T, T))
    place = jnp.sum(jnp.where(best.T > best, 1.0, 0.0), axis=0, keepdims=True)
    chosen = place == lax.broadcasted_iota(I32, (TOPK, T), 0).astype(F32)
    key = jnp.concatenate([jnp.where(chosen, key[n:n + 1], 0.0) for n in range(16)], axis=0)
    key = jnp.broadcast_to(jnp.max(key, axis=1, keepdims=True), key.shape)
    picked = []
    for _ in range(TOPK):
        top = jnp.max(key, axis=0, keepdims=True)
        key = jnp.where(key == top, 0.0, key)
        top = pltpu.bitcast(jnp.broadcast_to(top, (8, T)), I32)
        picked.append(S - 1 - (top[0, 0] & (S - 1)))

    wait(out_copies[:-2])

    def gather(at):
        return jnp.concatenate([w[pl.ds(at + r, 1), :] for r in picked], axis=0)

    x1 = [gather(_OFF["O"] + j * S) for j in range(MT)]
    mean, inv_std = gather(_OFF["MX"]), gather(_OFF["M"])
    h2 = [_rnd((t - mean) * inv_std * a + b)
          for t, a, b in zip(x1, vector("scale_b", 8), vector("shift_b", 8))]
    x1, h2 = jnp.concatenate(x1, axis=1), jnp.concatenate(h2, axis=1)
    r_sel = jnp.sum(h2 * w_r, axis=1, keepdims=True)
    gu = _rnd(jnp.concatenate([_nn(h2.astype(BF), pltpu.bitcast(wgu_t[j], BF))
                               for j in range(2 * F // T)], axis=1))
    g, u = gu[:, :F], gu[:, F:]
    hidden = (_rnd(g * jax.nn.sigmoid(g)) * u).astype(BF)
    wait(out_copies[-2:])
    y = _nn(hidden, wd_v[...])
    new = x1 + jnp.concatenate(vector("gate_b", 8), axis=1) * (h2 + y * jax.nn.sigmoid(r_sel))

    groups = [pl.ds(pl.multiple_of((r >> 4) << 4, 16), 16) for r in picked]
    line = lax.broadcasted_iota(I32, (16, M), 0)
    for n, r in enumerate(picked):
        old = out_v[groups[n], :].astype(F32)
        out_v[groups[n], :] = jnp.where(line == (r & 15), new[n:n + 1], old).astype(BF)

    fixes = []
    for n, r in enumerate(picked):
        fresh = True
        for earlier in picked[:n]:
            fresh = jnp.logical_and(fresh, (earlier >> 4) != (r >> 4))
        fixes.append((fresh, pltpu.make_async_copy(
            out_v.at[groups[n]], out_hbm.at[groups[n]], sem_a.at[n])))
    for fresh, copy in fixes:
        pl.when(fresh)(copy.start)
    for fresh, copy in fixes:
        pl.when(fresh)(copy.wait)


@jax.jit
def pallas_adaLN_cond__compressed_kv_cla__moe_arch_mod__prompt_kernel(
    A_x: jax.Array,
    A_c_kv: jax.Array,
    A_w_q: jax.Array,
    A_w_uk: jax.Array,
    A_w_uv: jax.Array,
    A_w_o: jax.Array,
    B_x: jax.Array,
    B_w_r: jax.Array,
    B_w_gate: jax.Array,
    B_w_up: jax.Array,
    B_w_down: jax.Array,
    c: jax.Array,
    w_mod: jax.Array,
):
    del B_x
    assert A_x.shape == (1, S, M) and A_c_kv.shape == (1, S, C)
    assert A_w_q.shape == (M, H, D) and B_w_gate.shape == (M, F)
    dma = pltpu.SemaphoreType.DMA
    out = pl.pallas_call(
        _kernel,
        in_specs=[pl.BlockSpec(memory_space=pl.ANY)] * 12,
        out_specs=pl.BlockSpec(memory_space=pl.ANY),
        out_shape=jax.ShapeDtypeStruct((S, M), BF),
        scratch_shapes=[
            pltpu.VMEM((_ROWS, T), F32),
            pltpu.VMEM((S, M), BF), pltpu.VMEM((S, C), BF),
            pltpu.VMEM((H // 2, M // 2, 2, 2, D), BF), pltpu.VMEM((H // 2, C // 2, 2, 2, D), BF),
            pltpu.VMEM((H // 2, C // 2, 2, 2, D), BF), pltpu.VMEM((H, D, M), BF),
            pltpu.VMEM((M,), BF),
            pltpu.VMEM((2 * F, M), BF), pltpu.VMEM((2 * F // T, M // 2, T), F32),
            pltpu.VMEM((F, M), BF),
            pltpu.VMEM((1, M), BF),
            pltpu.VMEM((6, M, M), BF), pltpu.VMEM((M, T), F32), pltpu.VMEM((6 * MT, 8, T), F32),
            pltpu.VMEM((M, T), U32),
            pltpu.VMEM((S, M), BF),
            dma((8,)), dma((4,)), dma((3,)), dma((3,)),
        ],
        compiler_params=pltpu.CompilerParams(vmem_limit_bytes=100 * 2 ** 20),
        name="adaln_attn_moe",
    )(A_x.reshape(S, M), A_c_kv.reshape(S, C),
      A_w_q.reshape(M // 2, 2, H, D), A_w_uk.reshape(C // 2, 2, H, D),
      A_w_uv.reshape(C // 2, 2, H, D), A_w_o, B_w_r,
      B_w_gate.T, B_w_up.T, B_w_down, c, w_mod)
    return out.reshape(1, S, M)
```
